```python
import jax
import jax.numpy as jnp

def _softmax(x, axis=-1):
    return jax.nn.softmax(x, axis=axis)

def _gelu(x):
    return jax.nn.gelu(x, approximate=True)

def _silu(x):
    return jax.nn.silu(x)

def _sigmoid(x):
    return jax.nn.sigmoid(x)

def _layernorm(x, axis=-1, eps=1e-05):
    m = jnp.mean(x, axis=axis, keepdims=True)
    v = jnp.var(x, axis=axis, keepdims=True)
    return (x - m) / jnp.sqrt(v + eps)

def _scatter_add(tgt, idx, src, axis=0):
    return tgt.at[idx].add(src)

def _segment_sum(src, seg, n):
    return jax.ops.segment_sum(src, seg, n)

class _Rng:

    def __init__(self, key):
        self._k = key

    def _next(self):
        self._k, sub = jax.random.split(self._k)
        return sub

    def normal(self, shape):
        return jax.random.normal(self._next(), shape, dtype=jnp.bfloat16)

    def randint(self, lo, hi, shape):
        return jax.random.randint(self._next(), shape, lo, hi, dtype=jnp.int32)

    def uniform(self, shape, lo=0.0, hi=1.0):
        return jax.random.uniform(self._next(), shape, jnp.bfloat16, lo, hi)

    def permutation(self, n):
        return jax.random.permutation(self._next(), n)
kernel_name = 'interleave_layers__linear_kernel_hedgehog__memory_aug_recurrent_mem_tr__prompt'

def setup_inputs():
    _rng = _Rng(jax.random.key(int.from_bytes(__import__("os").urandom(4), "little")))
    _w = lambda a: (lambda t: t.astype(jnp.bfloat16) if jnp.issubdtype(t.dtype, jnp.floating) else t)(jnp.asarray(a))

    def _A_setup():
        B, S, D, H = (1, 2048, 640, 32)
        Dh = D // H
        return {'x': _w((lambda *s: _rng.normal(s) * 0.05)(B, S, D)), 'wqkv': _w((lambda *s: _rng.normal(s) * 0.05)(D, 3 * D)), 'w_phi': _w((lambda *s: _rng.normal(s) * 0.05)(H, Dh, Dh) * Dh ** (-0.5)), 'wo': _w((lambda *s: _rng.normal(s) * 0.05)(D, D))}
    _A_in = _A_setup()

    def _B_setup():
        B, S, Dm = (1, 2048, 640)
        H, Dh = (32, 192)
        M, seg = (8, 32)
        seg = min(seg, S)
        S = S // seg * seg
        return {'x': _w((lambda *s: _rng.normal(s) * 0.05)(B, S, Dm)), 'mem0': _w((lambda *s: _rng.normal(s) * 0.05)(B, M, Dm)), 'Wq': _w((lambda *s: _rng.normal(s) * 0.05)(Dm, H, Dh) * Dm ** (-0.5)), 'Wk': _w((lambda *s: _rng.normal(s) * 0.05)(Dm, H, Dh) * Dm ** (-0.5)), 'Wv': _w((lambda *s: _rng.normal(s) * 0.05)(Dm, H, Dh) * Dm ** (-0.5)), 'Wo': _w((lambda *s: _rng.normal(s) * 0.05)(H, Dh, Dm) * (H * Dh) ** (-0.5)), 'seg_len': seg}
    _B_in = _B_setup()
    return {'A_x': _A_in['x'], 'A_wqkv': _A_in['wqkv'], 'A_w_phi': _A_in['w_phi'], 'A_wo': _A_in['wo'], 'B_x': _B_in['x'], 'B_mem0': _B_in['mem0'], 'B_Wq': _B_in['Wq'], 'B_Wk': _B_in['Wk'], 'B_Wv': _B_in['Wv'], 'B_Wo': _B_in['Wo'], 'B_seg_len': _B_in['seg_len']}

def reference(A_x, A_wqkv, A_w_phi, A_wo, B_x, B_mem0, B_Wq, B_Wk, B_Wv, B_Wo, B_seg_len):

    def _A_ref(x, wqkv, w_phi, wo):
        B, S, D = x.shape
        H = 32
        Dh = D // H
        qkv = (lambda x, *d: x.transpose(*d))((x @ wqkv).reshape(B, S, 3, H, Dh), 2, 0, 3, 1, 4)
        q, k, v = (qkv[0], qkv[1], qkv[2])
        pq = jnp.einsum('bhsd,hdf->bhsf', q, w_phi)
        pk = jnp.einsum('bhsd,hdf->bhsf', k, w_phi)
        phi_q = jnp.concatenate([_softmax(pq, axis=-1), _softmax(-pq, axis=-1)], axis=-1)
        phi_k = jnp.concatenate([_softmax(pk, axis=-1), _softmax(-pk, axis=-1)], axis=-1)
        kv = jnp.einsum('bhsf,bhsd->bhfd', phi_k, v)
        z = jnp.einsum('bhsf->bhf', phi_k)
        num = jnp.einsum('bhqf,bhfd->bhqd', phi_q, kv)
        den = jnp.einsum('bhqf,bhf->bhq', phi_q, z)[..., None] + 1e-06
        o = num / den
        return (lambda x, *d: x.transpose(*d))(o, 0, 2, 1, 3).reshape(B, S, D) @ wo

    def _B_ref(x, mem0, Wq, Wk, Wv, Wo, seg_len):
        B, S, Dm = x.shape
        H, Dh = (Wq.shape[1], Wq.shape[2])
        M = mem0.shape[1]
        scale = Dh ** (-0.5)
        n_seg = S // seg_len
        L = M + seg_len
        idx = jnp.arange(L)
        mask = (idx[:, None] < M) | (idx[:, None] >= idx[None, :])
        mem = mem0
        outs = []
        for s in range(n_seg):
            xs = x[:, s * seg_len:(s + 1) * seg_len, :].copy()
            h = jnp.concatenate([mem, xs], axis=1)
            q = jnp.einsum('btd,dhe->bhte', h, Wq)
            k = jnp.einsum('btd,dhe->bhte', h, Wk)
            v = jnp.einsum('btd,dhe->bhte', h, Wv)
            scores = jnp.einsum('bhqe,bhke->bhqk', q, k) * scale
            scores = jnp.where(mask[None, None], scores, -1000000000.0)
            p = _softmax(scores, axis=-1)
            o = jnp.einsum('bhqk,bhke->bhqe', p, v)
            o = jnp.einsum('bhte,hed->btd', o, Wo)
            mem = o[:, :M, :].copy()
            outs.append(o[:, M:, :])
        return jnp.concatenate(outs, axis=1)
    x = A_x
    x = x + _A_ref(_layernorm(x, axis=-1), A_wqkv, A_w_phi, A_wo)
    x = x + _B_ref(_layernorm(x, axis=-1), B_mem0, B_Wq, B_Wk, B_Wv, B_Wo, B_seg_len)
    x = x + _A_ref(_layernorm(x, axis=-1), A_wqkv, A_w_phi, A_wo)
    x = x + _B_ref(_layernorm(x, axis=-1), B_mem0, B_Wq, B_Wk, B_Wv, B_Wo, B_seg_len)
    return x
```

```python
import functools

import jax
import jax.numpy as jnp
from jax import lax
import jax.experimental.pallas as pl
import jax.experimental.pallas.tpu as pltpu

f32 = jnp.float32
bf16 = jnp.bfloat16
u32 = jnp.uint32

S = 2048
D = 640
HA = 32
DA = D // HA
HB = 32
DB = 192
MEM = 8
SEG = 32
L = MEM + SEG
NSEG = S // SEG
NP = HB // 2
PW = 2 * DB
NG = 4
GR = DA * 8
TB = 256
NB = S // TB
LN_EPS = 1e-5

_NT = (((1,), (1,)), ((), ()))


def _layernorm(x):
    m = jnp.mean(x, axis=-1, keepdims=True)
    xc = x - m
    v = jnp.mean(xc * xc, axis=-1, keepdims=True)
    return xc * lax.rsqrt(v + LN_EPS)


def _hedgehog(p):
    rows = [p[8 * f:8 * (f + 1), :] for f in range(DA)]
    mx = functools.reduce(jnp.maximum, rows)
    mn = functools.reduce(jnp.minimum, rows)
    ep = [jnp.exp(r - mx) for r in rows]
    en = [jnp.exp(mn - r) for r in rows]
    rp = 1.0 / functools.reduce(jnp.add, ep)
    rn = 1.0 / functools.reduce(jnp.add, en)
    return jnp.concatenate([e * rp for e in ep] + [e * rn for e in en], axis=0)


def _blockdiag(x):
    t0, t1, t2 = x[:, :128], x[:, 128:256], x[:, 256:]
    lane = lax.broadcasted_iota(jnp.int32, (L, 128), 1)
    z = jnp.zeros((L, 128), f32)
    top = jnp.concatenate([t0, jnp.where(lane < 64, t1, 0.0), z], axis=1)
    bot = jnp.concatenate([z, jnp.where(lane >= 64, t1, 0.0), t2], axis=1)
    return jnp.concatenate([top, bot], axis=0)


def _kernel(x_ref, wqkv_ref, wp_ref, wo_ref, mem0_ref, wqt_hbm, wkt_hbm, wvt_hbm, wob_hbm,
            out_ref,
            xres_ref, xn_ref, wt_ref, wop_ref, kvt_ref, stage_ref, wb_ref, mem_ref, sems):
    scale = DB ** -0.5

    copies = [pltpu.make_async_copy(src, stage_ref.at[i], sems.at[i])
              for i, src in enumerate((wqt_hbm, wkt_hbm, wvt_hbm, wob_hbm))]
    for c in copies:
        c.start()

    row = lax.broadcasted_iota(jnp.int32, (GR, 256), 0)
    col = lax.broadcasted_iota(jnp.int32, (GR, 256), 1)
    wp = wp_ref[...].astype(f32)
    for g in range(NG):
        c = col + 128 * g
        lo = (8 * g + (row & 7)) * DA
        wpg = wp[:, 128 * g:128 * g + 256]
        bc = jnp.concatenate(
            [jnp.broadcast_to(wpg[f:f + 1, :], (8, 256)) for f in range(DA)], axis=0)
        phit = jnp.where((c >= lo) & (c < lo + DA), bc, 0.0).astype(bf16)
        permt = jnp.where(c == lo + (row >> 3), 1.0, 0.0).astype(bf16)
        for m, lhs in enumerate((phit, phit, permt)):
            w = wqkv_ref[:, m * D + 128 * g:m * D + 128 * g + 256]
            r = lax.dot_general(lhs, w, _NT, preferred_element_type=f32)
            wt_ref[m * NG + g] = r.astype(bf16)
        wop_ref[g * GR:(g + 1) * GR, :] = jnp.dot(
            permt, wo_ref[128 * g:128 * g + 256, :], preferred_element_type=f32).astype(bf16)

    xres_ref[...] = x_ref[...].astype(f32)

    def layer_a():
        kvt_ref[...] = jnp.zeros(kvt_ref.shape, f32)

        def phase1(b, carry):
            r0 = pl.multiple_of(b * TB, TB)
            xn = _layernorm(xres_ref[pl.ds(r0, TB), :]).astype(bf16)
            ones = jnp.ones((8, TB), f32)
            pk, v1 = {}, {}
            for t in range(NG + 1):
                if t < NG:
                    pk[t] = lax.dot_general(wt_ref[NG + t], xn, _NT, preferred_element_type=f32)
                    v1[t] = lax.dot_general(wt_ref[2 * NG + t], xn, _NT, preferred_element_type=f32)
                if t >= 1:
                    g = t - 1
                    phik = _hedgehog(pk[g]).astype(bf16)
                    lhs = jnp.concatenate([v1[g], ones], axis=0)
                    kvt_ref[g] += lax.dot_general(lhs, phik, _NT, preferred_element_type=f32)
            return carry

        lax.fori_loop(0, NB, phase1, 0)

        rr = lax.broadcasted_iota(jnp.int32, (GR + 8, 2 * GR), 0)
        cc = lax.broadcasted_iota(jnp.int32, (GR + 8, 2 * GR), 1)
        same_head = (rr & 7) == (cc & 7)
        for g in range(NG):
            kvt_ref[g] = jnp.where(same_head, kvt_ref[g], 0.0)

        def phase2(b, carry):
            r0 = pl.multiple_of(b * TB, TB)
            xb = xres_ref[pl.ds(r0, TB), :]
            xn = _layernorm(xb).astype(bf16)
            pq, ot = {}, {}
            for t in range(NG + 1):
                if t < NG:
                    pq[t] = lax.dot_general(wt_ref[t], xn, _NT, preferred_element_type=f32)
                if t >= 1:
                    g = t - 1
                    phiq = _hedgehog(pq[g]).astype(bf16)
                    num = jnp.dot(kvt_ref[g], phiq, preferred_element_type=f32)
                    rden = 1.0 / (num[GR:, :] + 1e-6)
                    ot[g] = jnp.concatenate(
                        [num[8 * d:8 * (d + 1), :] * rden for d in range(DA)], axis=0)
            o = jnp.concatenate([ot[g] for g in range(NG)], axis=0).astype(bf16).T
            xb = xb + jnp.dot(o, wop_ref[...], preferred_element_type=f32)
            xres_ref[pl.ds(r0, TB), :] = xb
            xn_ref[pl.ds(r0, TB), :] = _layernorm(xb)
            return carry

        lax.fori_loop(0, NB, phase2, 0)

    def prep_b():
        for c in copies:
            c.wait()

        def body(p, carry):
            r0 = pl.multiple_of(p * PW, PW)
            for m in range(3):
                blk = stage_ref[m, pl.ds(r0, PW), :]
                wb_ref[p, :, m * PW:(m + 1) * PW] = pltpu.bitcast(blk.T, u32)
            return carry

        lax.fori_loop(0, NP, body, 0)

    def layer_b():
        mem_ref[...] = mem0_ref[...].astype(f32)
        srow = lax.broadcasted_iota(jnp.int32, (L, 2 * L), 0)
        scol = lax.broadcasted_iota(jnp.int32, (L, 2 * L), 1)
        first = scol < L
        kidx = jnp.where(first, scol, scol - L)
        mask = (srow < MEM) | (srow >= kidx)

        def softmax(s):
            s = jnp.where(mask, s * scale, -1e9)
            m1 = jnp.max(jnp.where(first, s, -jnp.inf), axis=1, keepdims=True)
            m2 = jnp.max(jnp.where(first, -jnp.inf, s), axis=1, keepdims=True)
            e = jnp.exp(s - jnp.where(first, m1, m2))
            l1 = jnp.sum(jnp.where(first, e, 0.0), axis=1, keepdims=True)
            l2 = jnp.sum(jnp.where(first, 0.0, e), axis=1, keepdims=True)
            return e * jnp.where(first, 1.0 / l1, 1.0 / l2)

        def oproj(os_, p0, p1):
            o = jnp.concatenate([os_[p] for p in range(p0, p1)], axis=1)
            return jnp.dot(o, stage_ref[3, p0 * PW:p1 * PW, :], preferred_element_type=f32)

        def step(s, carry):
            r0 = pl.multiple_of(s * SEG, SEG)
            h = jnp.concatenate([mem_ref[...], xn_ref[pl.ds(r0, SEG), :]], axis=0)
            qkv, pr, os_ = {}, {}, {}
            acc = jnp.concatenate([jnp.zeros((MEM, D), f32), xres_ref[pl.ds(r0, SEG), :]], axis=0)
            for t in range(NP + 2):
                if t < NP:
                    qkv[t] = jnp.dot(h, pltpu.bitcast(wb_ref[t], bf16), preferred_element_type=f32)
                if t == NP:
                    acc = acc + oproj(os_, 0, 3)
                if t == NP + 1:
                    acc = acc + oproj(os_, 3, 7)
                if 0 <= t - 1 < NP:
                    q, k = qkv[t - 1][:, :PW], qkv[t - 1][:, PW:2 * PW]
                    pr[t - 1] = softmax(
                        lax.dot_general(q, _blockdiag(k), _NT, preferred_element_type=f32))
                if 0 <= t - 2 < NP:
                    os_[t - 2] = jnp.dot(pr[t - 2], _blockdiag(qkv[t - 2][:, 2 * PW:]),
                                         preferred_element_type=f32)
            acc = acc + oproj(os_, 7, NP)
            mem_ref[...] = acc[:MEM]
            xnew = acc[MEM:]
            xres_ref[pl.ds(r0, SEG), :] = xnew
            out_ref[pl.ds(r0, SEG), :] = xnew.astype(bf16)
            return carry

        lax.fori_loop(0, NSEG, step, 0)

    def layer(i, carry):
        layer_a()

        @pl.when(i == 0)
        def _():
            prep_b()

        layer_b()
        return carry

    lax.fori_loop(0, 2, layer, 0)


@functools.partial(jax.jit, static_argnames=("B_seg_len",))
def pallas_interleave_layers__linear_kernel_hedgehog__memory_aug_recurrent_mem_tr__prompt_kernel(
    A_x, A_wqkv, A_w_phi, A_wo, B_x, B_mem0, B_Wq, B_Wk, B_Wv, B_Wo, B_seg_len=SEG,
):
    del B_x
    assert B_seg_len == SEG
    x = A_x.reshape(S, D)
    wp = A_w_phi.transpose(2, 0, 1).reshape(DA, D)
    mem0 = B_mem0.reshape(MEM, D)
    wqt, wkt, wvt = (w.transpose(1, 2, 0).reshape(HB * DB, D) for w in (B_Wq, B_Wk, B_Wv))
    wob = B_Wo.reshape(HB * DB, D)

    vmem = pl.BlockSpec(memory_space=pltpu.VMEM)
    hbm = pl.BlockSpec(memory_space=pl.ANY)
    out = pl.pallas_call(
        _kernel,
        out_shape=jax.ShapeDtypeStruct((S, D), bf16),
        in_specs=[vmem, vmem, vmem, vmem, vmem, hbm, hbm, hbm, hbm],
        out_specs=vmem,
        scratch_shapes=[
            pltpu.VMEM((S, D), f32),
            pltpu.VMEM((S, D), f32),
            pltpu.VMEM((3 * NG, GR, D), bf16),
            pltpu.VMEM((D, D), bf16),
            pltpu.VMEM((NG, GR + 8, 2 * GR), f32),
            pltpu.VMEM((4, HB * DB, D), bf16),
            pltpu.VMEM((NP, D // 2, 3 * PW), u32),
            pltpu.VMEM((MEM, D), f32),
            pltpu.SemaphoreType.DMA((4,)),
        ],
        compiler_params=pltpu.CompilerParams(vmem_limit_bytes=110 * 1024 * 1024),
    )(x, A_wqkv, wp, A_wo, mem0, wqt, wkt, wvt, wob)
    return out.reshape(1, S, D)
```

```python
import functools

import jax
import jax.numpy as jnp
from jax import lax
import jax.experimental.pallas as pl
import jax.experimental.pallas.tpu as pltpu

f32 = jnp.float32
bf16 = jnp.bfloat16
u32 = jnp.uint32

S = 2048
D = 640
HA = 32
DA = D // HA
HB = 32
DB = 192
MEM = 8
SEG = 32
L = MEM + SEG
NSEG = S // SEG
NP = HB // 2
PW = 2 * DB
NG = 4
GR = DA * 8
TB = 256
NB = S // TB
LN_EPS = 1e-5
UNROLL = 2

_NT = (((1,), (1,)), ((), ()))


def _layernorm(x):
    m = jnp.mean(x, axis=-1, keepdims=True)
    xc = x - m
    v = jnp.mean(xc * xc, axis=-1, keepdims=True)
    return xc * lax.rsqrt(v + LN_EPS)


def _hedgehog(p):
    rows = [p[8 * f:8 * (f + 1), :] for f in range(DA)]
    mx = functools.reduce(jnp.maximum, rows)
    mn = functools.reduce(jnp.minimum, rows)
    ep = [jnp.exp(r - mx) for r in rows]
    en = [jnp.exp(mn - r) for r in rows]
    rp = 1.0 / functools.reduce(jnp.add, ep)
    rn = 1.0 / functools.reduce(jnp.add, en)
    return jnp.concatenate([e * rp for e in ep] + [e * rn for e in en], axis=0)


def _blockdiag(x):
    t0, t1, t2 = x[:, :128], x[:, 128:256], x[:, 256:]
    lane = lax.broadcasted_iota(jnp.int32, (L, 128), 1)
    z = jnp.zeros((L, 128), f32)
    top = jnp.concatenate([t0, jnp.where(lane < 64, t1, 0.0), z], axis=1)
    bot = jnp.concatenate([z, jnp.where(lane >= 64, t1, 0.0), t2], axis=1)
    return jnp.concatenate([top, bot], axis=0)


def _kernel(x_hbm, wqkv_hbm, wp_ref, wo_hbm, mem0_ref, wqt_hbm, wkt_hbm, wvt_hbm, wob_hbm,
            out_hbm,
            x_ref, wqkv_ref, wo_ref, xres_ref, xnb_ref, xna_ref, wt_ref, wop_ref, kvt_ref, ot_ref,
            stage_ref, wob_ref, wb_ref, mem_ref, obuf_ref, sem_a, sem_b, sem_o):
    scale = DB ** -0.5
    HS = S // 2
    CH = HB * DB // NB

    cp_kv = pltpu.make_async_copy(wqkv_hbm.at[:, D:], wqkv_ref.at[:, D:], sem_a.at[0])
    cp_x0 = pltpu.make_async_copy(x_hbm.at[:HS], x_ref.at[:HS], sem_a.at[1])
    cp_x1 = pltpu.make_async_copy(x_hbm.at[HS:], x_ref.at[HS:], sem_a.at[2])
    cp_q = pltpu.make_async_copy(wqkv_hbm.at[:, :D], wqkv_ref.at[:, :D], sem_a.at[3])
    cp_wo = pltpu.make_async_copy(wo_hbm, wo_ref, sem_a.at[4])
    cp_wob = pltpu.make_async_copy(wob_hbm, wob_ref, sem_a.at[5])

    def cp_b(m, c):
        src = (wqt_hbm, wkt_hbm, wvt_hbm)[m]
        r0 = c * CH if isinstance(c, int) else pl.multiple_of(c * CH, CH)
        return pltpu.make_async_copy(src.at[pl.ds(r0, CH)], stage_ref.at[m, pl.ds(r0, CH)],
                                     sem_b.at[m * NB + c])

    cp_kv.start()
    cp_x0.start()

    def prep_a(first):
        row = lax.broadcasted_iota(jnp.int32, (GR, 256), 0)
        col = lax.broadcasted_iota(jnp.int32, (GR, 256), 1)
        wp = wp_ref[...].astype(f32)
        for g in range(NG):
            c = col + 128 * g
            lo = (8 * g + (row & 7)) * DA
            wpg = wp[:, 128 * g:128 * g + 256]
            bc = jnp.concatenate(
                [jnp.broadcast_to(wpg[f:f + 1, :], (8, 256)) for f in range(DA)], axis=0)
            phit = jnp.where((c >= lo) & (c < lo + DA), bc, 0.0).astype(bf16)
            permt = jnp.where(c == lo + (row >> 3), 1.0, 0.0).astype(bf16)
            for m in ((1, 2) if first else (0,)):
                w = wqkv_ref[:, m * D + 128 * g:m * D + 128 * g + 256]
                r = lax.dot_general(permt if m == 2 else phit, w, _NT, preferred_element_type=f32)
                wt_ref[m * NG + g] = pltpu.bitcast(r.astype(bf16), u32)
            if not first:
                r = jnp.dot(permt, wo_ref[128 * g:128 * g + 256, :], preferred_element_type=f32)
                wop_ref[g * GR // 2:(g + 1) * GR // 2, :] = pltpu.bitcast(r.astype(bf16), u32)

    def wt(i):
        return pltpu.bitcast(wt_ref[i], bf16)

    def rows(b, n=TB):
        return pl.ds(b * n if isinstance(b, int) else pl.multiple_of(b * n, n), n)

    def layer_a(first):
        src_ref = x_ref if first else xres_ref

        def ln_a(b):
            xn = _layernorm(src_ref[rows(b), :].astype(f32)).astype(bf16)
            xna_ref[rows(b, TB // 2), :] = pltpu.bitcast(xn, u32)

        def load_xn(b):
            return pltpu.bitcast(xna_ref[rows(b, TB // 2), :], bf16)

        if first:
            cp_kv.wait()
            for c in (cp_x1, cp_q, cp_wo):
                c.start()
            prep_a(True)
            cp_x0.wait()
            for c in range(NB):
                for m in range(3):
                    cp_b(m, c).start()
            cp_wob.start()
        kvt_ref[...] = jnp.zeros(kvt_ref.shape, f32)
        ln_a(0)

        def phase1(b, carry):
            if first:
                @pl.when(b == NB // 2 - 1)
                def _():
                    cp_x1.wait()
            xn = load_xn(b)
            ones = jnp.ones((8, TB), f32)
            pk, v1 = {}, {}

            def proj_k(g):
                pk[g] = lax.dot_general(wt(NG + g), xn, _NT, preferred_element_type=f32)

            def proj_v(g):
                v1[g] = lax.dot_general(wt(2 * NG + g), xn, _NT, preferred_element_type=f32)

            def kv(g):
                phik = _hedgehog(pk[g]).astype(bf16)
                lhs = jnp.concatenate([v1[g], ones], axis=0)
                kvt_ref[g] += lax.dot_general(lhs, phik, _NT, preferred_element_type=f32)

            proj_k(0); proj_k(1); proj_v(0); proj_k(2); proj_v(1); kv(0)
            proj_k(3); proj_v(2); kv(1); proj_v(3); kv(2); kv(3)
            ln_a(jnp.minimum(b + 1, NB - 1))
            return carry

        lax.fori_loop(0, NB, phase1, 0)

        if first:
            cp_q.wait()
            cp_wo.wait()
            prep_a(False)
        rr = lax.broadcasted_iota(jnp.int32, (GR + 8, 2 * GR), 0)
        cc = lax.broadcasted_iota(jnp.int32, (GR + 8, 2 * GR), 1)
        same_head = (rr & 7) == (cc & 7)
        for g in range(NG):
            kvt_ref[g] = jnp.where(same_head, kvt_ref[g], 0.0)

        def phase2(b, do_q, do_o):
            if first and do_q:
                for m in range(3):
                    cp_b(m, b).wait()
            pq = {}
            if do_q:
                xn = load_xn(b)
            if do_o:
                o = pltpu.bitcast(ot_ref[...], bf16).T
                wop = pltpu.bitcast(wop_ref[...], bf16)

            def proj_q(g):
                if do_q:
                    pq[g] = lax.dot_general(wt(g), xn, _NT, preferred_element_type=f32)

            def num(g):
                if do_q:
                    phiq = _hedgehog(pq[g]).astype(bf16)
                    n = jnp.dot(kvt_ref[g], phiq, preferred_element_type=f32)
                    rden = 1.0 / (n[GR:, :] + 1e-6)
                    ot = jnp.concatenate(
                        [n[8 * d:8 * (d + 1), :] * rden for d in range(DA)], axis=0)
                    ot_ref[g * GR // 2:(g + 1) * GR // 2, :] = pltpu.bitcast(ot.astype(bf16), u32)

            def out(j):
                if do_o:
                    hb = TB // 2
                    r = rows(2 * (b - 1) + j, hb)
                    xb = src_ref[r, :].astype(f32) + jnp.dot(
                        o[j * hb:(j + 1) * hb], wop, preferred_element_type=f32)
                    xres_ref[r, :] = xb
                    xnb_ref[r, :] = _layernorm(xb)

            proj_q(0); proj_q(1); out(0); num(0); proj_q(2); num(1); proj_q(3); out(1)
            num(2); num(3)

            if first and do_q:
                for j in range(CH // PW):
                    p = b * (CH // PW) + j
                    for m in range(3):
                        blk = stage_ref[m, rows(p, PW), :]
                        wb_ref[p, :, m * PW:(m + 1) * PW] = pltpu.bitcast(blk.T, u32)

        phase2(0, True, False)

        def body2(b, carry):
            phase2(b, True, True)
            return carry

        lax.fori_loop(1, NB, body2, 0)
        phase2(NB, False, True)
        if first:
            cp_wob.wait()

    def out_copy(i):
        r = rows(i, UNROLL * SEG)
        return pltpu.make_async_copy(obuf_ref.at[r], out_hbm.at[r], sem_o)

    def layer_b(layer):
        mem_ref[...] = mem0_ref[...].astype(f32)
        srow = lax.broadcasted_iota(jnp.int32, (L, 2 * L), 0)
        scol = lax.broadcasted_iota(jnp.int32, (L, 2 * L), 1)
        first = scol < L
        kidx = jnp.where(first, scol, scol - L)
        mask = (srow < MEM) | (srow >= kidx)

        def softmax(s):
            s = jnp.where(mask, s * scale, -1e9)
            m1 = jnp.max(jnp.where(first, s, -jnp.inf), axis=1, keepdims=True)
            m2 = jnp.max(jnp.where(first, -jnp.inf, s), axis=1, keepdims=True)
            e = jnp.exp(s - jnp.where(first, m1, m2))
            l1 = jnp.sum(jnp.where(first, e, 0.0), axis=1, keepdims=True)
            l2 = jnp.sum(jnp.where(first, 0.0, e), axis=1, keepdims=True)
            return e * jnp.where(first, 1.0 / l1, 1.0 / l2)

        def oproj(os_, p0, p1):
            o = jnp.concatenate([os_[p] for p in range(p0, p1)], axis=1)
            return jnp.dot(o, wob_ref[p0 * PW:p1 * PW, :], preferred_element_type=f32)

        def step(s, mem):
            r = rows(s, SEG)
            h = jnp.concatenate([mem, xnb_ref[r, :]], axis=0)
            qkv, pr, os_ = {}, {}, {}
            acc = jnp.concatenate([jnp.zeros((MEM, D), f32), xres_ref[r, :]], axis=0)
            for t in range(NP + 2):
                if t < NP:
                    w = pltpu.bitcast(wb_ref[t], bf16)
                    if t == 0:
                        ks = D - 128
                        part = jnp.dot(h[:, :ks], w[:ks], preferred_element_type=f32)
                        part = jnp.concatenate([part[:, :128], part[:, 128:]], axis=1)
                        qkv[t] = part + jnp.dot(h[:, ks:], w[ks:], preferred_element_type=f32)
                    else:
                        qkv[t] = jnp.dot(h, w, preferred_element_type=f32)
                if t == NP:
                    acc = acc + oproj(os_, 0, 3)
                if t == NP + 1:
                    acc = acc + oproj(os_, 3, 7)
                if 0 <= t - 1 < NP:
                    q, k = qkv[t - 1][:, :PW], qkv[t - 1][:, PW:2 * PW]
                    pr[t - 1] = softmax(
                        lax.dot_general(q, _blockdiag(k), _NT, preferred_element_type=f32))
                if 0 <= t - 2 < NP:
                    os_[t - 2] = jnp.dot(pr[t - 2], _blockdiag(qkv[t - 2][:, 2 * PW:]),
                                         preferred_element_type=f32)
            acc = acc + oproj(os_, 7, NP)
            xnew = acc[MEM:]
            xres_ref[r, :] = xnew
            obuf_ref[r, :] = xnew.astype(bf16)
            return acc[:MEM]

        def steps(i, carry):
            mem = mem_ref[...]
            for u in range(UNROLL):
                mem = step(i * UNROLL + u, mem)
            mem_ref[...] = mem

            @pl.when(layer == 1)
            def _():
                out_copy(i).start()
            return carry

        lax.fori_loop(0, NSEG // UNROLL, steps, 0)

    layer_a(True)

    def layer(i, carry):
        layer_b(i)

        @pl.when(i == 0)
        def _():
            layer_a(False)
        return carry

    lax.fori_loop(0, 2, layer, 0)
    for i in range(NSEG // UNROLL):
        out_copy(i).wait()


@functools.partial(jax.jit, static_argnames=("B_seg_len",))
def pallas_interleave_layers__linear_kernel_hedgehog__memory_aug_recurrent_mem_tr__prompt_kernel(
    A_x, A_wqkv, A_w_phi, A_wo, B_x, B_mem0, B_Wq, B_Wk, B_Wv, B_Wo, B_seg_len=SEG,
):
    del B_x
    assert B_seg_len == SEG
    x = A_x.reshape(S, D)
    wp = A_w_phi.transpose(2, 0, 1).reshape(DA, D)
    mem0 = B_mem0.reshape(MEM, D)
    wqt, wkt, wvt = (w.transpose(1, 2, 0).reshape(HB * DB, D) for w in (B_Wq, B_Wk, B_Wv))
    wob = B_Wo.reshape(HB * DB, D)

    vmem = pl.BlockSpec(memory_space=pltpu.VMEM)
    hbm = pl.BlockSpec(memory_space=pl.ANY)
    out = pl.pallas_call(
        _kernel,
        out_shape=jax.ShapeDtypeStruct((S, D), bf16),
        in_specs=[hbm, hbm, vmem, hbm, vmem, hbm, hbm, hbm, hbm],
        out_specs=hbm,
        scratch_shapes=[
            pltpu.VMEM((S, D), bf16),
            pltpu.VMEM((D, 3 * D), bf16),
            pltpu.VMEM((D, D), bf16),
            pltpu.VMEM((S, D), f32),
            pltpu.VMEM((S, D), f32),
            pltpu.VMEM((S // 2, D), u32),
            pltpu.VMEM((3 * NG, GR // 2, D), u32),
            pltpu.VMEM((D // 2, D), u32),
            pltpu.VMEM((NG, GR + 8, 2 * GR), f32),
            pltpu.VMEM((D // 2, TB), u32),
            pltpu.VMEM((3, HB * DB, D), bf16),
            pltpu.VMEM((HB * DB, D), bf16),
            pltpu.VMEM((NP, D // 2, 3 * PW), u32),
            pltpu.VMEM((MEM, D), f32),
            pltpu.VMEM((S, D), bf16),
            pltpu.SemaphoreType.DMA((6,)),
            pltpu.SemaphoreType.DMA((3 * NB,)),
            pltpu.SemaphoreType.DMA,
        ],
        compiler_params=pltpu.CompilerParams(vmem_limit_bytes=110 * 1024 * 1024),
    )(x, A_wqkv, wp, A_wo, mem0, wqt, wkt, wvt, wob)
    return out.reshape(1, S, D)
```

```python
import functools

import jax
import jax.numpy as jnp
from jax import lax
import jax.experimental.pallas as pl
import jax.experimental.pallas.tpu as pltpu

f32 = jnp.float32
bf16 = jnp.bfloat16
u32 = jnp.uint32

S = 2048
D = 640
HA = 32
DA = D // HA
HB = 32
DB = 192
MEM = 8
SEG = 32
L = MEM + SEG
NSEG = S // SEG
NP = HB // 2
PW = 2 * DB
NG = 4
PR = 2 * DA
GR = D // NG
TB = 256
NB = S // TB
LN_EPS = 1e-5
UNROLL = 2

_NT = (((1,), (1,)), ((), ()))


def _layernorm(x):
    m = jnp.mean(x, axis=-1, keepdims=True)
    xc = x - m
    v = jnp.mean(xc * xc, axis=-1, keepdims=True)
    return xc * lax.rsqrt(v + LN_EPS)


def _fold(op, rows):
    r = functools.reduce(op, rows)
    r = op(r, pltpu.roll(r, 4, 0))
    return op(r, pltpu.roll(r, 2, 0))


def _hedgehog(p):
    rows = [p[8 * i:8 * (i + 1), :] for i in range(PR // 8)]
    mx = _fold(jnp.maximum, rows)
    mn = _fold(jnp.minimum, rows)
    ep = [jnp.exp(r - mx) for r in rows]
    en = [jnp.exp(mn - r) for r in rows]
    rp = 1.0 / _fold(jnp.add, ep)
    rn = 1.0 / _fold(jnp.add, en)
    return jnp.concatenate([e * rp for e in ep] + [e * rn for e in en], axis=0)


def _blockdiag(x):
    t0, t1, t2 = x[:, :128], x[:, 128:256], x[:, 256:]
    lane = lax.broadcasted_iota(jnp.int32, (L, 128), 1)
    z = jnp.zeros((L, 128), f32)
    top = jnp.concatenate([t0, jnp.where(lane < 64, t1, 0.0), z], axis=1)
    bot = jnp.concatenate([z, jnp.where(lane >= 64, t1, 0.0), t2], axis=1)
    return jnp.concatenate([top, bot], axis=0)


def _kernel(x_hbm, wqkv_hbm, wphi_ref, wo_hbm, mem0_ref, wqt_hbm, wkt_hbm, wvt_hbm, wob_hbm,
            out_hbm,
            x_ref, wqkv_ref, wo_ref, xres_ref, xnb_ref, xna_ref, wt_ref, wp2_ref, kvt_ref, ot_ref,
            stage_ref, wob_ref, wb_ref, mem_ref, obuf_ref, sem_a, sem_b, sem_o):
    scale = DB ** -0.5
    HS = S // 2
    CH = HB * DB // NB

    cp_kv = pltpu.make_async_copy(wqkv_hbm.at[:, D:], wqkv_ref.at[:, D:], sem_a.at[0])
    cp_x0 = pltpu.make_async_copy(x_hbm.at[:HS], x_ref.at[:HS], sem_a.at[1])
    cp_x1 = pltpu.make_async_copy(x_hbm.at[HS:], x_ref.at[HS:], sem_a.at[2])
    cp_q = pltpu.make_async_copy(wqkv_hbm.at[:, :D], wqkv_ref.at[:, :D], sem_a.at[3])
    cp_wo = pltpu.make_async_copy(wo_hbm, wo_ref, sem_a.at[4])
    cp_wob = pltpu.make_async_copy(wob_hbm, wob_ref, sem_a.at[5])

    def cp_b(m, c):
        src = (wqt_hbm, wkt_hbm, wvt_hbm)[m]
        r0 = c * CH if isinstance(c, int) else pl.multiple_of(c * CH, CH)
        return pltpu.make_async_copy(src.at[pl.ds(r0, CH)], stage_ref.at[m, pl.ds(r0, CH)],
                                     sem_b.at[m * NB + c])

    cp_kv.start()
    cp_x0.start()

    hrow = lax.broadcasted_iota(jnp.int32, (HA, D), 0)
    hcol = lax.broadcasted_iota(jnp.int32, (HA, D), 1)
    wp = None
    for d in range(DA):
        sel = jnp.where(hcol == hrow * DA + d, 1.0, 0.0)
        t = jnp.dot(wphi_ref[d].astype(f32), sel, preferred_element_type=f32)
        wp = t if wp is None else wp + t
    dup = jnp.where((lax.broadcasted_iota(jnp.int32, (PR, DA), 0) >> 1)
                    == lax.broadcasted_iota(jnp.int32, (PR, DA), 1), 1.0, 0.0)
    wp2_ref[...] = jnp.dot(dup, wp, preferred_element_type=f32)

    def fold_phi(m):
        row = lax.broadcasted_iota(jnp.int32, (PR, 128), 0)
        col = lax.broadcasted_iota(jnp.int32, (PR, 128), 1)
        parts = []
        for t in range(D // 128):
            blocks = []
            for j in range(3 * t, 3 * t + 4):
                lo = (2 * j + (row & 1)) * DA - 128 * t
                blocks.append(jnp.where((col >= lo) & (col < lo + DA),
                                        wp2_ref[:, 128 * t:128 * (t + 1)], 0.0))
            w = wqkv_ref[:, m * D + 128 * t:m * D + 128 * (t + 1)]
            parts.append(lax.dot_general(jnp.concatenate(blocks, axis=0).astype(bf16), w, _NT,
                                         preferred_element_type=f32))
        out = [parts[0][:PR]]
        for t in range(D // 128):
            out.append(parts[t][PR:3 * PR])
            last = parts[t][3 * PR:]
            out.append(last + parts[t + 1][:PR] if t + 1 < D // 128 else last)
        wt_ref[m] = pltpu.bitcast(jnp.concatenate(out, axis=0).astype(bf16), u32)

    def wt(m, g):
        return pltpu.bitcast(wt_ref[m, g * GR // 2:(g + 1) * GR // 2, :], bf16)

    def rows(b, n=TB):
        return pl.ds(b * n if isinstance(b, int) else pl.multiple_of(b * n, n), n)

    def layer_a(first):
        src_ref = x_ref if first else xres_ref

        def ln_a(b):
            xn = _layernorm(src_ref[rows(b), :].astype(f32)).astype(bf16)
            xna_ref[rows(b, TB // 2), :] = pltpu.bitcast(xn, u32)

        def load_xn(b):
            return pltpu.bitcast(xna_ref[rows(b, TB // 2), :], bf16)

        if first:
            cp_kv.wait()
            for c in (cp_x1, cp_q, cp_wo):
                c.start()
            fold_phi(1)
            wt_ref[2] = pltpu.bitcast(wqkv_ref[:, 2 * D:].T, u32)
            cp_x0.wait()
            for c in range(NB):
                for m in range(3):
                    cp_b(m, c).start()
            cp_wob.start()
        kvt_ref[...] = jnp.zeros(kvt_ref.shape, f32)
        ln_a(0)

        def phase1(b, carry):
            if first:
                @pl.when(b == NB // 2 - 1)
                def _():
                    cp_x1.wait()
            xn = load_xn(b)
            ones = jnp.ones((8, TB), f32)
            pk, v1 = {}, {}

            def proj_k(g):
                pk[g] = lax.dot_general(wt(1, g), xn, _NT, preferred_element_type=f32)

            def proj_v(g):
                v1[g] = lax.dot_general(wt(2, g), xn, _NT, preferred_element_type=f32)

            def kv(g):
                for j in range(GR // PR):
                    phik = _hedgehog(pk[g][j * PR:(j + 1) * PR]).astype(bf16)
                    lhs = jnp.concatenate([v1[g][j * PR:(j + 1) * PR], ones], axis=0)
                    kvt_ref[g * (GR // PR) + j] += lax.dot_general(
                        lhs, phik, _NT, preferred_element_type=f32)

            proj_k(0); proj_k(1); proj_v(0); proj_k(2); proj_v(1); kv(0)
            proj_k(3); proj_v(2); kv(1); proj_v(3); kv(2); kv(3)
            ln_a(jnp.minimum(b + 1, NB - 1))
            return carry

        lax.fori_loop(0, NB, phase1, 0)

        if first:
            cp_q.wait()
            cp_wo.wait()
            fold_phi(0)
        rr = lax.broadcasted_iota(jnp.int32, (PR + 8, 2 * PR), 0)
        cc = lax.broadcasted_iota(jnp.int32, (PR + 8, 2 * PR), 1)
        second = ((rr >= DA) & (rr < PR)) | (rr >= PR + 4)
        same_head = second == ((cc & 1) == 1)
        for j in range(HA // 2):
            kvt_ref[j] = jnp.where(same_head, kvt_ref[j], 0.0)

        def phase2(b, do_q, do_o):
            if first and do_q:
                for m in range(3):
                    cp_b(m, b).wait()
            pq = {}
            if do_q:
                xn = load_xn(b)
            if do_o:
                o = pltpu.bitcast(ot_ref[...], bf16).T

            def proj_q(g):
                if do_q:
                    pq[g] = lax.dot_general(wt(0, g), xn, _NT, preferred_element_type=f32)

            def num(g):
                if do_q:
                    top = lax.broadcasted_iota(jnp.int32, (8, TB), 0) < 4
                    ot = []
                    for j in range(GR // PR):
                        phiq = _hedgehog(pq[g][j * PR:(j + 1) * PR]).astype(bf16)
                        n = jnp.dot(kvt_ref[g * (GR // PR) + j], phiq, preferred_element_type=f32)
                        r = 1.0 / (n[PR:, :] + 1e-6)
                        rs = pltpu.roll(r, 4, 0)
                        ra, rb = jnp.where(top, r, rs), jnp.where(top, rs, r)
                        ot += [n[8 * i:8 * (i + 1), :] * rr_
                               for i, rr_ in enumerate((ra, ra, r, rb, rb))]
                    ot = jnp.concatenate(ot, axis=0)
                    ot_ref[g * GR // 2:(g + 1) * GR // 2, :] = pltpu.bitcast(ot.astype(bf16), u32)

            def out(j):
                if do_o:
                    hb = TB // 2
                    r = rows(2 * (b - 1) + j, hb)
                    xb = src_ref[r, :].astype(f32) + jnp.dot(
                        o[j * hb:(j + 1) * hb], wo_ref[...], preferred_element_type=f32)
                    xres_ref[r, :] = xb
                    xnb_ref[r, :] = _layernorm(xb)

            proj_q(0); proj_q(1); out(0); num(0); proj_q(2); num(1); proj_q(3); out(1)
            num(2); num(3)

            if first and do_q:
                for j in range(CH // PW):
                    p = b * (CH // PW) + j
                    for m in range(3):
                        blk = stage_ref[m, rows(p, PW), :]
                        wb_ref[p, :, m * PW:(m + 1) * PW] = pltpu.bitcast(blk.T, u32)

        phase2(0, True, False)

        def body2(b, carry):
            phase2(b, True, True)
            return carry

        lax.fori_loop(1, NB, body2, 0)
        phase2(NB, False, True)
        if first:
            cp_wob.wait()

    def out_copy(i):
        r = rows(i, UNROLL * SEG)
        return pltpu.make_async_copy(obuf_ref.at[r], out_hbm.at[r], sem_o)

    def layer_b(layer):
        mem_ref[...] = mem0_ref[...].astype(f32)
        srow = lax.broadcasted_iota(jnp.int32, (L, 2 * L), 0)
        scol = lax.broadcasted_iota(jnp.int32, (L, 2 * L), 1)
        first = scol < L
        kidx = jnp.where(first, scol, scol - L)
        mask = (srow < MEM) | (srow >= kidx)

        def softmax(s):
            s = jnp.where(mask, s * scale, -1e9)
            m1 = jnp.max(jnp.where(first, s, -jnp.inf), axis=1, keepdims=True)
            m2 = jnp.max(jnp.where(first, -jnp.inf, s), axis=1, keepdims=True)
            e = jnp.exp(s - jnp.where(first, m1, m2))
            l1 = jnp.sum(jnp.where(first, e, 0.0), axis=1, keepdims=True)
            l2 = jnp.sum(jnp.where(first, 0.0, e), axis=1, keepdims=True)
            return e * jnp.where(first, 1.0 / l1, 1.0 / l2)

        def oproj(os_, p0, p1):
            o = jnp.concatenate([os_[p] for p in range(p0, p1)], axis=1)
            return jnp.dot(o, wob_ref[p0 * PW:p1 * PW, :], preferred_element_type=f32)

        def step(s, mem):
            r = rows(s, SEG)
            h = jnp.concatenate([mem, xnb_ref[r, :]], axis=0)
            qkv, pr, os_ = {}, {}, {}
            acc = jnp.concatenate([jnp.zeros((MEM, D), f32), xres_ref[r, :]], axis=0)
            for t in range(NP + 2):
                if t < NP:
                    w = pltpu.bitcast(wb_ref[t], bf16)
                    if t == 0:
                        ks = D - 128
                        part = jnp.dot(h[:, :ks], w[:ks], preferred_element_type=f32)
                        part = jnp.concatenate([part[:, :128], part[:, 128:]], axis=1)
                        qkv[t] = part + jnp.dot(h[:, ks:], w[ks:], preferred_element_type=f32)
                    else:
                        qkv[t] = jnp.dot(h, w, preferred_element_type=f32)
                if t == NP:
                    acc = acc + oproj(os_, 0, 3)
                if t == NP + 1:
                    acc = acc + oproj(os_, 3, 7)
                if 0 <= t - 1 < NP:
                    q, k = qkv[t - 1][:, :PW], qkv[t - 1][:, PW:2 * PW]
                    pr[t - 1] = softmax(
                        lax.dot_general(q, _blockdiag(k), _NT, preferred_element_type=f32))
                if 0 <= t - 2 < NP:
                    os_[t - 2] = jnp.dot(pr[t - 2], _blockdiag(qkv[t - 2][:, 2 * PW:]),
                                         preferred_element_type=f32)
            acc = acc + oproj(os_, 7, NP)
            xnew = acc[MEM:]
            xres_ref[r, :] = xnew
            obuf_ref[r, :] = xnew.astype(bf16)
            return acc[:MEM]

        def steps(i, carry):
            mem = mem_ref[...]
            for u in range(UNROLL):
                mem = step(i * UNROLL + u, mem)
            mem_ref[...] = mem

            @pl.when(layer == 1)
            def _():
                out_copy(i).start()
            return carry

        lax.fori_loop(0, NSEG // UNROLL, steps, 0)

    layer_a(True)

    def layer(i, carry):
        layer_b(i)

        @pl.when(i == 0)
        def _():
            layer_a(False)
        return carry

    lax.fori_loop(0, 2, layer, 0)
    for i in range(NSEG // UNROLL):
        out_copy(i).wait()


@functools.partial(jax.jit, static_argnames=("B_seg_len",))
def pallas_interleave_layers__linear_kernel_hedgehog__memory_aug_recurrent_mem_tr__prompt_kernel(
    A_x, A_wqkv, A_w_phi, A_wo, B_x, B_mem0, B_Wq, B_Wk, B_Wv, B_Wo, B_seg_len=SEG,
):
    del B_x
    assert B_seg_len == SEG
    x = A_x.reshape(S, D)
    wp = A_w_phi.transpose(1, 2, 0)
    mem0 = B_mem0.reshape(MEM, D)
    wqt, wkt, wvt = (w.transpose(1, 2, 0).reshape(HB * DB, D) for w in (B_Wq, B_Wk, B_Wv))
    wob = B_Wo.reshape(HB * DB, D)

    vmem = pl.BlockSpec(memory_space=pltpu.VMEM)
    hbm = pl.BlockSpec(memory_space=pl.ANY)
    out = pl.pallas_call(
        _kernel,
        out_shape=jax.ShapeDtypeStruct((S, D), bf16),
        in_specs=[hbm, hbm, vmem, hbm, vmem, hbm, hbm, hbm, hbm],
        out_specs=hbm,
        scratch_shapes=[
            pltpu.VMEM((S, D), bf16),
            pltpu.VMEM((D, 3 * D), bf16),
            pltpu.VMEM((D, D), bf16),
            pltpu.VMEM((S, D), f32),
            pltpu.VMEM((S, D), f32),
            pltpu.VMEM((S // 2, D), u32),
            pltpu.VMEM((3, D // 2, D), u32),
            pltpu.VMEM((PR, D), f32),
            pltpu.VMEM((HA // 2, PR + 8, 2 * PR), f32),
            pltpu.VMEM((D // 2, TB), u32),
            pltpu.VMEM((3, HB * DB, D), bf16),
            pltpu.VMEM((HB * DB, D), bf16),
            pltpu.VMEM((NP, D // 2, 3 * PW), u32),
            pltpu.VMEM((MEM, D), f32),
            pltpu.VMEM((S, D), bf16),
            pltpu.SemaphoreType.DMA((6,)),
            pltpu.SemaphoreType.DMA((3 * NB,)),
            pltpu.SemaphoreType.DMA,
        ],
        compiler_params=pltpu.CompilerParams(vmem_limit_bytes=110 * 1024 * 1024),
    )(x, A_wqkv, wp, A_wo, mem0, wqt, wkt, wvt, wob)
    return out.reshape(1, S, D)
```

```python
import functools

import jax
import jax.numpy as jnp
from jax import lax
import jax.experimental.pallas as pl
import jax.experimental.pallas.tpu as pltpu

f32 = jnp.float32
bf16 = jnp.bfloat16
u32 = jnp.uint32

S = 2048
D = 640
HA = 32
DA = D // HA
HB = 32
DB = 192
MEM = 8
SEG = 32
L = MEM + SEG
NSEG = S // SEG
NP = HB // 2
PW = 2 * DB
NG = 4
PR = 2 * DA
GR = D // NG
TB = 256
NB = S // TB
LN_EPS = 1e-5
UNROLL = 4

_NT = (((1,), (1,)), ((), ()))


def _layernorm(x):
    m = jnp.mean(x, axis=-1, keepdims=True)
    xc = x - m
    v = jnp.mean(xc * xc, axis=-1, keepdims=True)
    return xc * lax.rsqrt(v + LN_EPS)


def _fold(op, rows):
    r = functools.reduce(op, rows)
    r = op(r, pltpu.roll(r, 4, 0))
    return op(r, pltpu.roll(r, 2, 0))


def _hedgehog(p):
    rows = [p[8 * i:8 * (i + 1), :] for i in range(PR // 8)]
    mx = _fold(jnp.maximum, rows)
    mn = _fold(jnp.minimum, rows)
    ep = [jnp.exp(r - mx) for r in rows]
    en = [jnp.exp(mn - r) for r in rows]
    rp = 1.0 / _fold(jnp.add, ep)
    rn = 1.0 / _fold(jnp.add, en)
    return jnp.concatenate([e * rp for e in ep] + [e * rn for e in en], axis=0)


def _blockdiag(x):
    t0, t1, t2 = x[:, :128], x[:, 128:256], x[:, 256:]
    lane = lax.broadcasted_iota(jnp.int32, (L, 128), 1)
    z = jnp.zeros((L, 128), f32)
    top = jnp.concatenate([t0, jnp.where(lane < 64, t1, 0.0), z], axis=1)
    bot = jnp.concatenate([z, jnp.where(lane >= 64, t1, 0.0), t2], axis=1)
    return jnp.concatenate([top, bot], axis=0)


def _kernel(x_hbm, wqkv_hbm, wphi_ref, wo_hbm, mem0_ref, wqt_hbm, wkt_hbm, wvt_hbm, wob_hbm,
            out_hbm,
            x_ref, wqkv_ref, wo_ref, xres_ref, xnb_ref, xna_ref, wt_ref, wp2_ref, kvt_ref,
            stage_ref, wob_ref, wb_ref, mem_ref, obuf_ref, sem_a, sem_b, sem_o):
    scale = DB ** -0.5
    XH = 2 * TB
    HT = TB // 2
    CH = HB * DB // NB

    cp_x0 = pltpu.make_async_copy(x_hbm.at[:XH], x_ref.at[:XH], sem_a.at[0])
    cp_kv = pltpu.make_async_copy(wqkv_hbm.at[:, D:], wqkv_ref.at[:, D:], sem_a.at[1])
    cp_x1 = pltpu.make_async_copy(x_hbm.at[XH:], x_ref.at[XH:], sem_a.at[2])
    cp_q = pltpu.make_async_copy(wqkv_hbm.at[:, :D], wqkv_ref.at[:, :D], sem_a.at[3])
    cp_wo = pltpu.make_async_copy(wo_hbm, wo_ref, sem_a.at[4])
    cp_wob = pltpu.make_async_copy(wob_hbm, wob_ref, sem_a.at[5])

    def rows(b, n=TB):
        return pl.ds(b * n if isinstance(b, int) else pl.multiple_of(b * n, n), n)

    def cp_b(m, c):
        src = (wqt_hbm, wkt_hbm, wvt_hbm)[m]
        return pltpu.make_async_copy(src.at[rows(c, CH)], stage_ref.at[m, rows(c, CH)],
                                     sem_b.at[m * NB + c])

    cp_x0.start()
    cp_kv.start()
    for m in range(3):
        cp_b(m, 0).start(priority=1)

    hrow = lax.broadcasted_iota(jnp.int32, (HA, D), 0)
    hcol = lax.broadcasted_iota(jnp.int32, (HA, D), 1)
    wp = None
    for d in range(DA):
        sel = jnp.where(hcol == hrow * DA + d, 1.0, 0.0)
        t = jnp.dot(wphi_ref[d].astype(f32), sel, preferred_element_type=f32)
        wp = t if wp is None else wp + t
    dup = jnp.where((lax.broadcasted_iota(jnp.int32, (PR, DA), 0) >> 1)
                    == lax.broadcasted_iota(jnp.int32, (PR, DA), 1), 1.0, 0.0)
    wp2_ref[...] = jnp.dot(dup, wp, preferred_element_type=f32)

    def fold_phi(m):
        row = lax.broadcasted_iota(jnp.int32, (PR, 128), 0)
        col = lax.broadcasted_iota(jnp.int32, (PR, 128), 1)
        parts = []
        for t in range(D // 128):
            blocks = []
            for j in range(3 * t, 3 * t + 4):
                lo = (2 * j + (row & 1)) * DA - 128 * t
                blocks.append(jnp.where((col >= lo) & (col < lo + DA),
                                        wp2_ref[:, 128 * t:128 * (t + 1)], 0.0))
            w = wqkv_ref[:, m * D + 128 * t:m * D + 128 * (t + 1)]
            parts.append(lax.dot_general(jnp.concatenate(blocks, axis=0).astype(bf16), w, _NT,
                                         preferred_element_type=f32))
        out = [parts[0][:PR]]
        for t in range(D // 128):
            out.append(parts[t][PR:3 * PR])
            last = parts[t][3 * PR:]
            out.append(last + parts[t + 1][:PR] if t + 1 < D // 128 else last)
        wt_ref[m] = pltpu.bitcast(jnp.concatenate(out, axis=0).astype(bf16), u32)

    def wt(m, g):
        return pltpu.bitcast(wt_ref[m, g * GR // 2:(g + 1) * GR // 2, :], bf16)

    def layer_a(first):
        src_ref = x_ref if first else xres_ref

        def ln_a(b):
            xn = _layernorm(src_ref[rows(b), :].astype(f32)).astype(bf16)
            xna_ref[rows(b, HT), :] = pltpu.bitcast(xn, u32)

        kvt_ref[...] = jnp.zeros(kvt_ref.shape, f32)
        if first:
            cp_x0.wait()
        ln_a(0)
        if first:
            cp_kv.wait()
            cp_x1.start()
            fold_phi(1)
            wt_ref[2] = pltpu.bitcast(wqkv_ref[:, 2 * D:].T, u32)

        def phase1(b, carry):
            if first:
                @pl.when(b == XH // TB - 1)
                def _():
                    cp_x1.wait()
                    cp_q.start()
                    cp_wo.start()

                @pl.when(b < NB - 1)
                def _():
                    for m in range(3):
                        cp_b(m, b + 1).start(priority=1)
            xn = pltpu.bitcast(xna_ref[rows(b, HT), :], bf16)
            ones = jnp.ones((8, TB), f32)
            pk, v1 = {}, {}

            def proj_k(g):
                pk[g] = lax.dot_general(wt(1, g), xn, _NT, preferred_element_type=f32)

            def proj_v(g):
                v1[g] = lax.dot_general(wt(2, g), xn, _NT, preferred_element_type=f32)

            def kv(g):
                for j in range(GR // PR):
                    phik = _hedgehog(pk[g][j * PR:(j + 1) * PR]).astype(bf16)
                    lhs = jnp.concatenate([v1[g][j * PR:(j + 1) * PR], ones], axis=0)
                    kvt_ref[g * (GR // PR) + j] += lax.dot_general(
                        lhs, phik, _NT, preferred_element_type=f32)

            ln_a(jnp.minimum(b + 1, NB - 1))
            proj_k(0); proj_k(1); proj_v(0); proj_k(2); proj_v(1); kv(0)
            proj_k(3); proj_v(2); proj_v(3); kv(1); kv(2); kv(3)
            return carry

        lax.fori_loop(0, NB, phase1, 0)

        if first:
            cp_q.wait()
            cp_wo.wait()
            fold_phi(0)
        rr = lax.broadcasted_iota(jnp.int32, (PR + 8, 2 * PR), 0)
        cc = lax.broadcasted_iota(jnp.int32, (PR + 8, 2 * PR), 1)
        second = ((rr >= DA) & (rr < PR)) | (rr >= PR + 4)
        same_head = second == ((cc & 1) == 1)
        for j in range(HA // 2):
            kvt_ref[j] = jnp.where(same_head, kvt_ref[j], 0.0)

        def ln_b(i):
            xnb_ref[rows(i, HT), :] = _layernorm(xres_ref[rows(i, HT), :])

        def phase2(b, carry):
            if first:
                for m in range(3):
                    cp_b(m, b).wait()

                @pl.when(b == 2)
                def _():
                    cp_wob.start(priority=1)
            ln_b(jnp.maximum(2 * b - 1, 0))
            top = lax.broadcasted_iota(jnp.int32, (8, HT), 0) < 4
            xn = [pltpu.bitcast(xna_ref[rows(2 * b + i, HT // 2), :], bf16) for i in range(2)]
            pq, ot, o, y = {}, {}, {}, {}

            def proj_q(i, g):
                pq[i, g] = lax.dot_general(wt(0, g), xn[i], _NT, preferred_element_type=f32)

            def num(i, g):
                parts = []
                for j in range(GR // PR):
                    phiq = _hedgehog(pq[i, g][j * PR:(j + 1) * PR]).astype(bf16)
                    n = jnp.dot(kvt_ref[g * (GR // PR) + j], phiq, preferred_element_type=f32)
                    r = 1.0 / (n[PR:, :] + 1e-6)
                    rs = pltpu.roll(r, 4, 0)
                    ra, rb = jnp.where(top, r, rs), jnp.where(top, rs, r)
                    parts += [n[8 * t:8 * (t + 1), :] * rr_
                              for t, rr_ in enumerate((ra, ra, r, rb, rb))]
                ot[i, g] = jnp.concatenate(parts, axis=0).astype(bf16)

            def out(i, k0, k1, c0=0, c1=D):
                if i not in o:
                    o[i] = {}
                    y[i] = {}
                full = jnp.concatenate([ot[i, g] for g in range(NG) if (i, g) in ot], axis=0)
                for t in range(k0 // 128, k1 // 128):
                    if t not in o[i]:
                        o[i][t] = full[128 * t:128 * (t + 1)].T
                lhs = jnp.concatenate([o[i][t] for t in range(k0 // 128, k1 // 128)], axis=1)
                if (c0, c1) not in y[i]:
                    y[i][c0, c1] = src_ref[rows(2 * b + i, HT), c0:c1].astype(f32)
                y[i][c0, c1] = y[i][c0, c1] + jnp.dot(lhs, wo_ref[k0:k1, c0:c1],
                                                      preferred_element_type=f32)

            proj_q(0, 0); proj_q(0, 1); proj_q(0, 2); num(0, 0); proj_q(0, 3); num(0, 1)
            proj_q(1, 0); num(0, 2); proj_q(1, 1); num(0, 3); proj_q(1, 2); num(1, 0)
            proj_q(1, 3); num(1, 1)
            out(0, 0, D, 0, 128); num(1, 2); out(0, 0, D, 128, 256); num(1, 3)
            out(0, 0, D, 256, D)
            x0 = jnp.concatenate([y[0][0, 128], y[0][128, 256], y[0][256, D]], axis=1)
            xres_ref[rows(2 * b, HT), :] = x0
            xnb_ref[rows(2 * b, HT), :] = _layernorm(x0)
            out(1, 0, 384); out(1, 384, D)
            xres_ref[rows(2 * b + 1, HT), :] = y[1][0, D]

            if first:
                for j in range(CH // PW):
                    p = b * (CH // PW) + j
                    for m in range(3):
                        blk = stage_ref[m, rows(p, PW), :]
                        wb_ref[p, :, m * PW:(m + 1) * PW] = pltpu.bitcast(blk.T, u32)
            return carry

        lax.fori_loop(0, NB, phase2, 0)
        ln_b(2 * NB - 1)
        if first:
            cp_wob.wait()

    def out_copy(i):
        r = rows(i, UNROLL * SEG)
        return pltpu.make_async_copy(obuf_ref.at[r], out_hbm.at[r], sem_o)

    def layer_b(layer):
        mem_ref[...] = mem0_ref[...].astype(f32)
        srow = lax.broadcasted_iota(jnp.int32, (L, 2 * L), 0)
        scol = lax.broadcasted_iota(jnp.int32, (L, 2 * L), 1)
        first = scol < L
        kidx = jnp.where(first, scol, scol - L)
        mask = (srow < MEM) | (srow >= kidx)

        def softmax(s):
            s = jnp.where(mask, s * scale, -1e9)
            m1 = jnp.max(jnp.where(first, s, -jnp.inf), axis=1, keepdims=True)
            m2 = jnp.max(jnp.where(first, -jnp.inf, s), axis=1, keepdims=True)
            e = jnp.exp(s - jnp.where(first, m1, m2))
            l1 = jnp.sum(jnp.where(first, e, 0.0), axis=1, keepdims=True)
            l2 = jnp.sum(jnp.where(first, 0.0, e), axis=1, keepdims=True)
            return e * jnp.where(first, 1.0 / l1, 1.0 / l2)

        def oproj(os_, p0, p1):
            o = jnp.concatenate([os_[p] for p in range(p0, p1)], axis=1)
            return jnp.dot(o, wob_ref[p0 * PW:p1 * PW, :], preferred_element_type=f32)

        def step(s, mem):
            r = rows(s, SEG)
            h = jnp.concatenate([mem, xnb_ref[r, :]], axis=0)
            qkv, pr, os_ = {}, {}, {}
            acc = jnp.concatenate([jnp.zeros((MEM, D), f32), xres_ref[r, :]], axis=0)
            for t in range(NP + 2):
                if t < NP:
                    w = pltpu.bitcast(wb_ref[t], bf16)
                    if t == 0:
                        ks = D - 128
                        part = jnp.dot(h[:, :ks], w[:ks], preferred_element_type=f32)
                        part = jnp.concatenate([part[:, :128], part[:, 128:]], axis=1)
                        qkv[t] = part + jnp.dot(h[:, ks:], w[ks:], preferred_element_type=f32)
                    else:
                        qkv[t] = jnp.dot(h, w, preferred_element_type=f32)
                if t == NP:
                    acc = acc + oproj(os_, 0, 3)
                if t == NP + 1:
                    acc = acc + oproj(os_, 3, 7)
                if 0 <= t - 1 < NP:
                    q, k = qkv[t - 1][:, :PW], qkv[t - 1][:, PW:2 * PW]
                    pr[t - 1] = softmax(
                        lax.dot_general(q, _blockdiag(k), _NT, preferred_element_type=f32))
                if 0 <= t - 2 < NP:
                    os_[t - 2] = jnp.dot(pr[t - 2], _blockdiag(qkv[t - 2][:, 2 * PW:]),
                                         preferred_element_type=f32)
            acc = acc + oproj(os_, 7, NP)
            xnew = acc[MEM:]
            xres_ref[r, :] = xnew
            obuf_ref[r, :] = xnew.astype(bf16)
            return acc[:MEM]

        def steps(i, carry):
            mem = mem_ref[...]
            for u in range(UNROLL):
                mem = step(i * UNROLL + u, mem)
            mem_ref[...] = mem

            @pl.when(layer == 1)
            def _():
                out_copy(i).start()
            return carry

        lax.fori_loop(0, NSEG // UNROLL, steps, 0)

    layer_a(True)

    def layer(i, carry):
        layer_b(i)

        @pl.when(i == 0)
        def _():
            layer_a(False)
        return carry

    lax.fori_loop(0, 2, layer, 0)
    for i in range(NSEG // UNROLL):
        out_copy(i).wait()


@functools.partial(jax.jit, static_argnames=("B_seg_len",))
def pallas_interleave_layers__linear_kernel_hedgehog__memory_aug_recurrent_mem_tr__prompt_kernel(
    A_x, A_wqkv, A_w_phi, A_wo, B_x, B_mem0, B_Wq, B_Wk, B_Wv, B_Wo, B_seg_len=SEG,
):
    del B_x
    assert B_seg_len == SEG
    x = A_x.reshape(S, D)
    wp = A_w_phi.transpose(1, 2, 0)
    mem0 = B_mem0.reshape(MEM, D)
    wqt, wkt, wvt = (w.transpose(1, 2, 0).reshape(HB * DB, D) for w in (B_Wq, B_Wk, B_Wv))
    wob = B_Wo.reshape(HB * DB, D)

    vmem = pl.BlockSpec(memory_space=pltpu.VMEM)
    hbm = pl.BlockSpec(memory_space=pl.ANY)
    out = pl.pallas_call(
        _kernel,
        out_shape=jax.ShapeDtypeStruct((S, D), bf16),
        in_specs=[hbm, hbm, vmem, hbm, vmem, hbm, hbm, hbm, hbm],
        out_specs=hbm,
        scratch_shapes=[
            pltpu.VMEM((S, D), bf16),
            pltpu.VMEM((D, 3 * D), bf16),
            pltpu.VMEM((D, D), bf16),
            pltpu.VMEM((S, D), f32),
            pltpu.VMEM((S, D), f32),
            pltpu.VMEM((S // 2, D), u32),
            pltpu.VMEM((3, D // 2, D), u32),
            pltpu.VMEM((PR, D), f32),
            pltpu.VMEM((HA // 2, PR + 8, 2 * PR), f32),
            pltpu.VMEM((3, HB * DB, D), bf16),
            pltpu.VMEM((HB * DB, D), bf16),
            pltpu.VMEM((NP, D // 2, 3 * PW), u32),
            pltpu.VMEM((MEM, D), f32),
            pltpu.VMEM((S, D), bf16),
            pltpu.SemaphoreType.DMA((6,)),
            pltpu.SemaphoreType.DMA((3 * NB,)),
            pltpu.SemaphoreType.DMA,
        ],
        compiler_params=pltpu.CompilerParams(vmem_limit_bytes=110 * 1024 * 1024),
    )(x, A_wqkv, wp, A_wo, mem0, wqt, wkt, wvt, wob)
    return out.reshape(1, S, D)
```

```python
import functools

import jax
import jax.numpy as jnp
from jax import lax
import jax.experimental.pallas as pl
import jax.experimental.pallas.tpu as pltpu

f32 = jnp.float32
bf16 = jnp.bfloat16
u32 = jnp.uint32

S = 2048
D = 640
HA = 32
DA = D // HA
HB = 32
DB = 192
MEM = 8
SEG = 32
L = MEM + SEG
NSEG = S // SEG
NP = HB // 2
PW = 2 * DB
NG = 4
PR = 2 * DA
GR = D // NG
TB = 256
NB = S // TB
LN_EPS = 1e-5
UNROLL = 4

_NT = (((1,), (1,)), ((), ()))


def _layernorm(x):
    m = jnp.mean(x, axis=-1, keepdims=True)
    xc = x - m
    v = jnp.mean(xc * xc, axis=-1, keepdims=True)
    return xc * lax.rsqrt(v + LN_EPS)


def _fold(op, rows):
    r = functools.reduce(op, rows)
    r = op(r, pltpu.roll(r, 4, 0))
    return op(r, pltpu.roll(r, 2, 0))


def _hedgehog(p):
    rows = [p[8 * i:8 * (i + 1), :] for i in range(PR // 8)]
    mx = _fold(jnp.maximum, rows)
    mn = _fold(jnp.minimum, rows)
    ep = [jnp.exp(r - mx) for r in rows]
    en = [jnp.exp(mn - r) for r in rows]
    rp = 1.0 / _fold(jnp.add, ep)
    rn = 1.0 / _fold(jnp.add, en)
    return jnp.concatenate([e * rp for e in ep] + [e * rn for e in en], axis=0)


def _blockdiag(x):
    t0, t1, t2 = x[:, :128], x[:, 128:256], x[:, 256:]
    lane = lax.broadcasted_iota(jnp.int32, (L, 128), 1)
    z = jnp.zeros((L, 128), f32)
    top = jnp.concatenate([t0, jnp.where(lane < 64, t1, 0.0), z], axis=1)
    bot = jnp.concatenate([z, jnp.where(lane >= 64, t1, 0.0), t2], axis=1)
    return jnp.concatenate([top, bot], axis=0)


def _kernel(x_hbm, wqkv_hbm, wphi_ref, wo_hbm, mem0_ref, wqt_hbm, wkt_hbm, wvt_hbm, wob_hbm,
            out_hbm,
            x_ref, wqkv_ref, wo_ref, xres_ref, xnb_ref, xna_ref, wt_ref, wp2_ref, kvt_ref,
            stage_ref, wob_ref, wb_ref, mem_ref, obuf_ref, sem_a, sem_b, sem_o):
    scale = DB ** -0.5
    XH = 2 * TB
    HT = TB // 2
    CH = HB * DB // NB

    cp_x0 = pltpu.make_async_copy(x_hbm.at[:XH], x_ref.at[:XH], sem_a.at[0])
    cp_kv = pltpu.make_async_copy(wqkv_hbm.at[:, D:], wqkv_ref.at[:, D:], sem_a.at[1])
    cp_x1 = pltpu.make_async_copy(x_hbm.at[XH:], x_ref.at[XH:], sem_a.at[2])
    cp_q = pltpu.make_async_copy(wqkv_hbm.at[:, :D], wqkv_ref.at[:, :D], sem_a.at[3])
    cp_wo = pltpu.make_async_copy(wo_hbm, wo_ref, sem_a.at[4])
    cp_wob = pltpu.make_async_copy(wob_hbm, wob_ref, sem_a.at[5])

    def rows(b, n=TB):
        return pl.ds(b * n if isinstance(b, int) else pl.multiple_of(b * n, n), n)

    def cp_b(m, c):
        src = (wqt_hbm, wkt_hbm, wvt_hbm)[m]
        return pltpu.make_async_copy(src.at[rows(c, CH)], stage_ref.at[m, rows(c, CH)],
                                     sem_b.at[m * NB + c])

    cp_x0.start()
    cp_kv.start()
    for m in range(3):
        cp_b(m, 0).start(priority=1)

    hrow = lax.broadcasted_iota(jnp.int32, (HA, D), 0)
    hcol = lax.broadcasted_iota(jnp.int32, (HA, D), 1)
    wp = None
    for d in range(DA):
        sel = jnp.where(hcol == hrow * DA + d, 1.0, 0.0)
        t = jnp.dot(wphi_ref[d].astype(f32), sel, preferred_element_type=f32)
        wp = t if wp is None else wp + t
    dup = jnp.where((lax.broadcasted_iota(jnp.int32, (PR, DA), 0) >> 1)
                    == lax.broadcasted_iota(jnp.int32, (PR, DA), 1), 1.0, 0.0)
    wp2_ref[...] = jnp.dot(dup, wp, preferred_element_type=f32)

    def fold_phi(m):
        row = lax.broadcasted_iota(jnp.int32, (PR, 128), 0)
        col = lax.broadcasted_iota(jnp.int32, (PR, 128), 1)
        parts = []
        for t in range(D // 128):
            blocks = []
            for j in range(3 * t, 3 * t + 4):
                lo = (2 * j + (row & 1)) * DA - 128 * t
                blocks.append(jnp.where((col >= lo) & (col < lo + DA),
                                        wp2_ref[:, 128 * t:128 * (t + 1)], 0.0))
            w = wqkv_ref[:, m * D + 128 * t:m * D + 128 * (t + 1)]
            parts.append(lax.dot_general(jnp.concatenate(blocks, axis=0).astype(bf16), w, _NT,
                                         preferred_element_type=f32))
        out = [parts[0][:PR]]
        for t in range(D // 128):
            out.append(parts[t][PR:3 * PR])
            last = parts[t][3 * PR:]
            out.append(last + parts[t + 1][:PR] if t + 1 < D // 128 else last)
        wt_ref[m] = pltpu.bitcast(jnp.concatenate(out, axis=0).astype(bf16), u32)

    def wt(m, g):
        return pltpu.bitcast(wt_ref[m, g * GR // 2:(g + 1) * GR // 2, :], bf16)

    def layer_a(first):
        src_ref = x_ref if first else xres_ref

        def ln_a(b):
            xn = _layernorm(src_ref[rows(b), :].astype(f32)).astype(bf16)
            xna_ref[b] = pltpu.bitcast(xn.T, u32)

        kvt_ref[...] = jnp.zeros(kvt_ref.shape, f32)
        if first:
            cp_x0.wait()
        ln_a(0)
        if first:
            cp_kv.wait()
            cp_x1.start()
            fold_phi(1)
            wt_ref[2] = pltpu.bitcast(wqkv_ref[:, 2 * D:].T, u32)

        def phase1(b, carry):
            if first:
                @pl.when(b == XH // TB - 1)
                def _():
                    cp_x1.wait()
                    cp_q.start()
                    cp_wo.start()

                @pl.when(b < NB - 1)
                def _():
                    for m in range(3):
                        cp_b(m, b + 1).start(priority=1)
            xn = pltpu.bitcast(xna_ref[b], bf16)
            ones = jnp.ones((8, TB), f32)
            pk, v1 = {}, {}

            def proj_k(g):
                pk[g] = jnp.dot(wt(1, g), xn, preferred_element_type=f32)

            def proj_v(g):
                v1[g] = jnp.dot(wt(2, g), xn, preferred_element_type=f32)

            def kv(g):
                for j in range(GR // PR):
                    phik = _hedgehog(pk[g][j * PR:(j + 1) * PR]).astype(bf16)
                    lhs = jnp.concatenate([v1[g][j * PR:(j + 1) * PR], ones], axis=0)
                    kvt_ref[g * (GR // PR) + j] += lax.dot_general(
                        lhs, phik, _NT, preferred_element_type=f32)

            ln_a(jnp.minimum(b + 1, NB - 1))
            proj_k(0); proj_k(1); proj_v(0); proj_k(2); proj_v(1); kv(0)
            proj_k(3); proj_v(2); proj_v(3); kv(1); kv(2); kv(3)
            return carry

        lax.fori_loop(0, NB, phase1, 0)

        if first:
            cp_q.wait()
            cp_wo.wait()
            fold_phi(0)
        rr = lax.broadcasted_iota(jnp.int32, (PR + 8, 2 * PR), 0)
        cc = lax.broadcasted_iota(jnp.int32, (PR + 8, 2 * PR), 1)
        second = ((rr >= DA) & (rr < PR)) | (rr >= PR + 4)
        same_head = second == ((cc & 1) == 1)
        for j in range(HA // 2):
            kvt_ref[j] = jnp.where(same_head, kvt_ref[j], 0.0)

        def ln_b(i):
            xnb_ref[rows(i, HT), :] = _layernorm(xres_ref[rows(i, HT), :])

        def phase2(b, carry):
            if first:
                for m in range(3):
                    cp_b(m, b).wait()

                @pl.when(b == 2)
                def _():
                    cp_wob.start(priority=1)
            ln_b(jnp.maximum(2 * b - 1, 0))
            top = lax.broadcasted_iota(jnp.int32, (8, HT), 0) < 4
            xn = [pltpu.bitcast(xna_ref[b, :, i * HT:(i + 1) * HT], bf16) for i in range(2)]
            pq, ot, o, y = {}, {}, {}, {}

            def proj_q(i, g):
                pq[i, g] = jnp.dot(wt(0, g), xn[i], preferred_element_type=f32)

            def num(i, g):
                parts = []
                for j in range(GR // PR):
                    phiq = _hedgehog(pq[i, g][j * PR:(j + 1) * PR]).astype(bf16)
                    n = jnp.dot(kvt_ref[g * (GR // PR) + j], phiq, preferred_element_type=f32)
                    r = 1.0 / (n[PR:, :] + 1e-6)
                    rs = pltpu.roll(r, 4, 0)
                    ra, rb = jnp.where(top, r, rs), jnp.where(top, rs, r)
                    parts += [n[8 * t:8 * (t + 1), :] * rr_
                              for t, rr_ in enumerate((ra, ra, r, rb, rb))]
                ot[i, g] = jnp.concatenate(parts, axis=0).astype(bf16)

            def out(i, k0, k1, c0=0, c1=D):
                if i not in o:
                    o[i] = {}
                    y[i] = {}
                full = jnp.concatenate([ot[i, g] for g in range(NG) if (i, g) in ot], axis=0)
                for t in range(k0 // 128, k1 // 128):
                    if t not in o[i]:
                        o[i][t] = full[128 * t:128 * (t + 1)].T
                lhs = jnp.concatenate([o[i][t] for t in range(k0 // 128, k1 // 128)], axis=1)
                if (c0, c1) not in y[i]:
                    y[i][c0, c1] = src_ref[rows(2 * b + i, HT), c0:c1].astype(f32)
                y[i][c0, c1] = y[i][c0, c1] + jnp.dot(lhs, wo_ref[k0:k1, c0:c1],
                                                      preferred_element_type=f32)

            proj_q(0, 0); proj_q(0, 1); proj_q(0, 2); num(0, 0); proj_q(0, 3); num(0, 1)
            proj_q(1, 0); num(0, 2); proj_q(1, 1); num(0, 3); proj_q(1, 2); num(1, 0)
            proj_q(1, 3); num(1, 1)
            out(0, 0, D, 0, 128); num(1, 2); out(0, 0, D, 128, 256); num(1, 3)
            out(0, 0, D, 256, D)
            x0 = jnp.concatenate([y[0][0, 128], y[0][128, 256], y[0][256, D]], axis=1)
            xres_ref[rows(2 * b, HT), :] = x0
            xnb_ref[rows(2 * b, HT), :] = _layernorm(x0)
            out(1, 0, 384); out(1, 384, D)
            xres_ref[rows(2 * b + 1, HT), :] = y[1][0, D]

            if first:
                for j in range(CH // PW):
                    p = b * (CH // PW) + j
                    for m in range(3):
                        blk = stage_ref[m, rows(p, PW), :]
                        wb_ref[p, :, m * PW:(m + 1) * PW] = pltpu.bitcast(blk.T, u32)
            return carry

        lax.fori_loop(0, NB, phase2, 0)
        ln_b(2 * NB - 1)
        if first:
            cp_wob.wait()

    def out_copy(i):
        r = rows(i, UNROLL * SEG)
        return pltpu.make_async_copy(obuf_ref.at[r], out_hbm.at[r], sem_o)

    def layer_b(layer):
        mem_ref[...] = mem0_ref[...].astype(f32)
        srow = lax.broadcasted_iota(jnp.int32, (L, 2 * L), 0)
        scol = lax.broadcasted_iota(jnp.int32, (L, 2 * L), 1)
        first = scol < L
        kidx = jnp.where(first, scol, scol - L)
        mask = (srow < MEM) | (srow >= kidx)

        def softmax(s):
            s = jnp.where(mask, s * scale, -1e9)
            m1 = jnp.max(jnp.where(first, s, -jnp.inf), axis=1, keepdims=True)
            m2 = jnp.max(jnp.where(first, -jnp.inf, s), axis=1, keepdims=True)
            e = jnp.exp(s - jnp.where(first, m1, m2))
            l1 = jnp.sum(jnp.where(first, e, 0.0), axis=1, keepdims=True)
            l2 = jnp.sum(jnp.where(first, 0.0, e), axis=1, keepdims=True)
            return e * jnp.where(first, 1.0 / l1, 1.0 / l2)

        def oproj(os_, p0, p1):
            o = jnp.concatenate([os_[p] for p in range(p0, p1)], axis=1)
            return jnp.dot(o, wob_ref[p0 * PW:p1 * PW, :], preferred_element_type=f32)

        def step(s, mem):
            r = rows(s, SEG)
            h = jnp.concatenate([mem, xnb_ref[r, :]], axis=0)
            qkv, pr, os_ = {}, {}, {}
            acc = jnp.concatenate([jnp.zeros((MEM, D), f32), xres_ref[r, :]], axis=0)
            for t in range(NP + 2):
                if t < NP:
                    w = pltpu.bitcast(wb_ref[t], bf16)
                    if t == 0:
                        ks = D - 128
                        part = jnp.dot(h[:, :ks], w[:ks], preferred_element_type=f32)
                        part = jnp.concatenate([part[:, :128], part[:, 128:]], axis=1)
                        qkv[t] = part + jnp.dot(h[:, ks:], w[ks:], preferred_element_type=f32)
                    else:
                        qkv[t] = jnp.dot(h, w, preferred_element_type=f32)
                if t == NP:
                    acc = acc + oproj(os_, 0, 3)
                if t == NP + 1:
                    acc = acc + oproj(os_, 3, 7)
                if 0 <= t - 1 < NP:
                    q, k = qkv[t - 1][:, :PW], qkv[t - 1][:, PW:2 * PW]
                    pr[t - 1] = softmax(
                        lax.dot_general(q, _blockdiag(k), _NT, preferred_element_type=f32))
                if 0 <= t - 2 < NP:
                    os_[t - 2] = jnp.dot(pr[t - 2], _blockdiag(qkv[t - 2][:, 2 * PW:]).astype(bf16),
                                         preferred_element_type=f32)
            acc = acc + oproj(os_, 7, NP)
            xnew = acc[MEM:]
            xres_ref[r, :] = xnew
            obuf_ref[r, :] = xnew.astype(bf16)
            return acc[:MEM]

        def steps(i, carry):
            mem = mem_ref[...]
            for u in range(UNROLL):
                mem = step(i * UNROLL + u, mem)
            mem_ref[...] = mem

            @pl.when(layer == 1)
            def _():
                out_copy(i).start()
            return carry

        lax.fori_loop(0, NSEG // UNROLL, steps, 0)

    layer_a(True)

    def layer(i, carry):
        layer_b(i)

        @pl.when(i == 0)
        def _():
            layer_a(False)
        return carry

    lax.fori_loop(0, 2, layer, 0)
    for i in range(NSEG // UNROLL):
        out_copy(i).wait()


@functools.partial(jax.jit, static_argnames=("B_seg_len",))
def pallas_interleave_layers__linear_kernel_hedgehog__memory_aug_recurrent_mem_tr__prompt_kernel(
    A_x, A_wqkv, A_w_phi, A_wo, B_x, B_mem0, B_Wq, B_Wk, B_Wv, B_Wo, B_seg_len=SEG,
):
    del B_x
    assert B_seg_len == SEG
    x = A_x.reshape(S, D)
    wp = A_w_phi.transpose(1, 2, 0)
    mem0 = B_mem0.reshape(MEM, D)
    wqt, wkt, wvt = (w.transpose(1, 2, 0).reshape(HB * DB, D) for w in (B_Wq, B_Wk, B_Wv))
    wob = B_Wo.reshape(HB * DB, D)

    vmem = pl.BlockSpec(memory_space=pltpu.VMEM)
    hbm = pl.BlockSpec(memory_space=pl.ANY)
    out = pl.pallas_call(
        _kernel,
        out_shape=jax.ShapeDtypeStruct((S, D), bf16),
        in_specs=[hbm, hbm, vmem, hbm, vmem, hbm, hbm, hbm, hbm],
        out_specs=hbm,
        scratch_shapes=[
            pltpu.VMEM((S, D), bf16),
            pltpu.VMEM((D, 3 * D), bf16),
            pltpu.VMEM((D, D), bf16),
            pltpu.VMEM((S, D), f32),
            pltpu.VMEM((S, D), f32),
            pltpu.VMEM((NB, D // 2, TB), u32),
            pltpu.VMEM((3, D // 2, D), u32),
            pltpu.VMEM((PR, D), f32),
            pltpu.VMEM((HA // 2, PR + 8, 2 * PR), f32),
            pltpu.VMEM((3, HB * DB, D), bf16),
            pltpu.VMEM((HB * DB, D), bf16),
            pltpu.VMEM((NP, D // 2, 3 * PW), u32),
            pltpu.VMEM((MEM, D), f32),
            pltpu.VMEM((S, D), bf16),
            pltpu.SemaphoreType.DMA((6,)),
            pltpu.SemaphoreType.DMA((3 * NB,)),
            pltpu.SemaphoreType.DMA,
        ],
        compiler_params=pltpu.CompilerParams(vmem_limit_bytes=110 * 1024 * 1024),
    )(x, A_wqkv, wp, A_wo, mem0, wqt, wkt, wvt, wob)
    return out.reshape(1, S, D)
```

```python
import functools

import jax
import jax.numpy as jnp
from jax import lax
import jax.experimental.pallas as pl
import jax.experimental.pallas.tpu as pltpu

f32 = jnp.float32
bf16 = jnp.bfloat16
u32 = jnp.uint32

S = 2048
D = 640
HA = 32
DA = D // HA
HB = 32
DB = 192
MEM = 8
SEG = 32
L = MEM + SEG
NSEG = S // SEG
NP = HB // 2
PW = 2 * DB
NG = 4
PR = 2 * DA
GR = D // NG
TB = 512
NB = S // TB
LN_EPS = 1e-5
LOG2E = 1.4426950408889634
UNROLL = 4

_NT = (((1,), (1,)), ((), ()))


def _layernorm(x):
    m = jnp.mean(x, axis=-1, keepdims=True)
    xc = x - m
    v = jnp.mean(xc * xc, axis=-1, keepdims=True)
    return xc * lax.rsqrt(v + LN_EPS)


def _recip(x):
    r = pl.reciprocal(x, approx=True)
    return r * (2.0 - x * r)


def _fold(op, rows):
    r = functools.reduce(op, rows)
    r = op(r, pltpu.roll(r, 4, 0))
    return op(r, pltpu.roll(r, 2, 0))


def _hedgehog(p):
    rows = [p[8 * i:8 * (i + 1), :] for i in range(PR // 8)]
    mx = _fold(jnp.maximum, rows)
    mn = _fold(jnp.minimum, rows)
    ep = [jnp.exp2(r - mx) for r in rows]
    en = [jnp.exp2(mn - r) for r in rows]
    return ep, en, _fold(jnp.add, ep), _fold(jnp.add, en)


def _blockdiag(x):
    t0, t1, t2 = x[:, :128], x[:, 128:256], x[:, 256:]
    lane = lax.broadcasted_iota(jnp.int32, (L, 128), 1)
    z = jnp.zeros((L, 128), f32)
    top = jnp.concatenate([t0, jnp.where(lane < 64, t1, 0.0), z], axis=1)
    bot = jnp.concatenate([z, jnp.where(lane >= 64, t1, 0.0), t2], axis=1)
    return jnp.concatenate([top, bot], axis=0)


def _kernel(x_hbm, wqkv_hbm, wphi_hbm, wo_hbm, mem0_hbm, wqt_hbm, wkt_hbm, wvt_hbm, wob_hbm,
            out_hbm,
            x_ref, wqkv_ref, wphi_ref, wo_ref, mem0_ref, xres_ref, xnb_ref, xna_ref, wt_ref, wp2_ref,
            kvt_ref, o_ref, stage_ref, wob_ref, wb_ref, mem_ref, sem_a, sem_b, sem_o):
    scale = DB ** -0.5
    XH = 2 * TB
    HT = 128
    NH = TB // HT
    CH = HB * DB // NB

    cp_x0 = pltpu.make_async_copy(x_hbm.at[:XH], x_ref.at[:XH], sem_a.at[0])
    cp_kv = pltpu.make_async_copy(wqkv_hbm.at[:, D:], wqkv_ref.at[:, D:], sem_a.at[1])
    cp_x1 = pltpu.make_async_copy(x_hbm.at[XH:], x_ref.at[XH:], sem_a.at[2])
    cp_q = pltpu.make_async_copy(wqkv_hbm.at[:, :D], wqkv_ref.at[:, :D], sem_a.at[3])
    cp_wo = pltpu.make_async_copy(wo_hbm, wo_ref, sem_a.at[4])
    cp_wob = pltpu.make_async_copy(wob_hbm, wob_ref, sem_a.at[5])
    cp_phi = pltpu.make_async_copy(wphi_hbm, wphi_ref, sem_a.at[6])
    cp_mem = pltpu.make_async_copy(mem0_hbm, mem0_ref, sem_a.at[7])

    def rows(b, n=TB):
        return pl.ds(b * n if isinstance(b, int) else pl.multiple_of(b * n, n), n)

    def cp_b(m, c):
        src = (wqt_hbm, wkt_hbm, wvt_hbm)[m]
        return pltpu.make_async_copy(src.at[rows(c, CH)], stage_ref.at[m, rows(c, CH)],
                                     sem_b.at[c])

    for c in (cp_phi, cp_x0, cp_kv, cp_mem):
        c.start()
    for m in range(3):
        cp_b(m, 0).start(priority=1)

    xres_ref[:HT, :] = jnp.zeros((HT, D), f32)
    cp_phi.wait()
    hrow = lax.broadcasted_iota(jnp.int32, (HA, D), 0)
    hcol = lax.broadcasted_iota(jnp.int32, (HA, D), 1)
    wp = None
    for d in range(DA):
        sel = jnp.where(hcol == hrow * DA + d, 1.0, 0.0)
        t = jnp.dot(wphi_ref[d].astype(f32), sel, preferred_element_type=f32)
        wp = t if wp is None else wp + t
    dup = jnp.where((lax.broadcasted_iota(jnp.int32, (PR, DA), 0) >> 1)
                    == lax.broadcasted_iota(jnp.int32, (PR, DA), 1), 1.0, 0.0)
    wp2_ref[...] = jnp.dot(dup, wp, preferred_element_type=f32)
    cp_mem.wait()
    cp_x0.wait()

    def fold_phi(m):
        row = lax.broadcasted_iota(jnp.int32, (PR, 128), 0)
        col = lax.broadcasted_iota(jnp.int32, (PR, 128), 1)
        parts = []
        for t in range(D // 128):
            blocks = []
            for j in range(3 * t, 3 * t + 4):
                lo = (2 * j + (row & 1)) * DA - 128 * t
                blocks.append(jnp.where((col >= lo) & (col < lo + DA),
                                        wp2_ref[:, 128 * t:128 * (t + 1)], 0.0))
            w = wqkv_ref[:, m * D + 128 * t:m * D + 128 * (t + 1)]
            parts.append(lax.dot_general(jnp.concatenate(blocks, axis=0).astype(bf16), w, _NT,
                                         preferred_element_type=f32))
        out = [parts[0][:PR]]
        for t in range(D // 128):
            out.append(parts[t][PR:3 * PR])
            last = parts[t][3 * PR:]
            out.append(last + parts[t + 1][:PR] if t + 1 < D // 128 else last)
        wt_ref[m] = pltpu.bitcast((jnp.concatenate(out, axis=0) * LOG2E).astype(bf16), u32)

    def wt(m, g):
        return pltpu.bitcast(wt_ref[m, g * GR // 2:(g + 1) * GR // 2, :], bf16)

    def layer_a(first):
        def ln_a(b):
            xn = _layernorm(x_ref[rows(b), :].astype(f32)).astype(bf16)
            xna_ref[b] = pltpu.bitcast(xn.T, u32)

        kvt_ref[...] = jnp.zeros(kvt_ref.shape, f32)
        ln_a(0)

        @pl.when(first)
        def _():
            cp_kv.wait()
            cp_x1.start()
            fold_phi(1)
            wt_ref[2] = pltpu.bitcast(wqkv_ref[:, 2 * D:].T, u32)

        def phase1(b, carry):
            @pl.when(first & (b == XH // TB - 1))
            def _():
                cp_x1.wait()
                cp_q.start()
                cp_wo.start()

            for c in range(1, NB):
                @pl.when(first & (b == c - 1))
                def _():
                    for m in range(3):
                        cp_b(m, c).start(priority=1)

            xn = pltpu.bitcast(xna_ref[b], bf16)
            ones = jnp.ones((8, TB), f32)
            pk, v1 = {}, {}

            def proj_k(g):
                pk[g] = jnp.dot(wt(1, g), xn, preferred_element_type=f32)

            def proj_v(g):
                v1[g] = jnp.dot(wt(2, g), xn, preferred_element_type=f32)

            def kv(g):
                for j in range(GR // PR):
                    ep, en, sp, sn = _hedgehog(pk[g][j * PR:(j + 1) * PR])
                    rp, rn = _recip(sp), _recip(sn)
                    phik = jnp.concatenate([e * rp for e in ep] + [e * rn for e in en],
                                           axis=0).astype(bf16)
                    lhs = jnp.concatenate([v1[g][j * PR:(j + 1) * PR], ones], axis=0)
                    kvt_ref[g * (GR // PR) + j] += lax.dot_general(
                        lhs, phik, _NT, preferred_element_type=f32)

            ln_a(jnp.minimum(b + 1, NB - 1))
            proj_k(0); proj_k(1); proj_v(0); proj_k(2); proj_v(1); kv(0)
            proj_k(3); proj_v(2); proj_v(3); kv(1); kv(2); kv(3)
            return carry

        lax.fori_loop(0, NB, phase1, 0)

        @pl.when(first)
        def _():
            cp_q.wait()
            cp_wo.wait()
            fold_phi(0)
            wt_ref[3] = pltpu.bitcast(wo_ref[...], u32)

        rr = lax.broadcasted_iota(jnp.int32, (PR + 8, 2 * PR), 0)
        cc = lax.broadcasted_iota(jnp.int32, (PR + 8, 2 * PR), 1)
        second = ((rr >= DA) & (rr < PR)) | ((rr >= PR) & ((rr & 1) == 1))
        same_head = second == ((cc & 1) == 1)
        for j in range(HA // 2):
            kvt_ref[j] = jnp.where(same_head, kvt_ref[j], 0.0)

        def ln_b(i):
            xnb_ref[rows(i, HT), :] = _layernorm(xres_ref[rows(i, HT), :])

        def phase2(b, carry):
            @pl.when(first)
            def _():
                @pl.when(b == NB // 4)
                def _():
                    cp_wob.start(priority=1)

                for m in range(3):
                    cp_b(m, b).wait()

            for j in range(CH // PW):
                p = b * (CH // PW) + j
                for m in range(3):
                    blk = stage_ref[m, rows(p, PW), :]
                    wb_ref[p, :, m * PW:(m + 1) * PW] = pltpu.bitcast(blk.T, u32)

            ln_b(jnp.maximum(NH * b - 1, 0))
            sub = lax.broadcasted_iota(jnp.int32, (8, HT), 0)
            top, even = sub < 4, (sub & 1) == 0
            pq, ot, o, y = {}, {}, {}, {}

            def proj_q(i, g):
                xn = pltpu.bitcast(xna_ref[b, :, i * HT:(i + 1) * HT], bf16)
                pq[i, g] = jnp.dot(wt(0, g), xn, preferred_element_type=f32)

            def num(i, g):
                parts = []
                for j in range(GR // PR):
                    ep, en, sp, sn = _hedgehog(pq[i, g][j * PR:(j + 1) * PR])
                    ratio = sp * _recip(sn)
                    phiq = jnp.concatenate(ep + [e * ratio for e in en], axis=0).astype(bf16)
                    n = jnp.dot(kvt_ref[g * (GR // PR) + j], phiq, preferred_element_type=f32)
                    r = _recip(n[PR:, :] + 1e-6 * sp)
                    rs = pltpu.roll(r, 1, 0)
                    ra, rb = jnp.where(even, r, rs), jnp.where(even, rs, r)
                    parts += [n[8 * t:8 * (t + 1), :] * rr_
                              for t, rr_ in enumerate((ra, ra, jnp.where(top, ra, rb), rb, rb))]
                ot[i, g] = jnp.concatenate(parts, axis=0).astype(bf16)

            def out(i, k0, k1, c0=0, c1=D):
                if i not in o:
                    o_ref[i + (b >> 8)] = pltpu.bitcast(
                        jnp.concatenate([ot[i, g] for g in range(NG)], axis=0).T, u32)
                    o[i] = pltpu.bitcast(o_ref[i + (b >> 8)], bf16)
                    y[i] = {}
                if (c0, c1) not in y[i]:
                    y[i][c0, c1] = x_ref[rows(NH * b + i, HT), c0:c1].astype(f32)
                y[i][c0, c1] = y[i][c0, c1] + jnp.dot(
                    o[i][:, k0:k1], pltpu.bitcast(wt_ref[3, k0 // 2:k1 // 2, c0:c1], bf16),
                    preferred_element_type=f32)

            def finish(i, ln):
                xi = jnp.concatenate([y[i][c] for c in sorted(y[i])], axis=1)
                xres_ref[rows(NH * b + i, HT), :] = xi
                if ln:
                    xnb_ref[rows(NH * b + i, HT), :] = _layernorm(xi)

            proj_q(0, 0); proj_q(0, 1); proj_q(0, 2); num(0, 0); proj_q(0, 3); num(0, 1)
            proj_q(1, 0); num(0, 2); proj_q(1, 1); num(0, 3); proj_q(1, 2); num(1, 0)
            proj_q(1, 3); num(1, 1)
            for i in range(2, NH):
                proj_q(i, 0); num(i - 1, 2); proj_q(i, 1); num(i - 1, 3)
                out(i - 2, 0, D); finish(i - 2, True)
                proj_q(i, 2); num(i, 0); proj_q(i, 3); num(i, 1)
            i = NH - 2
            out(i, 0, D, 0, 128); num(i + 1, 2); out(i, 0, D, 128, 256); num(i + 1, 3)
            out(i, 0, D, 256, D); finish(i, True)
            out(i + 1, 0, 384); out(i + 1, 384, D); finish(i + 1, False)
            return carry

        lax.fori_loop(0, NB, phase2, 0)
        ln_b(NH * NB - 1)

        @pl.when(first)
        def _():
            cp_wob.wait()

    NI = NSEG // UNROLL
    out_at = [0, NI // 4, NI // 2, 3 * NI // 4, NI - 1, NI]

    def out_copy(k):
        r = pl.ds(out_at[k] * UNROLL * SEG, (out_at[k + 1] - out_at[k]) * UNROLL * SEG)
        return pltpu.make_async_copy(x_ref.at[r], out_hbm.at[r], sem_o)

    def layer_b(last):
        mem_ref[...] = mem0_ref[...].astype(f32)
        srow = lax.broadcasted_iota(jnp.int32, (L, 2 * L), 0)
        scol = lax.broadcasted_iota(jnp.int32, (L, 2 * L), 1)
        first = scol < L
        kidx = jnp.where(first, scol, scol - L)
        mask = (srow < MEM) | (srow >= kidx)

        def softmax(s):
            s = jnp.where(mask, s * scale, -1e9)
            m1 = jnp.max(jnp.where(first, s, -jnp.inf), axis=1, keepdims=True)
            m2 = jnp.max(jnp.where(first, -jnp.inf, s), axis=1, keepdims=True)
            e = jnp.exp(s - jnp.where(first, m1, m2))
            l1 = jnp.sum(jnp.where(first, e, 0.0), axis=1, keepdims=True)
            l2 = jnp.sum(jnp.where(first, 0.0, e), axis=1, keepdims=True)
            return e * _recip(jnp.where(first, l1, l2))

        def oproj(os_, p0, p1):
            o = jnp.concatenate([os_[p] for p in range(p0, p1)], axis=1)
            return jnp.dot(o, wob_ref[p0 * PW:p1 * PW, :], preferred_element_type=f32)

        def step(s, mem):
            r = rows(s, SEG)
            h = jnp.concatenate([mem, xnb_ref[r, :]], axis=0)
            qkv, pr, os_ = {}, {}, {}
            acc = jnp.concatenate([jnp.zeros((MEM, D), f32), xres_ref[r, :]], axis=0)
            for t in range(NP + 2):
                if t < NP:
                    w = pltpu.bitcast(wb_ref[t], bf16)
                    if t == 0:
                        ks = D - 128
                        part = jnp.dot(h[:, :ks], w[:ks], preferred_element_type=f32)
                        part = jnp.concatenate([part[:, :128], part[:, 128:]], axis=1)
                        qkv[t] = part + jnp.dot(h[:, ks:], w[ks:], preferred_element_type=f32)
                    else:
                        qkv[t] = jnp.dot(h, w, preferred_element_type=f32)
                if t == NP:
                    acc = acc + oproj(os_, 0, 3)
                if t == NP + 1:
                    acc = acc + oproj(os_, 3, 7)
                if 0 <= t - 1 < NP:
                    q, k = qkv[t - 1][:, :PW], qkv[t - 1][:, PW:2 * PW]
                    pr[t - 1] = softmax(
                        lax.dot_general(q, _blockdiag(k), _NT, preferred_element_type=f32))
                if 0 <= t - 2 < NP:
                    os_[t - 2] = jnp.dot(pr[t - 2],
                                         _blockdiag(qkv[t - 2][:, 2 * PW:]).astype(bf16),
                                         preferred_element_type=f32)
            acc = acc + oproj(os_, 7, NP)
            x_ref[r, :] = acc[MEM:].astype(bf16)
            return acc[:MEM]

        def steps(i, carry):
            for k in range(len(out_at) - 2):
                @pl.when(last & (i == out_at[k + 1]))
                def _():
                    out_copy(k).start()

            mem = mem_ref[...]
            for u in range(UNROLL):
                mem = step(i * UNROLL + u, mem)
            mem_ref[...] = mem
            return carry

        lax.fori_loop(0, NI, steps, 0)

    def layer(i, carry):
        layer_a(i == 0)
        layer_b(i == 1)
        return carry

    lax.fori_loop(0, 2, layer, 0)
    out_copy(len(out_at) - 2).start()
    for k in range(len(out_at) - 1):
        out_copy(k).wait()


@functools.partial(jax.jit, static_argnames=("B_seg_len",))
def pallas_interleave_layers__linear_kernel_hedgehog__memory_aug_recurrent_mem_tr__prompt_kernel(
    A_x, A_wqkv, A_w_phi, A_wo, B_x, B_mem0, B_Wq, B_Wk, B_Wv, B_Wo, B_seg_len=SEG,
):
    del B_x
    assert B_seg_len == SEG
    x = A_x.reshape(S, D)
    wp = A_w_phi.transpose(1, 2, 0)
    mem0 = B_mem0.reshape(MEM, D)
    wqt, wkt, wvt = (w.transpose(1, 2, 0).reshape(HB * DB, D) for w in (B_Wq, B_Wk, B_Wv))
    wob = B_Wo.reshape(HB * DB, D)

    hbm = pl.BlockSpec(memory_space=pl.ANY)
    out = pl.pallas_call(
        _kernel,
        out_shape=jax.ShapeDtypeStruct((S, D), bf16),
        in_specs=[hbm] * 9,
        out_specs=hbm,
        scratch_shapes=[
            pltpu.VMEM((S, D), bf16),
            pltpu.VMEM((D, 3 * D), bf16),
            pltpu.VMEM((DA, DA, HA), bf16),
            pltpu.VMEM((D, D), bf16),
            pltpu.VMEM((MEM, D), bf16),
            pltpu.VMEM((S, D), f32),
            pltpu.VMEM((S, D), f32),
            pltpu.VMEM((NB, D // 2, TB), u32),
            pltpu.VMEM((4, D // 2, D), u32),
            pltpu.VMEM((PR, D), f32),
            pltpu.VMEM((HA // 2, PR + 8, 2 * PR), f32),
            pltpu.VMEM((TB // 128, 64, D), u32),
            pltpu.VMEM((3, HB * DB, D), bf16),
            pltpu.VMEM((HB * DB, D), bf16),
            pltpu.VMEM((NP, D // 2, 3 * PW), u32),
            pltpu.VMEM((MEM, D), f32),
            pltpu.SemaphoreType.DMA((8,)),
            pltpu.SemaphoreType.DMA((NB,)),
            pltpu.SemaphoreType.DMA,
        ],
        compiler_params=pltpu.CompilerParams(vmem_limit_bytes=110 * 1024 * 1024),
    )(x, A_wqkv, wp, A_wo, mem0, wqt, wkt, wvt, wob)
    return out.reshape(1, S, D)
```

```python
import functools

import jax
import jax.numpy as jnp
from jax import lax
import jax.experimental.pallas as pl
import jax.experimental.pallas.tpu as pltpu

f32 = jnp.float32
bf16 = jnp.bfloat16
u32 = jnp.uint32

S = 2048
D = 640
HA = 32
DA = D // HA
HB = 32
DB = 192
MEM = 8
SEG = 32
L = MEM + SEG
NSEG = S // SEG
NP = HB // 2
PW = 2 * DB
NG = 4
PR = 2 * DA
GR = D // NG
TB = 512
NB = S // TB
T2 = 256
N2 = S // T2
LN_EPS = 1e-5
PB = 1024
NPRE = 256
LOG2E = 1.4426950408889634
UNROLL = 4

_NT = (((1,), (1,)), ((), ()))


def _layernorm(x):
    m = jnp.mean(x, axis=-1, keepdims=True)
    xc = x - m
    v = jnp.mean(xc * xc, axis=-1, keepdims=True)
    return xc * lax.rsqrt(v + LN_EPS)


def _recip(x):
    r = pl.reciprocal(x, approx=True)
    return r * (2.0 - x * r)


def _fold(op, rows):
    r = functools.reduce(op, rows)
    r = op(r, pltpu.roll(r, 4, 0))
    return op(r, pltpu.roll(r, 2, 0))


def _hedgehog(p):
    rows = [p[8 * i:8 * (i + 1), :] for i in range(PR // 8)]
    mx = _fold(jnp.maximum, rows)
    mn = _fold(jnp.minimum, rows)
    ep = [jnp.exp2(r - mx) for r in rows]
    en = [jnp.exp2(mn - r) for r in rows]
    return ep, en, _fold(jnp.add, ep), _fold(jnp.add, en)


def _blockdiag(x):
    t0, t1, t2 = x[:, :128], x[:, 128:256], x[:, 256:]
    lane = lax.broadcasted_iota(jnp.int32, (L, 128), 1)
    z = jnp.zeros((L, 128), f32)
    top = jnp.concatenate([t0, jnp.where(lane < 64, t1, 0.0), z], axis=1)
    bot = jnp.concatenate([z, jnp.where(lane >= 64, t1, 0.0), t2], axis=1)
    return jnp.concatenate([top, bot], axis=0)


def _kernel(x_hbm, wqkv_hbm, wphi_hbm, wo_hbm, mem0_hbm, wqt_hbm, wkt_hbm, wvt_hbm, wob_hbm,
            out_hbm,
            x_ref, wqkv_ref, wphi_ref, wo_ref, mem0_ref, xres_ref, xnb_ref, xna_ref, wt_ref, wp2_ref,
            kvt_ref, o_ref, stage_ref, wob_ref, wb_ref, pre_ref, mem_ref, sem_a, sem_b, sem_o):
    scale = DB ** -0.5
    XH = 2 * TB
    HT = 128
    NH = T2 // HT
    CH = HB * DB // N2

    cp_x0 = pltpu.make_async_copy(x_hbm.at[:TB], x_ref.at[:TB], sem_a.at[0])
    cp_k = pltpu.make_async_copy(wqkv_hbm.at[:, D:2 * D], wqkv_ref.at[:, D:2 * D], sem_a.at[1])
    cp_v = pltpu.make_async_copy(wqkv_hbm.at[:, 2 * D:], wqkv_ref.at[:, 2 * D:], sem_a.at[8])
    cp_x0b = pltpu.make_async_copy(x_hbm.at[TB:XH], x_ref.at[TB:XH], sem_a.at[9])
    cp_x1 = pltpu.make_async_copy(x_hbm.at[XH:], x_ref.at[XH:], sem_a.at[2])
    cp_q = pltpu.make_async_copy(wqkv_hbm.at[:, :D], wqkv_ref.at[:, :D], sem_a.at[3])
    cp_wo = pltpu.make_async_copy(wo_hbm, wo_ref, sem_a.at[4])
    cp_wob = pltpu.make_async_copy(wob_hbm, wob_ref, sem_a.at[5])
    cp_phi = pltpu.make_async_copy(wphi_hbm, wphi_ref, sem_a.at[6])
    cp_mem = pltpu.make_async_copy(mem0_hbm, mem0_ref, sem_a.at[7])

    def rows(b, n=TB):
        return pl.ds(b * n if isinstance(b, int) else pl.multiple_of(b * n, n), n)

    def cp_b(m, c):
        src = (wqt_hbm, wkt_hbm, wvt_hbm)[m]
        return pltpu.make_async_copy(src.at[rows(c, CH)], stage_ref.at[m, rows(c, CH)],
                                     sem_b.at[c])

    for c in (cp_phi, cp_x0, cp_k, cp_mem):
        c.start()
    for m in range(3):
        cp_b(m, 0).start(priority=1)

    xres_ref[:HT, :] = jnp.zeros((HT, D), f32)
    cp_phi.wait()
    cp_v.start()
    hrow = lax.broadcasted_iota(jnp.int32, (HA, D), 0)
    hcol = lax.broadcasted_iota(jnp.int32, (HA, D), 1)

    def expand(i, wp):
        for d in (4 * i, 4 * i + 1, 4 * i + 2, 4 * i + 3):
            sel = jnp.where(hcol == hrow * DA + d, 1.0, 0.0)
            wp = wp + jnp.dot(wphi_ref[d].astype(f32), sel, preferred_element_type=f32)
        return wp

    wp = lax.fori_loop(0, DA // 4, expand, jnp.zeros((DA, D), f32))
    dup = jnp.where((lax.broadcasted_iota(jnp.int32, (PR, DA), 0) >> 1)
                    == lax.broadcasted_iota(jnp.int32, (PR, DA), 1), 1.0, 0.0)
    wp2_ref[...] = jnp.dot(dup, wp, preferred_element_type=f32)
    cp_x0.wait()

    def fold_phi(m):
        row = lax.broadcasted_iota(jnp.int32, (PR, 128), 0)
        col = lax.broadcasted_iota(jnp.int32, (PR, 128), 1)
        parts = []
        for t in range(D // 128):
            blocks = []
            for j in range(3 * t, 3 * t + 4):
                lo = (2 * j + (row & 1)) * DA - 128 * t
                blocks.append(jnp.where((col >= lo) & (col < lo + DA),
                                        wp2_ref[:, 128 * t:128 * (t + 1)], 0.0))
            w = wqkv_ref[:, m * D + 128 * t:m * D + 128 * (t + 1)]
            parts.append(lax.dot_general(jnp.concatenate(blocks, axis=0).astype(bf16), w, _NT,
                                         preferred_element_type=f32))
        out = [parts[0][:PR]]
        for t in range(D // 128):
            out.append(parts[t][PR:3 * PR])
            last = parts[t][3 * PR:]
            out.append(last + parts[t + 1][:PR] if t + 1 < D // 128 else last)
        wt_ref[m] = pltpu.bitcast((jnp.concatenate(out, axis=0) * LOG2E).astype(bf16), u32)

    def wt(m, g):
        return pltpu.bitcast(wt_ref[m, g * GR // 2:(g + 1) * GR // 2, :], bf16)

    def layer_a(first):
        def ln_a(b):
            xn = _layernorm(x_ref[rows(b), :].astype(f32)).astype(bf16)
            for i in range(TB // HT):
                xna_ref[(TB // HT) * b + i] = pltpu.bitcast(xn[i * HT:(i + 1) * HT].T, u32)

        kvt_ref[...] = jnp.zeros(kvt_ref.shape, f32)
        ln_a(0)

        @pl.when(first)
        def _():
            cp_x0b.start()
            cp_k.wait()
            cp_v.wait()
            fold_phi(1)
            wt_ref[2] = pltpu.bitcast(wqkv_ref[:, 2 * D:].T, u32)
            cp_x1.start()
            cp_x0b.wait()

        def phase1(b, carry):
            @pl.when(first & (b == XH // TB - 1))
            def _():
                cp_x1.wait()
                cp_q.start()
                cp_wo.start()

            for c in range(1, N2):
                @pl.when(first & (b == (c - 1) * NB // N2))
                def _():
                    for m in range(3):
                        cp_b(m, c).start(priority=1)

            xn = pltpu.bitcast(jnp.concatenate(
                [xna_ref[(TB // HT) * b + i] for i in range(TB // HT)], axis=1), bf16)
            ones = jnp.ones((8, TB), f32)
            pk, v1 = {}, {}

            def proj_k(g):
                pk[g] = jnp.dot(wt(1, g), xn, preferred_element_type=f32)

            def proj_v(g):
                v1[g] = jnp.dot(wt(2, g), xn, preferred_element_type=f32)

            def kv(g):
                for j in range(GR // PR):
                    ep, en, sp, sn = _hedgehog(pk[g][j * PR:(j + 1) * PR])
                    rp, rn = _recip(sp), _recip(sn)
                    phik = jnp.concatenate([e * rp for e in ep] + [e * rn for e in en],
                                           axis=0).astype(bf16)
                    lhs = jnp.concatenate([v1[g][j * PR:(j + 1) * PR], ones], axis=0)
                    kvt_ref[g * (GR // PR) + j] += lax.dot_general(
                        lhs, phik, _NT, preferred_element_type=f32)

            ln_a(jnp.minimum(b + 1, NB - 1))
            proj_k(0); proj_k(1); proj_v(0); proj_k(2); proj_v(1); kv(0)
            proj_k(3); proj_v(2); proj_v(3); kv(1); kv(2); kv(3)
            return carry

        lax.fori_loop(0, NB, phase1, 0)

        @pl.when(first)
        def _():
            cp_q.wait()
            cp_wo.wait()
            fold_phi(0)
            wt_ref[3] = pltpu.bitcast(wo_ref[...], u32)

        rr = lax.broadcasted_iota(jnp.int32, (PR + 8, 2 * PR), 0)
        cc = lax.broadcasted_iota(jnp.int32, (PR + 8, 2 * PR), 1)
        second = ((rr >= DA) & (rr < PR)) | ((rr >= PR) & ((rr & 1) == 1))
        same_head = second == ((cc & 1) == 1)
        for j in range(HA // 2):
            kvt_ref[j] = jnp.where(same_head, kvt_ref[j], 0.0)

        def ln_b(i):
            xnb_ref[rows(i, HT), :] = _layernorm(xres_ref[rows(i, HT), :])

        def phase2(prep, b, carry):
            if prep:
                @pl.when(b == N2 // 4)
                def _():
                    cp_wob.start(priority=1)

                for m in range(3):
                    cp_b(m, b).wait()

                for j in range(CH // PW):
                    p = b * (CH // PW) + j
                    for m in range(3):
                        blk = stage_ref[m, rows(p, PW), :]
                        wb_ref[p, :, m * PW:(m + 1) * PW] = pltpu.bitcast(blk.T, u32)

            ln_b(jnp.maximum(NH * b - 1, 0))
            sub = lax.broadcasted_iota(jnp.int32, (8, HT), 0)
            top, even = sub < 4, (sub & 1) == 0
            pq, ot, o, y = {}, {}, {}, {}

            def proj_q(i, g):
                xn = pltpu.bitcast(xna_ref[NH * b + i], bf16)
                pq[i, g] = jnp.dot(wt(0, g), xn, preferred_element_type=f32)

            def num(i, g):
                parts = []
                for j in range(GR // PR):
                    ep, en, sp, sn = _hedgehog(pq[i, g][j * PR:(j + 1) * PR])
                    ratio = sp * _recip(sn)
                    phiq = jnp.concatenate(ep + [e * ratio for e in en], axis=0).astype(bf16)
                    n = jnp.dot(kvt_ref[g * (GR // PR) + j], phiq, preferred_element_type=f32)
                    r = _recip(n[PR:, :] + 1e-6 * sp)
                    rs = pltpu.roll(r, 1, 0)
                    ra, rb = jnp.where(even, r, rs), jnp.where(even, rs, r)
                    parts += [n[8 * t:8 * (t + 1), :] * rr_
                              for t, rr_ in enumerate((ra, ra, jnp.where(top, ra, rb), rb, rb))]
                ot[i, g] = jnp.concatenate(parts, axis=0).astype(bf16)

            def out(i, k0, k1, c0=0, c1=D):
                if i not in o:
                    o_ref[i + (b >> 8)] = pltpu.bitcast(
                        jnp.concatenate([ot[i, g] for g in range(NG)], axis=0).T, u32)
                    o[i] = pltpu.bitcast(o_ref[i + (b >> 8)], bf16)
                    y[i] = {}
                if (c0, c1) not in y[i]:
                    y[i][c0, c1] = x_ref[rows(NH * b + i, HT), c0:c1].astype(f32)
                y[i][c0, c1] = y[i][c0, c1] + jnp.dot(
                    o[i][:, k0:k1], pltpu.bitcast(wt_ref[3, k0 // 2:k1 // 2, c0:c1], bf16),
                    preferred_element_type=f32)

            def finish(i, ln):
                xi = jnp.concatenate([y[i][c] for c in sorted(y[i])], axis=1)
                xres_ref[rows(NH * b + i, HT), :] = xi
                if ln:
                    xnb_ref[rows(NH * b + i, HT), :] = _layernorm(xi)

            proj_q(0, 0); proj_q(0, 1); proj_q(0, 2); num(0, 0); proj_q(0, 3); num(0, 1)
            proj_q(1, 0); num(0, 2); proj_q(1, 1); num(0, 3); proj_q(1, 2); num(1, 0)
            proj_q(1, 3); num(1, 1)
            for i in range(2, NH):
                proj_q(i, 0); num(i - 1, 2); proj_q(i, 1); num(i - 1, 3)
                out(i - 2, 0, D); finish(i - 2, True)
                proj_q(i, 2); num(i, 0); proj_q(i, 3); num(i, 1)
            i = NH - 2
            out(i, 0, D, 0, 128); num(i + 1, 2); out(i, 0, D, 128, 256); num(i + 1, 3)
            out(i, 0, D, 256, D); finish(i, True)
            out(i + 1, 0, 384); out(i + 1, 384, D); finish(i + 1, False)
            return carry

        n_prep = jnp.where(first, N2, 0)
        lax.fori_loop(0, n_prep, functools.partial(phase2, True), 0)
        lax.fori_loop(n_prep, N2, functools.partial(phase2, False), 0)
        def pre(i, carry):
            w = pltpu.bitcast(wb_ref[NP - 1, :, 3 * PW - NPRE:], bf16)
            pre_ref[rows(i, PB), :] = jnp.dot(xnb_ref[rows(i, PB), :], w, preferred_element_type=f32)
            ln_b(NH * N2 - 1)
            return carry

        lax.fori_loop(0, S // PB, pre, 0)

        @pl.when(first)
        def _():
            cp_mem.wait()
            cp_wob.wait()

    NI = NSEG // UNROLL
    out_at = [0, NI // 4, NI // 2, 3 * NI // 4, NI - 1, NI]

    def out_copy(k):
        r = pl.ds(out_at[k] * UNROLL * SEG, (out_at[k + 1] - out_at[k]) * UNROLL * SEG)
        return pltpu.make_async_copy(x_ref.at[r], out_hbm.at[r], sem_o)

    def layer_b(last):
        mem_ref[...] = mem0_ref[...].astype(f32)
        srow = lax.broadcasted_iota(jnp.int32, (L, 2 * L), 0)
        scol = lax.broadcasted_iota(jnp.int32, (L, 2 * L), 1)
        first = scol < L
        kidx = jnp.where(first, scol, scol - L)
        mask = (srow < MEM) | (srow >= kidx)

        def softmax(s):
            s = jnp.where(mask, s * scale, -1e9)
            m1 = jnp.max(jnp.where(first, s, -jnp.inf), axis=1, keepdims=True)
            m2 = jnp.max(jnp.where(first, -jnp.inf, s), axis=1, keepdims=True)
            e = jnp.exp(s - jnp.where(first, m1, m2))
            l1 = jnp.sum(jnp.where(first, e, 0.0), axis=1, keepdims=True)
            l2 = jnp.sum(jnp.where(first, 0.0, e), axis=1, keepdims=True)
            return e * _recip(jnp.where(first, l1, l2))

        def oproj(os_, p0, p1):
            o = jnp.concatenate([os_[p] for p in range(p0, p1)], axis=1)
            return jnp.dot(o, wob_ref[p0 * PW:p1 * PW, :], preferred_element_type=f32)

        pre_at = {4: (0, 256), 8: (256, 512), 12: (512, D)}

        def step(s, mem):
            r = rows(s, SEG)
            h = jnp.concatenate([mem, xnb_ref[r, :]], axis=0)
            qkv, pr, os_ = {}, {}, {}
            acc = jnp.concatenate([jnp.zeros((MEM, D), f32), xres_ref[r, :]], axis=0)
            for t in range(NP + 2):
                if t < NP:
                    w = pltpu.bitcast(wb_ref[t], bf16)
                    if t == 0:
                        ks = D - 128
                        part = jnp.dot(h[:, :ks], w[:ks], preferred_element_type=f32)
                        part = jnp.concatenate([part[:, :128], part[:, 128:]], axis=1)
                        qkv[t] = part + jnp.dot(h[:, ks:], w[ks:], preferred_element_type=f32)
                    elif t == NP - 1:
                        tail = jnp.concatenate([pm, pre_ref[r, :]], axis=0)
                        qkv[t] = jnp.concatenate(
                            [jnp.dot(h, w[:, :3 * PW - NPRE], preferred_element_type=f32), tail], axis=1)
                    else:
                        qkv[t] = jnp.dot(h, w, preferred_element_type=f32)
                if t in pre_at:
                    k0, k1 = pre_at[t]
                    w = pltpu.bitcast(wb_ref[NP - 1, k0 // 2:k1 // 2, 3 * PW - NPRE:], bf16)
                    y = jnp.dot(mem[:, k0:k1], w, preferred_element_type=f32)
                    pm = jnp.concatenate([y[:, :128], y[:, 128:]], axis=1) if k0 == 0 else pm + y
                if t == NP:
                    acc = acc + oproj(os_, 0, 3)
                if t == NP + 1:
                    acc = acc + oproj(os_, 3, 7)
                if 0 <= t - 1 < NP:
                    q, k = qkv[t - 1][:, :PW], qkv[t - 1][:, PW:2 * PW]
                    pr[t - 1] = softmax(
                        lax.dot_general(q, _blockdiag(k), _NT, preferred_element_type=f32))
                if 0 <= t - 2 < NP:
                    os_[t - 2] = jnp.dot(pr[t - 2],
                                         _blockdiag(qkv[t - 2][:, 2 * PW:]).astype(bf16),
                                         preferred_element_type=f32)
            acc = acc + oproj(os_, 7, NP)
            x_ref[r, :] = acc[MEM:].astype(bf16)
            return acc[:MEM]

        def steps(i, carry):
            for k in range(len(out_at) - 2):
                @pl.when(last & (i == out_at[k + 1]))
                def _():
                    out_copy(k).start()

            mem = mem_ref[...]
            for u in range(UNROLL):
                mem = step(i * UNROLL + u, mem)
            mem_ref[...] = mem
            return carry

        lax.fori_loop(0, NI, steps, 0)

    def layer(i, carry):
        layer_a(i == 0)
        layer_b(i == 1)
        return carry

    lax.fori_loop(0, 2, layer, 0)
    out_copy(len(out_at) - 2).start()
    for k in range(len(out_at) - 1):
        out_copy(k).wait()


@functools.partial(jax.jit, static_argnames=("B_seg_len",))
def pallas_interleave_layers__linear_kernel_hedgehog__memory_aug_recurrent_mem_tr__prompt_kernel(
    A_x, A_wqkv, A_w_phi, A_wo, B_x, B_mem0, B_Wq, B_Wk, B_Wv, B_Wo, B_seg_len=SEG,
):
    del B_x
    assert B_seg_len == SEG
    x = A_x.reshape(S, D)
    wp = A_w_phi.transpose(1, 2, 0)
    mem0 = B_mem0.reshape(MEM, D)
    wqt, wkt, wvt = (w.transpose(1, 2, 0).reshape(HB * DB, D) for w in (B_Wq, B_Wk, B_Wv))
    wob = B_Wo.reshape(HB * DB, D)

    hbm = pl.BlockSpec(memory_space=pl.ANY)
    out = pl.pallas_call(
        _kernel,
        out_shape=jax.ShapeDtypeStruct((S, D), bf16),
        in_specs=[hbm] * 9,
        out_specs=hbm,
        scratch_shapes=[
            pltpu.VMEM((S, D), bf16),
            pltpu.VMEM((D, 3 * D), bf16),
            pltpu.VMEM((DA, DA, HA), bf16),
            pltpu.VMEM((D, D), bf16),
            pltpu.VMEM((MEM, D), bf16),
            pltpu.VMEM((S, D), f32),
            pltpu.VMEM((S, D), f32),
            pltpu.VMEM((S // 128, D // 2, 128), u32),
            pltpu.VMEM((4, D // 2, D), u32),
            pltpu.VMEM((PR, D), f32),
            pltpu.VMEM((HA // 2, PR + 8, 2 * PR), f32),
            pltpu.VMEM((T2 // 128, 64, D), u32),
            pltpu.VMEM((3, HB * DB, D), bf16),
            pltpu.VMEM((HB * DB, D), bf16),
            pltpu.VMEM((NP, D // 2, 3 * PW), u32),
            pltpu.VMEM((S, NPRE), f32),
            pltpu.VMEM((MEM, D), f32),
            pltpu.SemaphoreType.DMA((10,)),
            pltpu.SemaphoreType.DMA((N2,)),
            pltpu.SemaphoreType.DMA,
        ],
        compiler_params=pltpu.CompilerParams(vmem_limit_bytes=110 * 1024 * 1024),
    )(x, A_wqkv, wp, A_wo, mem0, wqt, wkt, wvt, wob)
    return out.reshape(1, S, D)
```

```python
import functools

import jax
import jax.numpy as jnp
from jax import lax
import jax.experimental.pallas as pl
import jax.experimental.pallas.tpu as pltpu

f32 = jnp.float32
bf16 = jnp.bfloat16
u32 = jnp.uint32

S = 2048
D = 640
HA = 32
DA = D // HA
HB = 32
DB = 192
MEM = 8
SEG = 32
L = MEM + SEG
NSEG = S // SEG
NP = HB // 2
PW = 2 * DB
NG = 4
PR = 2 * DA
GR = D // NG
TB = 512
NB = S // TB
T2 = 256
N2 = S // T2
LN_EPS = 1e-5
PB = 1024
NPRE = 256
LOG2E = 1.4426950408889634
UNROLL = 4

_NT = (((1,), (1,)), ((), ()))


def _layernorm(x):
    m = jnp.mean(x, axis=-1, keepdims=True)
    xc = x - m
    v = jnp.mean(xc * xc, axis=-1, keepdims=True)
    return xc * lax.rsqrt(v + LN_EPS)


def _recip(x):
    r = pl.reciprocal(x, approx=True)
    return r * (2.0 - x * r)


def _fold(op, rows):
    r = functools.reduce(op, rows)
    r = op(r, pltpu.roll(r, 4, 0))
    return op(r, pltpu.roll(r, 2, 0))


def _hedgehog(p):
    rows = [p[8 * i:8 * (i + 1), :] for i in range(PR // 8)]
    mx = _fold(jnp.maximum, rows)
    mn = _fold(jnp.minimum, rows)
    ep = [jnp.exp2(r - mx) for r in rows]
    en = [jnp.exp2(mn - r) for r in rows]
    return ep, en, _fold(jnp.add, ep), _fold(jnp.add, en)


def _blockdiag(x):
    t0, t1, t2 = x[:, :128], x[:, 128:256], x[:, 256:]
    lane = lax.broadcasted_iota(jnp.int32, (L, 128), 1)
    z = jnp.zeros((L, 128), f32)
    top = jnp.concatenate([t0, jnp.where(lane < 64, t1, 0.0), z], axis=1)
    bot = jnp.concatenate([z, jnp.where(lane >= 64, t1, 0.0), t2], axis=1)
    return jnp.concatenate([top, bot], axis=0)


def _kernel(x_hbm, wqkv_hbm, wphi_hbm, wo_hbm, mem0_hbm, wqt_hbm, wkt_hbm, wvt_hbm, wob_hbm,
            out_hbm,
            x_ref, wqkv_ref, wphi_ref, wo_ref, mem0_ref, xres_ref, xnb_ref, xna_ref, wt_ref, wp2_ref,
            kvt_ref, o_ref, stage_ref, wob_ref, wb_ref, pre_ref, mem_ref, sem_a, sem_b, sem_o):
    scale = DB ** -0.5
    XH = 2 * TB
    HT = 128
    NH = T2 // HT
    CH = HB * DB // N2

    cp_x0 = pltpu.make_async_copy(x_hbm.at[:TB], x_ref.at[:TB], sem_a.at[0])
    cp_k = pltpu.make_async_copy(wqkv_hbm.at[:, D:2 * D], wqkv_ref.at[:, D:2 * D], sem_a.at[1])
    cp_v = pltpu.make_async_copy(wqkv_hbm.at[:, 2 * D:], wqkv_ref.at[:, 2 * D:], sem_a.at[8])
    cp_x0b = pltpu.make_async_copy(x_hbm.at[TB:XH], x_ref.at[TB:XH], sem_a.at[9])
    cp_x1 = pltpu.make_async_copy(x_hbm.at[XH:], x_ref.at[XH:], sem_a.at[2])
    cp_q = pltpu.make_async_copy(wqkv_hbm.at[:, :D], wqkv_ref.at[:, :D], sem_a.at[3])
    cp_wo = pltpu.make_async_copy(wo_hbm, wo_ref, sem_a.at[4])
    cp_wob = pltpu.make_async_copy(wob_hbm, wob_ref, sem_a.at[5])
    cp_phi = pltpu.make_async_copy(wphi_hbm, wphi_ref, sem_a.at[6])
    cp_mem = pltpu.make_async_copy(mem0_hbm, mem0_ref, sem_a.at[7])

    def rows(b, n=TB):
        return pl.ds(b * n if isinstance(b, int) else pl.multiple_of(b * n, n), n)

    def cp_b(m, c):
        src = (wqt_hbm, wkt_hbm, wvt_hbm)[m]
        return pltpu.make_async_copy(src.at[rows(c, CH)], stage_ref.at[m, rows(c, CH)],
                                     sem_b.at[c])

    for c in (cp_phi, cp_x0, cp_k, cp_mem):
        c.start()
    for m in range(3):
        cp_b(m, 0).start(priority=1)

    xres_ref[:HT, :] = jnp.zeros((HT, D), f32)
    cp_phi.wait()
    cp_v.start()
    hrow = lax.broadcasted_iota(jnp.int32, (HA, D), 0)
    hcol = lax.broadcasted_iota(jnp.int32, (HA, D), 1)

    def expand(i, wp):
        for d in (4 * i, 4 * i + 1, 4 * i + 2, 4 * i + 3):
            sel = jnp.where(hcol == hrow * DA + d, 1.0, 0.0)
            wp = wp + jnp.dot(wphi_ref[d].astype(f32), sel, preferred_element_type=f32)
        return wp

    wp = lax.fori_loop(0, DA // 4, expand, jnp.zeros((DA, D), f32))
    dup = jnp.where((lax.broadcasted_iota(jnp.int32, (PR, DA), 0) >> 1)
                    == lax.broadcasted_iota(jnp.int32, (PR, DA), 1), 1.0, 0.0)
    wp2_ref[...] = jnp.dot(dup, wp, preferred_element_type=f32)
    cp_x0.wait()

    def fold_phi(m):
        row = lax.broadcasted_iota(jnp.int32, (PR, 128), 0)
        col = lax.broadcasted_iota(jnp.int32, (PR, 128), 1)
        parts = []
        for t in range(D // 128):
            blocks = []
            for j in range(3 * t, 3 * t + 4):
                lo = (2 * j + (row & 1)) * DA - 128 * t
                blocks.append(jnp.where((col >= lo) & (col < lo + DA),
                                        wp2_ref[:, 128 * t:128 * (t + 1)], 0.0))
            w = wqkv_ref[:, m * D + 128 * t:m * D + 128 * (t + 1)]
            parts.append(lax.dot_general(jnp.concatenate(blocks, axis=0).astype(bf16), w, _NT,
                                         preferred_element_type=f32))
        out = [parts[0][:PR]]
        for t in range(D // 128):
            out.append(parts[t][PR:3 * PR])
            last = parts[t][3 * PR:]
            out.append(last + parts[t + 1][:PR] if t + 1 < D // 128 else last)
        wt_ref[m] = pltpu.bitcast((jnp.concatenate(out, axis=0) * LOG2E).astype(bf16), u32)

    def wt(m, g, dep=None):
        w = wt_ref[m, g * GR // 2:(g + 1) * GR // 2, :]
        if dep is not None:
            never, val = dep
            top = jnp.concatenate([jnp.where(never, val, w[:8, :128]), w[:8, 128:]], axis=1)
            w = jnp.concatenate([top, w[8:]], axis=0)
        return pltpu.bitcast(w, bf16)

    def layer_a(first):
        def ln_a(i):
            xn = _layernorm(x_ref[rows(i, HT), :].astype(f32)).astype(bf16)
            xt = pltpu.bitcast(xn.T, u32)
            xna_ref[i] = xt
            return functools.reduce(jnp.bitwise_or, [xt[64 * t:64 * t + 8] for t in range(D // 128)])

        kvt_ref[...] = jnp.zeros(kvt_ref.shape, f32)
        xn0 = _layernorm(x_ref[:TB, :].astype(f32)).astype(bf16).T
        for i in range(TB // HT):
            xna_ref[i] = pltpu.bitcast(xn0[:, i * HT:(i + 1) * HT], u32)

        @pl.when(first)
        def _():
            cp_x0b.start()
            cp_k.wait()
            cp_v.wait()
            fold_phi(1)
            wt_ref[2] = pltpu.bitcast(wqkv_ref[:, 2 * D:].T, u32)
            cp_x1.start()
            cp_x0b.wait()

        def phase1(b, carry):
            @pl.when(first & (b == XH // TB - 1))
            def _():
                cp_x1.wait()
                cp_q.start()
                cp_wo.start()

            for c in range(1, N2):
                @pl.when(first & (b == (c - 1) * NB // N2))
                def _():
                    for m in range(3):
                        cp_b(m, c).start(priority=1)

            xn = pltpu.bitcast(jnp.concatenate(
                [xna_ref[(TB // HT) * b + i] for i in range(TB // HT)], axis=1), bf16)
            ones = jnp.ones((8, TB), f32)
            pk, v1 = {}, {}

            never = lax.broadcasted_iota(jnp.int32, (8, 128), 0) > b + 64

            def proj_k(g, dep=None):
                pk[g] = jnp.dot(wt(1, g, dep), xn, preferred_element_type=f32)

            def proj_v(g, dep=None):
                v1[g] = jnp.dot(wt(2, g, dep), xn, preferred_element_type=f32)

            def kv(g):
                for j in range(GR // PR):
                    ep, en, sp, sn = _hedgehog(pk[g][j * PR:(j + 1) * PR])
                    rp, rn = _recip(sp), _recip(sn)
                    phik = jnp.concatenate([e * rp for e in ep] + [e * rn for e in en],
                                           axis=0).astype(bf16)
                    lhs = jnp.concatenate([v1[g][j * PR:(j + 1) * PR], ones], axis=0)
                    kvt_ref[g * (GR // PR) + j] += lax.dot_general(
                        lhs, phik, _NT, preferred_element_type=f32)

            nxt = jnp.minimum(b + 1, NB - 1) * (TB // HT)
            dep = [(never, ln_a(nxt + i)) for i in range(TB // HT)]
            proj_k(0); proj_k(1); proj_v(0); proj_k(2, dep[0]); proj_v(1); kv(0)
            proj_k(3, dep[1]); proj_v(2); proj_v(3, dep[2]); kv(1); kv(2); kv(3)
            return carry

        lax.fori_loop(0, NB, phase1, 0)

        @pl.when(first)
        def _():
            cp_q.wait()
            cp_wo.wait()
            fold_phi(0)
            wt_ref[3] = pltpu.bitcast(wo_ref[...], u32)

        rr = lax.broadcasted_iota(jnp.int32, (PR + 8, 2 * PR), 0)
        cc = lax.broadcasted_iota(jnp.int32, (PR + 8, 2 * PR), 1)
        second = ((rr >= DA) & (rr < PR)) | ((rr >= PR) & ((rr & 1) == 1))
        same_head = second == ((cc & 1) == 1)
        for j in range(HA // 2):
            kvt_ref[j] = jnp.where(same_head, kvt_ref[j], 0.0)

        def ln_b(i):
            xn = _layernorm(xres_ref[rows(i, HT), :])
            xnb_ref[rows(i, HT), :] = xn
            return pltpu.bitcast(functools.reduce(
                jnp.add, [xn[8 * t:8 * (t + 1), D - 128:] for t in range(HT // 8)]), u32)

        def phase2(prep, b, carry):
            if prep:
                @pl.when(b == N2 // 4)
                def _():
                    cp_wob.start(priority=1)

                for m in range(3):
                    cp_b(m, b).wait()

                for j in range(CH // PW):
                    p = b * (CH // PW) + j
                    for m in range(3):
                        blk = stage_ref[m, rows(p, PW), :]
                        wb_ref[p, :, m * PW:(m + 1) * PW] = pltpu.bitcast(blk.T, u32)

            never = lax.broadcasted_iota(jnp.int32, (8, 128), 0) > b + 64
            dep = (never, ln_b(jnp.maximum(NH * b - 1, 0)))
            sub = lax.broadcasted_iota(jnp.int32, (8, HT), 0)
            top, even = sub < 4, (sub & 1) == 0
            pq, ot, o, y = {}, {}, {}, {}

            def proj_q(i, g, dep=None):
                xn = pltpu.bitcast(xna_ref[NH * b + i], bf16)
                pq[i, g] = jnp.dot(wt(0, g, dep), xn, preferred_element_type=f32)

            def num(i, g):
                parts = []
                for j in range(GR // PR):
                    ep, en, sp, sn = _hedgehog(pq[i, g][j * PR:(j + 1) * PR])
                    ratio = sp * _recip(sn)
                    phiq = jnp.concatenate(ep + [e * ratio for e in en], axis=0).astype(bf16)
                    n = jnp.dot(kvt_ref[g * (GR // PR) + j], phiq, preferred_element_type=f32)
                    r = _recip(n[PR:, :] + 1e-6 * sp)
                    rs = pltpu.roll(r, 1, 0)
                    ra, rb = jnp.where(even, r, rs), jnp.where(even, rs, r)
                    parts += [n[8 * t:8 * (t + 1), :] * rr_
                              for t, rr_ in enumerate((ra, ra, jnp.where(top, ra, rb), rb, rb))]
                ot[i, g] = jnp.concatenate(parts, axis=0).astype(bf16)

            def out(i, k0, k1, c0=0, c1=D):
                if i not in o:
                    o_ref[i + (b >> 8)] = pltpu.bitcast(
                        jnp.concatenate([ot[i, g] for g in range(NG)], axis=0).T, u32)
                    o[i] = pltpu.bitcast(o_ref[i + (b >> 8)], bf16)
                    y[i] = {}
                if (c0, c1) not in y[i]:
                    y[i][c0, c1] = x_ref[rows(NH * b + i, HT), c0:c1].astype(f32)
                y[i][c0, c1] = y[i][c0, c1] + jnp.dot(
                    o[i][:, k0:k1], pltpu.bitcast(wt_ref[3, k0 // 2:k1 // 2, c0:c1], bf16),
                    preferred_element_type=f32)

            def finish(i, ln):
                xi = jnp.concatenate([y[i][c] for c in sorted(y[i])], axis=1)
                xres_ref[rows(NH * b + i, HT), :] = xi
                if ln:
                    xnb_ref[rows(NH * b + i, HT), :] = _layernorm(xi)

            proj_q(0, 0); proj_q(0, 1); proj_q(0, 2, dep); num(0, 0); proj_q(0, 3); num(0, 1)
            proj_q(1, 0); num(0, 2); proj_q(1, 1); num(0, 3); proj_q(1, 2); num(1, 0)
            proj_q(1, 3); num(1, 1)
            for i in range(2, NH):
                proj_q(i, 0); num(i - 1, 2); proj_q(i, 1); num(i - 1, 3)
                out(i - 2, 0, D); finish(i - 2, True)
                proj_q(i, 2); num(i, 0); proj_q(i, 3); num(i, 1)
            i = NH - 2
            out(i, 0, D, 0, 128); num(i + 1, 2); out(i, 0, D, 128, 256); num(i + 1, 3)
            out(i, 0, D, 256, D); finish(i, True)
            out(i + 1, 0, 384); out(i + 1, 384, D); finish(i + 1, False)
            return carry

        n_prep = jnp.where(first, N2, 0)
        lax.fori_loop(0, n_prep, functools.partial(phase2, True), 0)
        lax.fori_loop(n_prep, N2, functools.partial(phase2, False), 0)
        def pre(i, carry):
            w = pltpu.bitcast(wb_ref[NP - 1, :, 3 * PW - NPRE:], bf16)
            pre_ref[rows(i, PB), :] = jnp.dot(xnb_ref[rows(i, PB), :], w, preferred_element_type=f32)
            ln_b(NH * N2 - 1)
            return carry

        lax.fori_loop(0, S // PB, pre, 0)

        @pl.when(first)
        def _():
            cp_mem.wait()
            cp_wob.wait()

    NI = NSEG // UNROLL
    out_at = [0, NI // 4, NI // 2, 3 * NI // 4, NI - 1, NI]

    def out_copy(k):
        r = pl.ds(out_at[k] * UNROLL * SEG, (out_at[k + 1] - out_at[k]) * UNROLL * SEG)
        return pltpu.make_async_copy(x_ref.at[r], out_hbm.at[r], sem_o)

    def layer_b(last):
        mem_ref[...] = mem0_ref[...].astype(f32)
        srow = lax.broadcasted_iota(jnp.int32, (L, 2 * L), 0)
        scol = lax.broadcasted_iota(jnp.int32, (L, 2 * L), 1)
        first = scol < L
        kidx = jnp.where(first, scol, scol - L)
        mask = (srow < MEM) | (srow >= kidx)

        def softmax(s):
            s = jnp.where(mask, s * scale, -1e9)
            m1 = jnp.max(jnp.where(first, s, -jnp.inf), axis=1, keepdims=True)
            m2 = jnp.max(jnp.where(first, -jnp.inf, s), axis=1, keepdims=True)
            e = jnp.exp(s - jnp.where(first, m1, m2))
            l1 = jnp.sum(jnp.where(first, e, 0.0), axis=1, keepdims=True)
            l2 = jnp.sum(jnp.where(first, 0.0, e), axis=1, keepdims=True)
            return e * _recip(jnp.where(first, l1, l2))

        def oproj(os_, p0, p1):
            o = jnp.concatenate([os_[p] for p in range(p0, p1)], axis=1)
            return jnp.dot(o, wob_ref[p0 * PW:p1 * PW, :], preferred_element_type=f32)

        pre_at = {4: (0, 256), 8: (256, 512), 12: (512, D)}

        def step(s, mem):
            r = rows(s, SEG)
            h = jnp.concatenate([mem, xnb_ref[r, :]], axis=0)
            qkv, pr, os_ = {}, {}, {}
            acc = jnp.concatenate([jnp.zeros((MEM, D), f32), xres_ref[r, :]], axis=0)
            for t in range(NP + 2):
                if t < NP:
                    w = pltpu.bitcast(wb_ref[t], bf16)
                    if t == 0:
                        ks = D - 128
                        part = jnp.dot(h[:, :ks], w[:ks], preferred_element_type=f32)
                        part = jnp.concatenate([part[:, :128], part[:, 128:]], axis=1)
                        qkv[t] = part + jnp.dot(h[:, ks:], w[ks:], preferred_element_type=f32)
                    elif t == NP - 1:
                        tail = jnp.concatenate([pm, pre_ref[r, :]], axis=0)
                        qkv[t] = jnp.concatenate(
                            [jnp.dot(h, w[:, :3 * PW - NPRE], preferred_element_type=f32), tail], axis=1)
                    else:
                        qkv[t] = jnp.dot(h, w, preferred_element_type=f32)
                if t in pre_at:
                    k0, k1 = pre_at[t]
                    w = pltpu.bitcast(wb_ref[NP - 1, k0 // 2:k1 // 2, 3 * PW - NPRE:], bf16)
                    y = jnp.dot(mem[:, k0:k1], w, preferred_element_type=f32)
                    pm = jnp.concatenate([y[:, :128], y[:, 128:]], axis=1) if k0 == 0 else pm + y
                if t == NP:
                    acc = acc + oproj(os_, 0, 3)
                if t == NP + 1:
                    acc = acc + oproj(os_, 3, 7)
                if 0 <= t - 1 < NP:
                    q, k = qkv[t - 1][:, :PW], qkv[t - 1][:, PW:2 * PW]
                    pr[t - 1] = softmax(
                        lax.dot_general(q, _blockdiag(k), _NT, preferred_element_type=f32))
                if 0 <= t - 2 < NP:
                    os_[t - 2] = jnp.dot(pr[t - 2],
                                         _blockdiag(qkv[t - 2][:, 2 * PW:]).astype(bf16),
                                         preferred_element_type=f32)
            acc = acc + oproj(os_, 7, NP)
            x_ref[r, :] = acc[MEM:].astype(bf16)
            return acc[:MEM]

        def steps(i, carry):
            for k in range(len(out_at) - 2):
                @pl.when(last & (i == out_at[k + 1]))
                def _():
                    out_copy(k).start()

            mem = mem_ref[...]
            for u in range(UNROLL):
                mem = step(i * UNROLL + u, mem)
            mem_ref[...] = mem
            return carry

        lax.fori_loop(0, NI, steps, 0)

    def layer(i, carry):
        layer_a(i == 0)
        layer_b(i == 1)
        return carry

    lax.fori_loop(0, 2, layer, 0)
    out_copy(len(out_at) - 2).start()
    for k in range(len(out_at) - 1):
        out_copy(k).wait()


@functools.partial(jax.jit, static_argnames=("B_seg_len",))
def pallas_interleave_layers__linear_kernel_hedgehog__memory_aug_recurrent_mem_tr__prompt_kernel(
    A_x, A_wqkv, A_w_phi, A_wo, B_x, B_mem0, B_Wq, B_Wk, B_Wv, B_Wo, B_seg_len=SEG,
):
    del B_x
    assert B_seg_len == SEG
    x = A_x.reshape(S, D)
    wp = A_w_phi.transpose(1, 2, 0)
    mem0 = B_mem0.reshape(MEM, D)
    wqt, wkt, wvt = (w.transpose(1, 2, 0).reshape(HB * DB, D) for w in (B_Wq, B_Wk, B_Wv))
    wob = B_Wo.reshape(HB * DB, D)

    hbm = pl.BlockSpec(memory_space=pl.ANY)
    out = pl.pallas_call(
        _kernel,
        out_shape=jax.ShapeDtypeStruct((S, D), bf16),
        in_specs=[hbm] * 9,
        out_specs=hbm,
        scratch_shapes=[
            pltpu.VMEM((S, D), bf16),
            pltpu.VMEM((D, 3 * D), bf16),
            pltpu.VMEM((DA, DA, HA), bf16),
            pltpu.VMEM((D, D), bf16),
            pltpu.VMEM((MEM, D), bf16),
            pltpu.VMEM((S, D), f32),
            pltpu.VMEM((S, D), f32),
            pltpu.VMEM((S // 128, D // 2, 128), u32),
            pltpu.VMEM((4, D // 2, D), u32),
            pltpu.VMEM((PR, D), f32),
            pltpu.VMEM((HA // 2, PR + 8, 2 * PR), f32),
            pltpu.VMEM((T2 // 128, 64, D), u32),
            pltpu.VMEM((3, HB * DB, D), bf16),
            pltpu.VMEM((HB * DB, D), bf16),
            pltpu.VMEM((NP, D // 2, 3 * PW), u32),
            pltpu.VMEM((S, NPRE), f32),
            pltpu.VMEM((MEM, D), f32),
            pltpu.SemaphoreType.DMA((10,)),
            pltpu.SemaphoreType.DMA((N2,)),
            pltpu.SemaphoreType.DMA,
        ],
        compiler_params=pltpu.CompilerParams(vmem_limit_bytes=110 * 1024 * 1024),
    )(x, A_wqkv, wp, A_wo, mem0, wqt, wkt, wvt, wob)
    return out.reshape(1, S, D)
```

```python
import functools

import jax
import jax.numpy as jnp
from jax import lax
import jax.experimental.pallas as pl
import jax.experimental.pallas.tpu as pltpu

f32 = jnp.float32
bf16 = jnp.bfloat16
u32 = jnp.uint32

S = 2048
D = 640
HA = 32
DA = D // HA
HB = 32
DB = 192
MEM = 8
SEG = 32
L = MEM + SEG
NSEG = S // SEG
NP = HB // 2
PW = 2 * DB
NG = 4
PR = 2 * DA
GR = D // NG
TB = 256
NB = S // TB
T2 = 256
N2 = S // T2
T2B = 512
LN_EPS = 1e-5
PB = 1024
NPRE = 256
LOG2E = 1.4426950408889634
UNROLL = 4

_NT = (((1,), (1,)), ((), ()))


def _layernorm(x):
    m = jnp.mean(x, axis=-1, keepdims=True)
    xc = x - m
    v = jnp.mean(xc * xc, axis=-1, keepdims=True)
    return xc * lax.rsqrt(v + LN_EPS)


def _recip(x):
    r = pl.reciprocal(x, approx=True)
    return r * (2.0 - x * r)


def _fold(op, rows):
    r = functools.reduce(op, rows)
    r = op(r, pltpu.roll(r, 4, 0))
    return op(r, pltpu.roll(r, 2, 0))


def _hedgehog(p):
    rows = [p[8 * i:8 * (i + 1), :] for i in range(PR // 8)]
    mx = _fold(jnp.maximum, rows)
    mn = _fold(jnp.minimum, rows)
    ep = [jnp.exp2(r - mx) for r in rows]
    en = [jnp.exp2(mn - r) for r in rows]
    return ep, en, _fold(jnp.add, ep), _fold(jnp.add, en)


def _blockdiag(x):
    t0, t1, t2 = x[:, :128], x[:, 128:256], x[:, 256:]
    lane = lax.broadcasted_iota(jnp.int32, (L, 128), 1)
    z = jnp.zeros((L, 128), f32)
    top = jnp.concatenate([t0, jnp.where(lane < 64, t1, 0.0), z], axis=1)
    bot = jnp.concatenate([z, jnp.where(lane >= 64, t1, 0.0), t2], axis=1)
    return jnp.concatenate([top, bot], axis=0)


def _kernel(x_hbm, wqkv_hbm, wphi_hbm, wo_hbm, mem0_hbm, wqt_hbm, wkt_hbm, wvt_hbm, wob_hbm,
            out_hbm,
            x_ref, wqkv_ref, wphi_ref, wo_ref, mem0_ref, xres_ref, xnb_ref, xna_ref, wt_ref, wp2_ref,
            kvt_ref, o_ref, stage_ref, wob_ref, wb_ref, pre_ref, mem_ref, sem_a, sem_b, sem_o):
    scale = DB ** -0.5
    XH = 2 * TB
    HT = 128
    CH = HB * DB // N2

    cp_x0 = pltpu.make_async_copy(x_hbm.at[:TB], x_ref.at[:TB], sem_a.at[0])
    cp_k = pltpu.make_async_copy(wqkv_hbm.at[:, D:2 * D], wqkv_ref.at[:, D:2 * D], sem_a.at[1])
    cp_v = pltpu.make_async_copy(wqkv_hbm.at[:, 2 * D:], wqkv_ref.at[:, 2 * D:], sem_a.at[8])
    cp_x0b = pltpu.make_async_copy(x_hbm.at[TB:XH], x_ref.at[TB:XH], sem_a.at[9])
    cp_x1 = pltpu.make_async_copy(x_hbm.at[XH:], x_ref.at[XH:], sem_a.at[2])
    cp_q = pltpu.make_async_copy(wqkv_hbm.at[:, :D], wqkv_ref.at[:, :D], sem_a.at[3])
    cp_wo = pltpu.make_async_copy(wo_hbm, wo_ref, sem_a.at[4])
    cp_wob = pltpu.make_async_copy(wob_hbm, wob_ref, sem_a.at[5])
    cp_phi = pltpu.make_async_copy(wphi_hbm, wphi_ref, sem_a.at[6])
    cp_mem = pltpu.make_async_copy(mem0_hbm, mem0_ref, sem_a.at[7])

    def rows(b, n=TB):
        return pl.ds(b * n if isinstance(b, int) else pl.multiple_of(b * n, n), n)

    def cp_b(m, c):
        src = (wqt_hbm, wkt_hbm, wvt_hbm)[m]
        return pltpu.make_async_copy(src.at[rows(c, CH)], stage_ref.at[c, m * CH:(m + 1) * CH],
                                     sem_b.at[c])

    for c in (cp_phi, cp_x0, cp_k, cp_mem):
        c.start()
    for m in range(3):
        cp_b(m, 0).start(priority=1)

    xres_ref[:HT, :] = jnp.zeros((HT, D), f32)
    cp_phi.wait()
    cp_v.start()
    hrow = lax.broadcasted_iota(jnp.int32, (HA, D), 0)
    hcol = lax.broadcasted_iota(jnp.int32, (HA, D), 1)

    def expand(i, wp):
        for d in (4 * i, 4 * i + 1, 4 * i + 2, 4 * i + 3):
            sel = jnp.where(hcol == hrow * DA + d, 1.0, 0.0)
            wp = wp + jnp.dot(wphi_ref[d].astype(f32), sel, preferred_element_type=f32)
        return wp

    wp = lax.fori_loop(0, DA // 4, expand, jnp.zeros((DA, D), f32))
    dup = jnp.where((lax.broadcasted_iota(jnp.int32, (PR, DA), 0) >> 1)
                    == lax.broadcasted_iota(jnp.int32, (PR, DA), 1), 1.0, 0.0)
    wp2_ref[...] = jnp.dot(dup, wp, preferred_element_type=f32)
    cp_x0.wait()

    def fold_phi(m):
        row = lax.broadcasted_iota(jnp.int32, (PR, 128), 0)
        col = lax.broadcasted_iota(jnp.int32, (PR, 128), 1)
        parts = []
        for t in range(D // 128):
            blocks = []
            for j in range(3 * t, 3 * t + 4):
                lo = (2 * j + (row & 1)) * DA - 128 * t
                blocks.append(jnp.where((col >= lo) & (col < lo + DA),
                                        wp2_ref[:, 128 * t:128 * (t + 1)], 0.0))
            w = wqkv_ref[:, m * D + 128 * t:m * D + 128 * (t + 1)]
            parts.append(lax.dot_general(jnp.concatenate(blocks, axis=0).astype(bf16), w, _NT,
                                         preferred_element_type=f32))
        out = [parts[0][:PR]]
        for t in range(D // 128):
            out.append(parts[t][PR:3 * PR])
            last = parts[t][3 * PR:]
            out.append(last + parts[t + 1][:PR] if t + 1 < D // 128 else last)
        wt_ref[m] = pltpu.bitcast((jnp.concatenate(out, axis=0) * LOG2E).astype(bf16), u32)

    def wt(m, g, dep=None):
        w = wt_ref[m, g * GR // 2:(g + 1) * GR // 2, :]
        if dep is not None:
            never, val = dep
            top = jnp.concatenate([jnp.where(never, val, w[:8, :128]), w[:8, 128:]], axis=1)
            w = jnp.concatenate([top, w[8:]], axis=0)
        return pltpu.bitcast(w, bf16)

    def layer_a(first):
        def ln_a(i):
            xn = _layernorm(x_ref[rows(i, HT), :].astype(f32)).astype(bf16)
            xt = pltpu.bitcast(xn.T, u32)
            xna_ref[i] = xt
            return functools.reduce(jnp.bitwise_or, [xt[64 * t:64 * t + 8] for t in range(D // 128)])

        kvt_ref[...] = jnp.zeros(kvt_ref.shape, f32)
        xn0 = _layernorm(x_ref[:TB, :].astype(f32)).astype(bf16).T
        for i in range(TB // HT):
            xna_ref[i] = pltpu.bitcast(xn0[:, i * HT:(i + 1) * HT], u32)

        @pl.when(first)
        def _():
            cp_x0b.start()
            cp_k.wait()
            cp_v.wait()
            fold_phi(1)
            wt_ref[2] = pltpu.bitcast(wqkv_ref[:, 2 * D:].T, u32)
            cp_x1.start()
            cp_x0b.wait()

        def phase1(b, carry):
            @pl.when(first & (b == XH // TB - 1))
            def _():
                cp_x1.wait()
                cp_q.start()
                cp_wo.start()

            for c in range(1, N2):
                @pl.when(first & (b == (c - 1) * NB // N2))
                def _():
                    for m in range(3):
                        cp_b(m, c).start(priority=1)

            xn = pltpu.bitcast(jnp.concatenate(
                [xna_ref[(TB // HT) * b + i] for i in range(TB // HT)], axis=1), bf16)
            ones = jnp.ones((8, TB), f32)
            pk, v1 = {}, {}

            never = lax.broadcasted_iota(jnp.int32, (8, 128), 0) > b + 64

            def proj_k(g, dep=None):
                pk[g] = jnp.dot(wt(1, g, dep), xn, preferred_element_type=f32)

            def proj_v(g, dep=None):
                v1[g] = jnp.dot(wt(2, g, dep), xn, preferred_element_type=f32)

            def kv(g):
                for j in range(GR // PR):
                    ep, en, sp, sn = _hedgehog(pk[g][j * PR:(j + 1) * PR])
                    rp, rn = _recip(sp), _recip(sn)
                    phik = jnp.concatenate([e * rp for e in ep] + [e * rn for e in en],
                                           axis=0).astype(bf16)
                    lhs = jnp.concatenate([v1[g][j * PR:(j + 1) * PR], ones], axis=0)
                    kvt_ref[g * (GR // PR) + j] += lax.dot_general(
                        lhs, phik, _NT, preferred_element_type=f32)

            nxt = jnp.minimum(b + 1, NB - 1) * (TB // HT)
            dep = [(never, ln_a(nxt + i)) for i in range(TB // HT)]
            proj_k(0); proj_k(1); proj_v(0); proj_k(2); proj_v(1, dep[0]); kv(0)
            proj_k(3); proj_v(2); proj_v(3); kv(1); kv(2); kv(3)
            return carry

        lax.fori_loop(0, NB, phase1, 0)

        @pl.when(first)
        def _():
            cp_q.wait()
            cp_wo.wait()
            fold_phi(0)
            wt_ref[3] = pltpu.bitcast(wo_ref[...], u32)

        rr = lax.broadcasted_iota(jnp.int32, (PR + 8, 2 * PR), 0)
        cc = lax.broadcasted_iota(jnp.int32, (PR + 8, 2 * PR), 1)
        second = ((rr >= DA) & (rr < PR)) | ((rr >= PR) & ((rr & 1) == 1))
        same_head = second == ((cc & 1) == 1)
        for j in range(HA // 2):
            kvt_ref[j] = jnp.where(same_head, kvt_ref[j], 0.0)

        def ln_b(i):
            xn = _layernorm(xres_ref[rows(i, HT), :])
            xnb_ref[rows(i, HT), :] = xn
            return pltpu.bitcast(functools.reduce(
                jnp.add, [xn[8 * t:8 * (t + 1), D - 128:] for t in range(HT // 8)]), u32)

        def phase2(prep, b, carry):
            NH = (T2 if prep else T2B) // HT
            if prep:
                @pl.when(b == N2 // 4)
                def _():
                    cp_wob.start(priority=1)

                for m in range(3):
                    cp_b(m, b).wait()

                for j in range(CH // PW):
                    p = b * (CH // PW) + j
                    for m in range(3):
                        blk = stage_ref[b, m * CH + j * PW:m * CH + (j + 1) * PW, :]
                        wb_ref[p, :, m * PW:(m + 1) * PW] = pltpu.bitcast(blk.T, u32)

            never = lax.broadcasted_iota(jnp.int32, (8, 128), 0) > b + 64
            dep = (never, ln_b(jnp.maximum(NH * b - 1, 0)))
            sub = lax.broadcasted_iota(jnp.int32, (8, HT), 0)
            top, even = sub < 4, (sub & 1) == 0
            pq, ot, o, y = {}, {}, {}, {}

            def proj_q(i, g, dep=None):
                xn = pltpu.bitcast(xna_ref[NH * b + i], bf16)
                pq[i, g] = jnp.dot(wt(0, g, dep), xn, preferred_element_type=f32)

            def num(i, g):
                parts = []
                for j in range(GR // PR):
                    ep, en, sp, sn = _hedgehog(pq[i, g][j * PR:(j + 1) * PR])
                    ratio = sp * _recip(sn)
                    phiq = jnp.concatenate(ep + [e * ratio for e in en], axis=0).astype(bf16)
                    n = jnp.dot(kvt_ref[g * (GR // PR) + j], phiq, preferred_element_type=f32)
                    r = _recip(n[PR:, :] + 1e-6 * sp)
                    rs = pltpu.roll(r, 1, 0)
                    ra, rb = jnp.where(even, r, rs), jnp.where(even, rs, r)
                    parts += [n[8 * t:8 * (t + 1), :] * rr_
                              for t, rr_ in enumerate((ra, ra, jnp.where(top, ra, rb), rb, rb))]
                ot[i, g] = jnp.concatenate(parts, axis=0).astype(bf16)

            def out(i, k0, k1, c0=0, c1=D):
                if i not in o:
                    o_ref[i + (b >> 8)] = pltpu.bitcast(
                        jnp.concatenate([ot[i, g] for g in range(NG)], axis=0).T, u32)
                    o[i] = pltpu.bitcast(o_ref[i + (b >> 8)], bf16)
                    y[i] = {}
                if (c0, c1) not in y[i]:
                    y[i][c0, c1] = x_ref[rows(NH * b + i, HT), c0:c1].astype(f32)
                y[i][c0, c1] = y[i][c0, c1] + jnp.dot(
                    o[i][:, k0:k1], pltpu.bitcast(wt_ref[3, k0 // 2:k1 // 2, c0:c1], bf16),
                    preferred_element_type=f32)

            def finish(i, ln):
                xi = jnp.concatenate([y[i][c] for c in sorted(y[i])], axis=1)
                xres_ref[rows(NH * b + i, HT), :] = xi
                if ln:
                    xnb_ref[rows(NH * b + i, HT), :] = _layernorm(xi)

            proj_q(0, 0); proj_q(0, 1); proj_q(0, 2, dep); num(0, 0); proj_q(0, 3); num(0, 1)
            proj_q(1, 0); num(0, 2); proj_q(1, 1); num(0, 3); proj_q(1, 2); num(1, 0)
            proj_q(1, 3); num(1, 1)
            for i in range(2, NH):
                proj_q(i, 0); num(i - 1, 2); proj_q(i, 1); num(i - 1, 3)
                out(i - 2, 0, D); finish(i - 2, True)
                proj_q(i, 2); num(i, 0); proj_q(i, 3); num(i, 1)
            i = NH - 2
            out(i, 0, D, 0, 128); num(i + 1, 2); out(i, 0, D, 128, 256); num(i + 1, 3)
            out(i, 0, D, 256, D); finish(i, True)
            out(i + 1, 0, 384); out(i + 1, 384, D); finish(i + 1, False)
            return carry

        n_prep = jnp.where(first, N2, 0)
        lax.fori_loop(0, n_prep, functools.partial(phase2, True), 0)
        lax.fori_loop(0, jnp.where(first, 0, S // T2B), functools.partial(phase2, False), 0)
        def pre(i, carry):
            w = pltpu.bitcast(wb_ref[NP - 1, :, 3 * PW - NPRE:], bf16)
            pre_ref[rows(i, PB), :] = jnp.dot(xnb_ref[rows(i, PB), :], w, preferred_element_type=f32)
            ln_b(S // HT - 1)
            return carry

        lax.fori_loop(0, S // PB, pre, 0)

        @pl.when(first)
        def _():
            cp_mem.wait()
            cp_wob.wait()

    NI = NSEG // UNROLL
    out_at = [0, NI // 4, NI // 2, 3 * NI // 4, NI - 1, NI]

    def out_copy(k):
        r = pl.ds(out_at[k] * UNROLL * SEG, (out_at[k + 1] - out_at[k]) * UNROLL * SEG)
        return pltpu.make_async_copy(x_ref.at[r], out_hbm.at[r], sem_o)

    def layer_b(last):
        mem_ref[...] = mem0_ref[...].astype(f32)
        srow = lax.broadcasted_iota(jnp.int32, (L, 2 * L), 0)
        scol = lax.broadcasted_iota(jnp.int32, (L, 2 * L), 1)
        first = scol < L
        kidx = jnp.where(first, scol, scol - L)
        mask = (srow < MEM) | (srow >= kidx)

        def softmax(s):
            s = jnp.where(mask, s * scale, -1e9)
            m1 = jnp.max(jnp.where(first, s, -jnp.inf), axis=1, keepdims=True)
            m2 = jnp.max(jnp.where(first, -jnp.inf, s), axis=1, keepdims=True)
            e = jnp.exp(s - jnp.where(first, m1, m2))
            l1 = jnp.sum(jnp.where(first, e, 0.0), axis=1, keepdims=True)
            l2 = jnp.sum(jnp.where(first, 0.0, e), axis=1, keepdims=True)
            return e * _recip(jnp.where(first, l1, l2))

        def oproj(os_, p0, p1):
            o = jnp.concatenate([os_[p] for p in range(p0, p1)], axis=1)
            return jnp.dot(o, wob_ref[p0 * PW:p1 * PW, :], preferred_element_type=f32)

        pre_at = {4: (0, 256), 8: (256, 512), 12: (512, D)}

        def step(s, mem):
            r = rows(s, SEG)
            h = jnp.concatenate([mem, xnb_ref[r, :]], axis=0)
            qkv, pr, os_ = {}, {}, {}
            acc = jnp.concatenate([jnp.zeros((MEM, D), f32), xres_ref[r, :]], axis=0)
            for t in range(NP + 2):
                if t < NP:
                    w = pltpu.bitcast(wb_ref[t], bf16)
                    if t == 0:
                        ks = D - 128
                        part = jnp.dot(h[:, :ks], w[:ks], preferred_element_type=f32)
                        part = jnp.concatenate([part[:, :128], part[:, 128:]], axis=1)
                        qkv[t] = part + jnp.dot(h[:, ks:], w[ks:], preferred_element_type=f32)
                    elif t == NP - 1:
                        tail = jnp.concatenate([pm, pre_ref[r, :]], axis=0)
                        qkv[t] = jnp.concatenate(
                            [jnp.dot(h, w[:, :3 * PW - NPRE], preferred_element_type=f32), tail], axis=1)
                    else:
                        qkv[t] = jnp.dot(h, w, preferred_element_type=f32)
                if t in pre_at:
                    k0, k1 = pre_at[t]
                    w = pltpu.bitcast(wb_ref[NP - 1, k0 // 2:k1 // 2, 3 * PW - NPRE:], bf16)
                    y = jnp.dot(mem[:, k0:k1], w, preferred_element_type=f32)
                    pm = jnp.concatenate([y[:, :128], y[:, 128:]], axis=1) if k0 == 0 else pm + y
                if t == NP:
                    acc = acc + oproj(os_, 0, 3)
                if t == NP + 1:
                    acc = acc + oproj(os_, 3, 7)
                if 0 <= t - 1 < NP:
                    q, k = qkv[t - 1][:, :PW], qkv[t - 1][:, PW:2 * PW]
                    pr[t - 1] = softmax(
                        lax.dot_general(q, _blockdiag(k), _NT, preferred_element_type=f32))
                if 0 <= t - 2 < NP:
                    os_[t - 2] = jnp.dot(pr[t - 2],
                                         _blockdiag(qkv[t - 2][:, 2 * PW:]).astype(bf16),
                                         preferred_element_type=f32)
            acc = acc + oproj(os_, 7, NP)
            x_ref[r, :] = acc[MEM:].astype(bf16)
            return acc[:MEM]

        def steps(i, carry):
            for k in range(len(out_at) - 2):
                @pl.when(last & (i == out_at[k + 1]))
                def _():
                    out_copy(k).start()

            mem = mem_ref[...]
            for u in range(UNROLL):
                mem = step(i * UNROLL + u, mem)
            mem_ref[...] = mem
            return carry

        lax.fori_loop(0, NI, steps, 0)

    def layer(i, carry):
        layer_a(i == 0)
        layer_b(i == 1)
        return carry

    lax.fori_loop(0, 2, layer, 0)
    out_copy(len(out_at) - 2).start()
    for k in range(len(out_at) - 1):
        out_copy(k).wait()


@functools.partial(jax.jit, static_argnames=("B_seg_len",))
def pallas_interleave_layers__linear_kernel_hedgehog__memory_aug_recurrent_mem_tr__prompt_kernel(
    A_x, A_wqkv, A_w_phi, A_wo, B_x, B_mem0, B_Wq, B_Wk, B_Wv, B_Wo, B_seg_len=SEG,
):
    del B_x
    assert B_seg_len == SEG
    x = A_x.reshape(S, D)
    wp = A_w_phi.transpose(1, 2, 0)
    mem0 = B_mem0.reshape(MEM, D)
    wqt, wkt, wvt = (w.transpose(1, 2, 0).reshape(HB * DB, D) for w in (B_Wq, B_Wk, B_Wv))
    wob = B_Wo.reshape(HB * DB, D)

    hbm = pl.BlockSpec(memory_space=pl.ANY)
    out = pl.pallas_call(
        _kernel,
        out_shape=jax.ShapeDtypeStruct((S, D), bf16),
        in_specs=[hbm] * 9,
        out_specs=hbm,
        scratch_shapes=[
            pltpu.VMEM((S, D), bf16),
            pltpu.VMEM((D, 3 * D), bf16),
            pltpu.VMEM((DA, DA, HA), bf16),
            pltpu.VMEM((D, D), bf16),
            pltpu.VMEM((MEM, D), bf16),
            pltpu.VMEM((S, D), f32),
            pltpu.VMEM((S, D), f32),
            pltpu.VMEM((S // 128, D // 2, 128), u32),
            pltpu.VMEM((4, D // 2, D), u32),
            pltpu.VMEM((PR, D), f32),
            pltpu.VMEM((HA // 2, PR + 8, 2 * PR), f32),
            pltpu.VMEM((T2B // 128, 64, D), u32),
            pltpu.VMEM((N2, 3 * HB * DB // N2, D), bf16),
            pltpu.VMEM((HB * DB, D), bf16),
            pltpu.VMEM((NP, D // 2, 3 * PW), u32),
            pltpu.VMEM((S, NPRE), f32),
            pltpu.VMEM((MEM, D), f32),
            pltpu.SemaphoreType.DMA((10,)),
            pltpu.SemaphoreType.DMA((N2,)),
            pltpu.SemaphoreType.DMA,
        ],
        compiler_params=pltpu.CompilerParams(vmem_limit_bytes=110 * 1024 * 1024),
    )(x, A_wqkv, wp, A_wo, mem0, wqt, wkt, wvt, wob)
    return out.reshape(1, S, D)
```

```python
import functools

import jax
import jax.numpy as jnp
from jax import lax
import jax.experimental.pallas as pl
import jax.experimental.pallas.tpu as pltpu

f32 = jnp.float32
bf16 = jnp.bfloat16
u32 = jnp.uint32

S = 2048
D = 640
HA = 32
DA = D // HA
HB = 32
DB = 192
MEM = 8
SEG = 32
L = MEM + SEG
NSEG = S // SEG
NP = HB // 2
PW = 2 * DB
NG = 4
PR = 2 * DA
GR = D // NG
TB = 256
NB = S // TB
T2 = 256
N2 = S // T2
T2B = 512
LN_EPS = 1e-5
PB = 1024
NPRE = 256
LOG2E = 1.4426950408889634
UNROLL = 4

_NT = (((1,), (1,)), ((), ()))
_INTERLEAVE = [h * DB + c * 64 for c in range(3) for h in range(2)]


def _layernorm(x):
    m = jnp.mean(x, axis=-1, keepdims=True)
    xc = x - m
    v = jnp.mean(xc * xc, axis=-1, keepdims=True)
    return xc * lax.rsqrt(v + LN_EPS)


def _recip(x):
    r = pl.reciprocal(x, approx=True)
    return r * (2.0 - x * r)


def _fold(op, rows):
    r = functools.reduce(op, rows)
    r = op(r, pltpu.roll(r, 4, 0))
    return op(r, pltpu.roll(r, 2, 0))


def _hedgehog(p):
    rows = [p[8 * i:8 * (i + 1), :] for i in range(PR // 8)]
    mx = _fold(jnp.maximum, rows)
    mn = _fold(jnp.minimum, rows)
    ep = [jnp.exp2(r - mx) for r in rows]
    en = [jnp.exp2(mn - r) for r in rows]
    return ep, en, _fold(jnp.add, ep), _fold(jnp.add, en)


def _blockdiag(x):
    t0, t1, t2 = x[:, :128], x[:, 128:256], x[:, 256:]
    lane = lax.broadcasted_iota(jnp.int32, (L, 128), 1)
    z = jnp.zeros((L, 128), f32)
    top = jnp.concatenate([t0, jnp.where(lane < 64, t1, 0.0), z], axis=1)
    bot = jnp.concatenate([z, jnp.where(lane >= 64, t1, 0.0), t2], axis=1)
    return jnp.concatenate([top, bot], axis=0)


def _kernel(x_hbm, wqkv_hbm, wphi_hbm, wo_hbm, mem0_hbm, wqt_hbm, wkt_hbm, wvt_hbm, wob_hbm,
            out_hbm,
            x_ref, wqkv_ref, wphi_ref, wo_ref, mem0_ref, xres_ref, xnb_ref, xna_ref, wt_ref, wp2_ref,
            kvt_ref, o_ref, stage_ref, wob_ref, wo2_ref, wb_ref, pre_ref, mem_ref, sem_a, sem_b, sem_o):
    scale = DB ** -0.5
    XH = 2 * TB
    HT = 128
    CH = HB * DB // N2

    cp_x0 = pltpu.make_async_copy(x_hbm.at[:TB], x_ref.at[:TB], sem_a.at[0])
    cp_k = pltpu.make_async_copy(wqkv_hbm.at[:, D:2 * D], wqkv_ref.at[:, D:2 * D], sem_a.at[1])
    cp_v = pltpu.make_async_copy(wqkv_hbm.at[:, 2 * D:], wqkv_ref.at[:, 2 * D:], sem_a.at[8])
    cp_x0b = pltpu.make_async_copy(x_hbm.at[TB:XH], x_ref.at[TB:XH], sem_a.at[9])
    cp_x1 = pltpu.make_async_copy(x_hbm.at[XH:], x_ref.at[XH:], sem_a.at[2])
    cp_q = pltpu.make_async_copy(wqkv_hbm.at[:, :D], wqkv_ref.at[:, :D], sem_a.at[3])
    cp_wo = pltpu.make_async_copy(wo_hbm, wo_ref, sem_a.at[4])
    cp_wob = pltpu.make_async_copy(wob_hbm, wob_ref, sem_a.at[5])
    cp_phi = pltpu.make_async_copy(wphi_hbm, wphi_ref, sem_a.at[6])
    cp_mem = pltpu.make_async_copy(mem0_hbm, mem0_ref, sem_a.at[7])

    def rows(b, n=TB):
        return pl.ds(b * n if isinstance(b, int) else pl.multiple_of(b * n, n), n)

    def cp_b(m, c):
        src = (wqt_hbm, wkt_hbm, wvt_hbm)[m]
        return pltpu.make_async_copy(src.at[rows(c, CH)], stage_ref.at[c, m * CH:(m + 1) * CH],
                                     sem_b.at[c])

    for c in (cp_phi, cp_x0, cp_k, cp_mem):
        c.start()
    for m in range(3):
        cp_b(m, 0).start(priority=1)

    xres_ref[:HT, :] = jnp.zeros((HT, D), f32)
    cp_phi.wait()
    cp_v.start()
    hrow = lax.broadcasted_iota(jnp.int32, (HA, D), 0)
    hcol = lax.broadcasted_iota(jnp.int32, (HA, D), 1)

    def expand(i, wp):
        for d in (4 * i, 4 * i + 1, 4 * i + 2, 4 * i + 3):
            sel = jnp.where(hcol == hrow * DA + d, 1.0, 0.0)
            wp = wp + jnp.dot(wphi_ref[d].astype(f32), sel, preferred_element_type=f32)
        return wp

    wp = lax.fori_loop(0, DA // 4, expand, jnp.zeros((DA, D), f32))
    dup = jnp.where((lax.broadcasted_iota(jnp.int32, (PR, DA), 0) >> 1)
                    == lax.broadcasted_iota(jnp.int32, (PR, DA), 1), 1.0, 0.0)
    wp2_ref[...] = jnp.dot(dup, wp, preferred_element_type=f32)
    cp_x0.wait()

    def fold_phi(m):
        row = lax.broadcasted_iota(jnp.int32, (PR, 128), 0)
        col = lax.broadcasted_iota(jnp.int32, (PR, 128), 1)
        parts = []
        for t in range(D // 128):
            blocks = []
            for j in range(3 * t, 3 * t + 4):
                lo = (2 * j + (row & 1)) * DA - 128 * t
                blocks.append(jnp.where((col >= lo) & (col < lo + DA),
                                        wp2_ref[:, 128 * t:128 * (t + 1)], 0.0))
            w = wqkv_ref[:, m * D + 128 * t:m * D + 128 * (t + 1)]
            parts.append(lax.dot_general(jnp.concatenate(blocks, axis=0).astype(bf16), w, _NT,
                                         preferred_element_type=f32))
        out = [parts[0][:PR]]
        for t in range(D // 128):
            out.append(parts[t][PR:3 * PR])
            last = parts[t][3 * PR:]
            out.append(last + parts[t + 1][:PR] if t + 1 < D // 128 else last)
        wt_ref[m] = pltpu.bitcast((jnp.concatenate(out, axis=0) * LOG2E).astype(bf16), u32)

    def wt(m, g, dep=None):
        w = wt_ref[m, g * GR // 2:(g + 1) * GR // 2, :]
        if dep is not None:
            never, val = dep
            top = jnp.concatenate([jnp.where(never, val, w[:8, :128]), w[:8, 128:]], axis=1)
            w = jnp.concatenate([top, w[8:]], axis=0)
        return pltpu.bitcast(w, bf16)

    def layer_a(first):
        def ln_a(i):
            xn = _layernorm(x_ref[rows(i, HT), :].astype(f32)).astype(bf16)
            xt = pltpu.bitcast(xn.T, u32)
            xna_ref[i] = xt
            return functools.reduce(jnp.bitwise_or, [xt[64 * t:64 * t + 8] for t in range(D // 128)])

        kvt_ref[...] = jnp.zeros(kvt_ref.shape, f32)
        xn0 = _layernorm(x_ref[:TB, :].astype(f32)).astype(bf16).T
        for i in range(TB // HT):
            xna_ref[i] = pltpu.bitcast(xn0[:, i * HT:(i + 1) * HT], u32)

        @pl.when(first)
        def _():
            cp_x0b.start()
            cp_k.wait()
            cp_v.wait()
            fold_phi(1)
            wt_ref[2] = pltpu.bitcast(wqkv_ref[:, 2 * D:].T, u32)
            cp_x1.start()
            cp_x0b.wait()

        def phase1(b, carry):
            @pl.when(first & (b == XH // TB - 1))
            def _():
                cp_x1.wait()
                cp_q.start()
                cp_wo.start()

            for c in range(1, N2):
                @pl.when(first & (b == (c - 1) * NB // N2))
                def _():
                    for m in range(3):
                        cp_b(m, c).start(priority=1)

            xn = pltpu.bitcast(jnp.concatenate(
                [xna_ref[(TB // HT) * b + i] for i in range(TB // HT)], axis=1), bf16)
            ones = jnp.ones((8, TB), f32)
            pk, v1 = {}, {}

            never = lax.broadcasted_iota(jnp.int32, (8, 128), 0) > b + 64

            def proj_k(g, dep=None):
                pk[g] = jnp.dot(wt(1, g, dep), xn, preferred_element_type=f32)

            def proj_v(g, dep=None):
                v1[g] = jnp.dot(wt(2, g, dep), xn, preferred_element_type=f32)

            def kv(g):
                for j in range(GR // PR):
                    ep, en, sp, sn = _hedgehog(pk[g][j * PR:(j + 1) * PR])
                    rp, rn = _recip(sp), _recip(sn)
                    phik = jnp.concatenate([e * rp for e in ep] + [e * rn for e in en],
                                           axis=0).astype(bf16)
                    lhs = jnp.concatenate([v1[g][j * PR:(j + 1) * PR], ones], axis=0)
                    kvt_ref[g * (GR // PR) + j] += lax.dot_general(
                        lhs, phik, _NT, preferred_element_type=f32)

            nxt = jnp.minimum(b + 1, NB - 1) * (TB // HT)
            dep = [(never, ln_a(nxt + i)) for i in range(TB // HT)]
            proj_k(0); proj_k(1); proj_v(0); proj_k(2); proj_v(1, dep[0]); kv(0)
            proj_k(3); proj_v(2); proj_v(3); kv(1); kv(2); kv(3)
            return carry

        lax.fori_loop(0, NB, phase1, 0)

        @pl.when(first)
        def _():
            cp_q.wait()
            cp_wo.wait()
            fold_phi(0)
            wt_ref[3] = pltpu.bitcast(wo_ref[...], u32)

        rr = lax.broadcasted_iota(jnp.int32, (PR + 8, 2 * PR), 0)
        cc = lax.broadcasted_iota(jnp.int32, (PR + 8, 2 * PR), 1)
        second = ((rr >= DA) & (rr < PR)) | ((rr >= PR) & ((rr & 1) == 1))
        same_head = second == ((cc & 1) == 1)
        for j in range(HA // 2):
            kvt_ref[j] = jnp.where(same_head, kvt_ref[j], 0.0)

        def ln_b(i):
            xn = _layernorm(xres_ref[rows(i, HT), :])
            xnb_ref[rows(i, HT), :] = xn
            return pltpu.bitcast(functools.reduce(
                jnp.add, [xn[8 * t:8 * (t + 1), D - 128:] for t in range(HT // 8)]), u32)

        def phase2(prep, b, carry):
            NH = (T2 if prep else T2B) // HT
            if prep:
                @pl.when(b == N2 // 4)
                def _():
                    cp_wob.start(priority=1)

                for m in range(3):
                    cp_b(m, b).wait()

                for j in range(CH // PW):
                    p = b * (CH // PW) + j
                    for m in range(3):
                        r0 = m * CH + j * PW
                        if m == 2:
                            blk = jnp.concatenate(
                                [stage_ref[b, r0 + r:r0 + r + 64, :] for r in _INTERLEAVE], axis=0)
                        else:
                            blk = stage_ref[b, r0:r0 + PW, :]
                        wb_ref[p, :, m * PW:(m + 1) * PW] = pltpu.bitcast(blk.T, u32)

            never = lax.broadcasted_iota(jnp.int32, (8, 128), 0) > b + 64
            dep = (never, ln_b(jnp.maximum(NH * b - 1, 0)))
            sub = lax.broadcasted_iota(jnp.int32, (8, HT), 0)
            top, even = sub < 4, (sub & 1) == 0
            pq, ot, o, y = {}, {}, {}, {}

            def proj_q(i, g, dep=None):
                xn = pltpu.bitcast(xna_ref[NH * b + i], bf16)
                pq[i, g] = jnp.dot(wt(0, g, dep), xn, preferred_element_type=f32)

            def num(i, g):
                parts = []
                for j in range(GR // PR):
                    ep, en, sp, sn = _hedgehog(pq[i, g][j * PR:(j + 1) * PR])
                    ratio = sp * _recip(sn)
                    phiq = jnp.concatenate(ep + [e * ratio for e in en], axis=0).astype(bf16)
                    n = jnp.dot(kvt_ref[g * (GR // PR) + j], phiq, preferred_element_type=f32)
                    r = _recip(n[PR:, :] + 1e-6 * sp)
                    rs = pltpu.roll(r, 1, 0)
                    ra, rb = jnp.where(even, r, rs), jnp.where(even, rs, r)
                    parts += [n[8 * t:8 * (t + 1), :] * rr_
                              for t, rr_ in enumerate((ra, ra, jnp.where(top, ra, rb), rb, rb))]
                ot[i, g] = jnp.concatenate(parts, axis=0).astype(bf16)

            def out(i, k0, k1, c0=0, c1=D):
                if i not in o:
                    o_ref[i + (b >> 8)] = pltpu.bitcast(
                        jnp.concatenate([ot[i, g] for g in range(NG)], axis=0).T, u32)
                    o[i] = pltpu.bitcast(o_ref[i + (b >> 8)], bf16)
                    y[i] = {}
                if (c0, c1) not in y[i]:
                    y[i][c0, c1] = x_ref[rows(NH * b + i, HT), c0:c1].astype(f32)
                y[i][c0, c1] = y[i][c0, c1] + jnp.dot(
                    o[i][:, k0:k1], pltpu.bitcast(wt_ref[3, k0 // 2:k1 // 2, c0:c1], bf16),
                    preferred_element_type=f32)

            def finish(i, ln):
                xi = jnp.concatenate([y[i][c] for c in sorted(y[i])], axis=1)
                xres_ref[rows(NH * b + i, HT), :] = xi
                if ln:
                    xnb_ref[rows(NH * b + i, HT), :] = _layernorm(xi)

            proj_q(0, 0); proj_q(0, 1); proj_q(0, 2, dep); num(0, 0); proj_q(0, 3); num(0, 1)
            proj_q(1, 0); num(0, 2); proj_q(1, 1); num(0, 3); proj_q(1, 2); num(1, 0)
            proj_q(1, 3); num(1, 1)
            for i in range(2, NH):
                proj_q(i, 0); num(i - 1, 2); proj_q(i, 1); num(i - 1, 3)
                out(i - 2, 0, D); finish(i - 2, True)
                proj_q(i, 2); num(i, 0); proj_q(i, 3); num(i, 1)
            i = NH - 2
            out(i, 0, D, 0, 128); num(i + 1, 2); out(i, 0, D, 128, 256); num(i + 1, 3)
            out(i, 0, D, 256, D); finish(i, True)
            out(i + 1, 0, 384); out(i + 1, 384, D); finish(i + 1, False)
            return carry

        n_prep = jnp.where(first, N2, 0)
        lax.fori_loop(0, n_prep, functools.partial(phase2, True), 0)
        lax.fori_loop(0, jnp.where(first, 0, S // T2B), functools.partial(phase2, False), 0)
        def pre(i, carry):
            w = pltpu.bitcast(wb_ref[NP - 1, :, 3 * PW - NPRE:], bf16)
            pre_ref[rows(i, PB), :] = jnp.dot(xnb_ref[rows(i, PB), :], w, preferred_element_type=f32)
            ln_b(S // HT - 1)
            return carry

        lax.fori_loop(0, S // PB, pre, 0)

        @pl.when(first)
        def _():
            cp_mem.wait()
            cp_wob.wait()

            def pack(p, carry):
                for i, r in enumerate(_INTERLEAVE):
                    src = wob_ref[pl.ds(pl.multiple_of(p * PW + r, 64), 64), :]
                    wo2_ref[p, 32 * i:32 * (i + 1), :] = pltpu.bitcast(src, u32)
                return carry

            lax.fori_loop(0, NP, pack, 0)

    NI = NSEG // UNROLL
    out_at = [0, NI // 4, NI // 2, 3 * NI // 4, NI - 1, NI]

    def out_copy(k):
        r = pl.ds(out_at[k] * UNROLL * SEG, (out_at[k + 1] - out_at[k]) * UNROLL * SEG)
        return pltpu.make_async_copy(x_ref.at[r], out_hbm.at[r], sem_o)

    def layer_b(last):
        mem_ref[...] = mem0_ref[...].astype(f32)
        LM = L - 8
        srow = lax.broadcasted_iota(jnp.int32, (LM, 2 * L), 0)
        scol = lax.broadcasted_iota(jnp.int32, (LM, 2 * L), 1)
        first = scol < L
        kidx = jnp.where(first, scol, scol - L)
        mask = (srow < MEM) | (srow + 8 >= kidx)
        lo40 = lax.broadcasted_iota(jnp.int32, (L, PW), 1) % 128 < 64
        lo8 = lax.broadcasted_iota(jnp.int32, (8, 128), 1) < 64
        sub8 = lax.broadcasted_iota(jnp.int32, (8, 128), 0)
        NA = 384

        def softmax(s):
            s = jnp.where(mask, s * scale, -1e9)
            m1 = jnp.max(jnp.where(first, s, -jnp.inf), axis=1, keepdims=True)
            m2 = jnp.max(jnp.where(first, -jnp.inf, s), axis=1, keepdims=True)
            e = jnp.exp(s - jnp.where(first, m1, m2))
            l1 = jnp.sum(jnp.where(first, e, 0.0), axis=1, keepdims=True)
            l2 = jnp.sum(jnp.where(first, 0.0, e), axis=1, keepdims=True)
            return e * _recip(jnp.where(first, l1, l2))

        pre_at = {4: (0, 256), 8: (256, 512), 12: (512, D)}

        def step(s, mem):
            never = sub8 > s + 128

            def bc(x, j, t, dep):
                blk = x[8 * (j // 8):8 * (j // 8) + 8, 128 * t:128 * (t + 1)]
                if dep is not None:
                    blk = jnp.where(never, dep, blk)
                return jnp.broadcast_to(blk[j % 8:j % 8 + 1], (8, 128))

            def vpu_attn(q, k, v):
                qg = q[MEM:MEM + 8] * (scale * LOG2E)
                a0, b2 = qg[:, :128], qg[:, 256:]
                a1 = jnp.where(lo8, qg[:, 128:256], 0.0)
                b1 = jnp.where(lo8, 0.0, qg[:, 128:256])
                cols, dep = [], None
                for j in range(MEM + 8):
                    k0, k1, k2 = bc(k, j, 0, dep), bc(k, j, 1, dep), bc(k, j, 2, dep)
                    dep = b1 * k1 + b2 * k2
                    sc = jnp.where(lo8, jnp.sum(a0 * k0 + a1 * k1, axis=1, keepdims=True),
                                   jnp.sum(dep, axis=1, keepdims=True))
                    if j > MEM:
                        sc = jnp.where(sub8 >= j - MEM, sc, -1e9 * LOG2E)
                    cols.append(sc)
                m = functools.reduce(jnp.maximum, cols)
                es = [jnp.exp2(c - m) for c in cols]
                rl = _recip(functools.reduce(jnp.add, es))
                accs = [None] * 3
                for j in range(MEM + 8):
                    for t in range(3):
                        x = es[j] * bc(v, j, t, accs[t] if j else es[0])
                        accs[t] = x if j == 0 else accs[t] + x
                return jnp.concatenate([x * rl for x in accs], axis=1)

            r = rows(s, SEG)
            h = jnp.concatenate([mem, xnb_ref[r, :]], axis=0)
            qkv, pr, os_, ov, pm = {}, {}, {}, {}, []
            acc = {(0, NA): None, (NA, D): None}
            for c0, c1 in acc:
                acc[c0, c1] = jnp.concatenate(
                    [jnp.zeros((MEM, c1 - c0), f32), xres_ref[r, c0:c1]], axis=0)

            def proj(t):
                w = pltpu.bitcast(wb_ref[t], bf16)
                if t == 0:
                    part = jnp.dot(h[:, :NA], w[:NA], preferred_element_type=f32)
                    part = jnp.concatenate([part[:, :128], part[:, 128:]], axis=1)
                    qkv[t] = part + jnp.dot(h[:, NA:], w[NA:], preferred_element_type=f32)
                elif t == NP - 1:
                    tail = jnp.concatenate([pm[0], pre_ref[r, :]], axis=0)
                    qkv[t] = jnp.concatenate(
                        [jnp.dot(h, w[:, :3 * PW - NPRE], preferred_element_type=f32), tail], axis=1)
                else:
                    qkv[t] = jnp.dot(h, w, preferred_element_type=f32)
                ov[t] = vpu_attn(qkv[t][:, :PW], qkv[t][:, PW:2 * PW], qkv[t][:, 2 * PW:])
                if t in pre_at:
                    k0, k1 = pre_at[t]
                    w = pltpu.bitcast(wb_ref[NP - 1, k0 // 2:k1 // 2, 3 * PW - NPRE:], bf16)
                    y = jnp.dot(mem[:, k0:k1], w, preferred_element_type=f32)
                    pm[:] = [pm[0] + y if pm else jnp.concatenate([y[:, :128], y[:, 128:]], axis=1)]

            def scores(t):
                q, k = qkv[t][:, :PW], qkv[t][:, PW:2 * PW]
                qm = jnp.concatenate([q[:MEM], q[MEM + 8:]], axis=0)
                pr[t] = softmax(lax.dot_general(qm, _blockdiag(k), _NT, preferred_element_type=f32))

            def pv(t):
                v = qkv[t][:, 2 * PW:]
                vv = jnp.concatenate([jnp.where(lo40, v, 0.0), jnp.where(lo40, 0.0, v)], axis=0)
                om = jnp.dot(pr[t], vv.astype(bf16), preferred_element_type=f32)
                os_[t] = jnp.concatenate([om[:MEM], ov[t], om[MEM:]], axis=0)

            def oproj(late, p0, p1):
                c0, c1 = (NA, D) if late else (0, NA)
                o = jnp.concatenate([os_[p] for p in range(p0, p1)], axis=1)
                w = pltpu.bitcast(jnp.concatenate(
                    [wo2_ref[p, :, c0:c1] for p in range(p0, p1)], axis=0), bf16)
                acc[c0, c1] = acc[c0, c1] + jnp.dot(o, w, preferred_element_type=f32)

            for t in range(NP):
                proj(t)
                if t >= 1:
                    scores(t - 1)
                if t >= 2:
                    pv(t - 2)
                if t >= 3:
                    oproj(False, t - 3, t - 2)
            oproj(True, 0, 3); scores(NP - 1); oproj(True, 3, 5); pv(NP - 2); oproj(True, 5, 7)
            oproj(False, NP - 3, NP - 2); oproj(True, 7, 9); oproj(False, NP - 2, NP - 1)
            pv(NP - 1); oproj(True, 9, 12); oproj(False, NP - 1, NP); oproj(True, 12, NP)
            y = jnp.concatenate([acc[0, NA], acc[NA, D]], axis=1)
            x_ref[r, :] = y[MEM:].astype(bf16)
            return y[:MEM]

        def steps(i, carry):
            for k in range(len(out_at) - 2):
                @pl.when(last & (i == out_at[k + 1]))
                def _():
                    out_copy(k).start()

            mem = mem_ref[...]
            for u in range(UNROLL):
                mem = step(i * UNROLL + u, mem)
            mem_ref[...] = mem
            return carry

        lax.fori_loop(0, NI, steps, 0)

    def layer(i, carry):
        layer_a(i == 0)
        layer_b(i == 1)
        return carry

    lax.fori_loop(0, 2, layer, 0)
    out_copy(len(out_at) - 2).start()
    for k in range(len(out_at) - 1):
        out_copy(k).wait()


@functools.partial(jax.jit, static_argnames=("B_seg_len",))
def pallas_interleave_layers__linear_kernel_hedgehog__memory_aug_recurrent_mem_tr__prompt_kernel(
    A_x, A_wqkv, A_w_phi, A_wo, B_x, B_mem0, B_Wq, B_Wk, B_Wv, B_Wo, B_seg_len=SEG,
):
    del B_x
    assert B_seg_len == SEG
    x = A_x.reshape(S, D)
    wp = A_w_phi.transpose(1, 2, 0)
    mem0 = B_mem0.reshape(MEM, D)
    wqt, wkt, wvt = (w.transpose(1, 2, 0).reshape(HB * DB, D) for w in (B_Wq, B_Wk, B_Wv))
    wob = B_Wo.reshape(HB * DB, D)

    hbm = pl.BlockSpec(memory_space=pl.ANY)
    out = pl.pallas_call(
        _kernel,
        out_shape=jax.ShapeDtypeStruct((S, D), bf16),
        in_specs=[hbm] * 9,
        out_specs=hbm,
        scratch_shapes=[
            pltpu.VMEM((S, D), bf16),
            pltpu.VMEM((D, 3 * D), bf16),
            pltpu.VMEM((DA, DA, HA), bf16),
            pltpu.VMEM((D, D), bf16),
            pltpu.VMEM((MEM, D), bf16),
            pltpu.VMEM((S, D), f32),
            pltpu.VMEM((S, D), f32),
            pltpu.VMEM((S // 128, D // 2, 128), u32),
            pltpu.VMEM((4, D // 2, D), u32),
            pltpu.VMEM((PR, D), f32),
            pltpu.VMEM((HA // 2, PR + 8, 2 * PR), f32),
            pltpu.VMEM((T2B // 128, 64, D), u32),
            pltpu.VMEM((N2, 3 * HB * DB // N2, D), bf16),
            pltpu.VMEM((HB * DB, D), bf16),
            pltpu.VMEM((NP, PW // 2, D), u32),
            pltpu.VMEM((NP, D // 2, 3 * PW), u32),
            pltpu.VMEM((S, NPRE), f32),
            pltpu.VMEM((MEM, D), f32),
            pltpu.SemaphoreType.DMA((10,)),
            pltpu.SemaphoreType.DMA((N2,)),
            pltpu.SemaphoreType.DMA,
        ],
        compiler_params=pltpu.CompilerParams(vmem_limit_bytes=110 * 1024 * 1024),
    )(x, A_wqkv, wp, A_wo, mem0, wqt, wkt, wvt, wob)
    return out.reshape(1, S, D)
```

```python
import functools

import jax
import jax.numpy as jnp
from jax import lax
import jax.experimental.pallas as pl
import jax.experimental.pallas.tpu as pltpu

f32 = jnp.float32
bf16 = jnp.bfloat16
u32 = jnp.uint32

S = 2048
D = 640
HA = 32
DA = D // HA
HB = 32
DB = 192
MEM = 8
SEG = 32
L = MEM + SEG
NSEG = S // SEG
NP = HB // 2
PW = 2 * DB
NG = 4
PR = 2 * DA
GR = D // NG
TB = 256
NB = S // TB
T2 = 256
N2 = S // T2
T2B = 512
LN_EPS = 1e-5
PB = 1024
NPRE = 256
LOG2E = 1.4426950408889634
UNROLL = 4

_NT = (((1,), (1,)), ((), ()))
_INTERLEAVE = [h * DB + c * 64 for c in range(3) for h in range(2)]


def _layernorm(x):
    m = jnp.mean(x, axis=-1, keepdims=True)
    xc = x - m
    v = jnp.mean(xc * xc, axis=-1, keepdims=True)
    return xc * lax.rsqrt(v + LN_EPS)


def _recip(x):
    r = pl.reciprocal(x, approx=True)
    return r * (2.0 - x * r)


def _fold(op, rows):
    r = functools.reduce(op, rows)
    r = op(r, pltpu.roll(r, 4, 0))
    return op(r, pltpu.roll(r, 2, 0))


def _hedgehog(p):
    rows = [p[8 * i:8 * (i + 1), :] for i in range(PR // 8)]
    mx = _fold(jnp.maximum, rows)
    mn = _fold(jnp.minimum, rows)
    ep = [jnp.exp2(r - mx) for r in rows]
    en = [jnp.exp2(mn - r) for r in rows]
    return ep, en, _fold(jnp.add, ep), _fold(jnp.add, en)


def _blockdiag(x):
    t0, t1, t2 = x[:, :128], x[:, 128:256], x[:, 256:]
    lane = lax.broadcasted_iota(jnp.int32, (L, 128), 1)
    z = jnp.zeros((L, 128), f32)
    top = jnp.concatenate([t0, jnp.where(lane < 64, t1, 0.0), z], axis=1)
    bot = jnp.concatenate([z, jnp.where(lane >= 64, t1, 0.0), t2], axis=1)
    return jnp.concatenate([top, bot], axis=0)


def _kernel(x_hbm, wqkv_hbm, wphi_hbm, wo_hbm, mem0_hbm, wqt_hbm, wkt_hbm, wvt_hbm, wob_hbm,
            out_hbm,
            x_ref, wqkv_ref, wphi_ref, wo_ref, mem0_ref, xres_ref, xnb_ref, xna_ref, wt_ref, wp2_ref,
            kvt_ref, o_ref, stage_ref, wob_ref, wo2_ref, wb_ref, pre_ref, mem_ref, sem_a, sem_b, sem_o):
    scale = DB ** -0.5
    XH = 2 * TB
    HT = 128
    CH = HB * DB // N2

    cp_x0 = pltpu.make_async_copy(x_hbm.at[:TB], x_ref.at[:TB], sem_a.at[0])
    cp_k = pltpu.make_async_copy(wqkv_hbm.at[:, D:2 * D], wqkv_ref.at[:, D:2 * D], sem_a.at[1])
    cp_v = pltpu.make_async_copy(wqkv_hbm.at[:, 2 * D:], wqkv_ref.at[:, 2 * D:], sem_a.at[8])
    cp_x0b = pltpu.make_async_copy(x_hbm.at[TB:XH], x_ref.at[TB:XH], sem_a.at[9])
    cp_x1 = pltpu.make_async_copy(x_hbm.at[XH:], x_ref.at[XH:], sem_a.at[2])
    cp_q = pltpu.make_async_copy(wqkv_hbm.at[:, :D], wqkv_ref.at[:, :D], sem_a.at[3])
    cp_wo = pltpu.make_async_copy(wo_hbm, wo_ref, sem_a.at[4])
    cp_wob = pltpu.make_async_copy(wob_hbm, wob_ref, sem_a.at[5])
    cp_phi = pltpu.make_async_copy(wphi_hbm, wphi_ref, sem_a.at[6])
    cp_mem = pltpu.make_async_copy(mem0_hbm, mem0_ref, sem_a.at[7])

    def rows(b, n=TB):
        return pl.ds(b * n if isinstance(b, int) else pl.multiple_of(b * n, n), n)

    def cp_b(m, c):
        src = (wqt_hbm, wkt_hbm, wvt_hbm)[m]
        return pltpu.make_async_copy(src.at[rows(c, CH)], stage_ref.at[c, m * CH:(m + 1) * CH],
                                     sem_b.at[c])

    for c in (cp_phi, cp_x0, cp_k, cp_mem):
        c.start()
    for m in range(3):
        cp_b(m, 0).start(priority=1)

    xres_ref[:HT, :] = jnp.zeros((HT, D), f32)
    cp_phi.wait()
    cp_v.start()
    hrow = lax.broadcasted_iota(jnp.int32, (HA, D), 0)
    hcol = lax.broadcasted_iota(jnp.int32, (HA, D), 1)

    def expand(i, wp):
        for d in (4 * i, 4 * i + 1, 4 * i + 2, 4 * i + 3):
            sel = jnp.where(hcol == hrow * DA + d, 1.0, 0.0)
            wp = wp + jnp.dot(wphi_ref[d].astype(f32), sel, preferred_element_type=f32)
        return wp

    wp = lax.fori_loop(0, DA // 4, expand, jnp.zeros((DA, D), f32))
    dup = jnp.where((lax.broadcasted_iota(jnp.int32, (PR, DA), 0) >> 1)
                    == lax.broadcasted_iota(jnp.int32, (PR, DA), 1), 1.0, 0.0)
    wp2_ref[...] = jnp.dot(dup, wp, preferred_element_type=f32)
    cp_x0.wait()

    def fold_phi(m):
        row = lax.broadcasted_iota(jnp.int32, (PR, 128), 0)
        col = lax.broadcasted_iota(jnp.int32, (PR, 128), 1)
        parts = []
        for t in range(D // 128):
            blocks = []
            for j in range(3 * t, 3 * t + 4):
                lo = (2 * j + (row & 1)) * DA - 128 * t
                blocks.append(jnp.where((col >= lo) & (col < lo + DA),
                                        wp2_ref[:, 128 * t:128 * (t + 1)], 0.0))
            w = wqkv_ref[:, m * D + 128 * t:m * D + 128 * (t + 1)]
            parts.append(lax.dot_general(jnp.concatenate(blocks, axis=0).astype(bf16), w, _NT,
                                         preferred_element_type=f32))
        out = [parts[0][:PR]]
        for t in range(D // 128):
            out.append(parts[t][PR:3 * PR])
            last = parts[t][3 * PR:]
            out.append(last + parts[t + 1][:PR] if t + 1 < D // 128 else last)
        wt_ref[m] = pltpu.bitcast((jnp.concatenate(out, axis=0) * LOG2E).astype(bf16), u32)

    def wt(m, g, dep=None):
        w = wt_ref[m, g * GR // 2:(g + 1) * GR // 2, :]
        if dep is not None:
            never, val = dep
            top = jnp.concatenate([jnp.where(never, val, w[:8, :128]), w[:8, 128:]], axis=1)
            w = jnp.concatenate([top, w[8:]], axis=0)
        return pltpu.bitcast(w, bf16)

    def layer_a(first):
        def ln_a(i):
            xn = _layernorm(x_ref[rows(i, HT), :].astype(f32)).astype(bf16)
            xt = pltpu.bitcast(xn.T, u32)
            xna_ref[i] = xt
            return functools.reduce(jnp.bitwise_or, [xt[64 * t:64 * t + 8] for t in range(D // 128)])

        kvt_ref[...] = jnp.zeros(kvt_ref.shape, f32)
        xn0 = _layernorm(x_ref[:TB, :].astype(f32)).astype(bf16).T
        for i in range(TB // HT):
            xna_ref[i] = pltpu.bitcast(xn0[:, i * HT:(i + 1) * HT], u32)

        @pl.when(first)
        def _():
            cp_x0b.start()
            cp_k.wait()
            cp_v.wait()
            fold_phi(1)
            wt_ref[2] = pltpu.bitcast(wqkv_ref[:, 2 * D:].T, u32)
            cp_x1.start()
            cp_x0b.wait()

        def phase1(b, carry):
            @pl.when(first & (b == XH // TB - 1))
            def _():
                cp_x1.wait()
                cp_q.start()
                cp_wo.start()

            for c in range(1, N2):
                @pl.when(first & (b == (c - 1) * NB // N2))
                def _():
                    for m in range(3):
                        cp_b(m, c).start(priority=1)

            xn = pltpu.bitcast(jnp.concatenate(
                [xna_ref[(TB // HT) * b + i] for i in range(TB // HT)], axis=1), bf16)
            ones = jnp.ones((8, TB), f32)
            pk, v1 = {}, {}

            never = lax.broadcasted_iota(jnp.int32, (8, 128), 0) > b + 64

            def proj_k(g, dep=None):
                pk[g] = jnp.dot(wt(1, g, dep), xn, preferred_element_type=f32)

            def proj_v(g, dep=None):
                v1[g] = jnp.dot(wt(2, g, dep), xn, preferred_element_type=f32)

            def kv(g):
                for j in range(GR // PR):
                    ep, en, sp, sn = _hedgehog(pk[g][j * PR:(j + 1) * PR])
                    rp, rn = _recip(sp), _recip(sn)
                    phik = jnp.concatenate([e * rp for e in ep] + [e * rn for e in en],
                                           axis=0).astype(bf16)
                    lhs = jnp.concatenate([v1[g][j * PR:(j + 1) * PR], ones], axis=0)
                    kvt_ref[g * (GR // PR) + j] += lax.dot_general(
                        lhs, phik, _NT, preferred_element_type=f32)

            nxt = jnp.minimum(b + 1, NB - 1) * (TB // HT)
            dep = [(never, ln_a(nxt + i)) for i in range(TB // HT)]
            proj_k(0); proj_k(1); proj_v(0); proj_k(2); proj_v(1, dep[0]); kv(0)
            proj_k(3); proj_v(2); proj_v(3); kv(1); kv(2); kv(3)
            return carry

        lax.fori_loop(0, NB, phase1, 0)

        @pl.when(first)
        def _():
            cp_q.wait()
            cp_wo.wait()
            fold_phi(0)
            wt_ref[3] = pltpu.bitcast(wo_ref[...], u32)

        rr = lax.broadcasted_iota(jnp.int32, (PR + 8, 2 * PR), 0)
        cc = lax.broadcasted_iota(jnp.int32, (PR + 8, 2 * PR), 1)
        second = ((rr >= DA) & (rr < PR)) | ((rr >= PR) & ((rr & 1) == 1))
        same_head = second == ((cc & 1) == 1)
        for j in range(HA // 2):
            kvt_ref[j] = jnp.where(same_head, kvt_ref[j], 0.0)

        def ln_b(i):
            xn = _layernorm(xres_ref[rows(i, HT), :])
            xnb_ref[rows(i, HT), :] = xn
            return pltpu.bitcast(functools.reduce(
                jnp.add, [xn[8 * t:8 * (t + 1), D - 128:] for t in range(HT // 8)]), u32)

        def phase2(prep, b, carry):
            NH = (T2 if prep else T2B) // HT
            if prep:
                @pl.when(b == N2 // 4)
                def _():
                    cp_wob.start(priority=1)

                for m in range(3):
                    cp_b(m, b).wait()

                for j in range(CH // PW):
                    p = b * (CH // PW) + j
                    for m in range(3):
                        r0 = m * CH + j * PW
                        if m == 2:
                            blk = jnp.concatenate(
                                [stage_ref[b, r0 + r:r0 + r + 64, :] for r in _INTERLEAVE], axis=0)
                        else:
                            blk = stage_ref[b, r0:r0 + PW, :]
                        wb_ref[p, :, m * PW:(m + 1) * PW] = pltpu.bitcast(blk.T, u32)

            never = lax.broadcasted_iota(jnp.int32, (8, 128), 0) > b + 64
            dep = (never, ln_b(jnp.maximum(NH * b - 1, 0)))
            sub = lax.broadcasted_iota(jnp.int32, (8, HT), 0)
            top, even = sub < 4, (sub & 1) == 0
            pq, ot, o, y = {}, {}, {}, {}

            def proj_q(i, g, dep=None):
                xn = pltpu.bitcast(xna_ref[NH * b + i], bf16)
                pq[i, g] = jnp.dot(wt(0, g, dep), xn, preferred_element_type=f32)

            def num(i, g):
                parts = []
                for j in range(GR // PR):
                    ep, en, sp, sn = _hedgehog(pq[i, g][j * PR:(j + 1) * PR])
                    ratio = sp * _recip(sn)
                    phiq = jnp.concatenate(ep + [e * ratio for e in en], axis=0).astype(bf16)
                    n = jnp.dot(kvt_ref[g * (GR // PR) + j], phiq, preferred_element_type=f32)
                    r = _recip(n[PR:, :] + 1e-6 * sp)
                    rs = pltpu.roll(r, 1, 0)
                    ra, rb = jnp.where(even, r, rs), jnp.where(even, rs, r)
                    parts += [n[8 * t:8 * (t + 1), :] * rr_
                              for t, rr_ in enumerate((ra, ra, jnp.where(top, ra, rb), rb, rb))]
                ot[i, g] = jnp.concatenate(parts, axis=0).astype(bf16)

            def out(i, k0, k1, c0=0, c1=D):
                if i not in o:
                    o_ref[i + (b >> 8)] = pltpu.bitcast(
                        jnp.concatenate([ot[i, g] for g in range(NG)], axis=0).T, u32)
                    o[i] = pltpu.bitcast(o_ref[i + (b >> 8)], bf16)
                    y[i] = {}
                if (c0, c1) not in y[i]:
                    y[i][c0, c1] = x_ref[rows(NH * b + i, HT), c0:c1].astype(f32)
                y[i][c0, c1] = y[i][c0, c1] + jnp.dot(
                    o[i][:, k0:k1], pltpu.bitcast(wt_ref[3, k0 // 2:k1 // 2, c0:c1], bf16),
                    preferred_element_type=f32)

            def finish(i, ln):
                xi = jnp.concatenate([y[i][c] for c in sorted(y[i])], axis=1)
                xres_ref[rows(NH * b + i, HT), :] = xi
                if ln:
                    xnb_ref[rows(NH * b + i, HT), :] = _layernorm(xi)

            proj_q(0, 0); proj_q(0, 1); proj_q(0, 2, dep); num(0, 0); proj_q(0, 3); num(0, 1)
            proj_q(1, 0); num(0, 2); proj_q(1, 1); num(0, 3); proj_q(1, 2); num(1, 0)
            proj_q(1, 3); num(1, 1)
            for i in range(2, NH):
                proj_q(i, 0); num(i - 1, 2); proj_q(i, 1); num(i - 1, 3)
                out(i - 2, 0, D); finish(i - 2, True)
                proj_q(i, 2); num(i, 0); proj_q(i, 3); num(i, 1)
            i = NH - 2
            out(i, 0, D, 0, 128); num(i + 1, 2); out(i, 0, D, 128, 256); num(i + 1, 3)
            out(i, 0, D, 256, D); finish(i, True)
            out(i + 1, 0, 384); out(i + 1, 384, D); finish(i + 1, False)
            return carry

        n_prep = jnp.where(first, N2, 0)
        lax.fori_loop(0, n_prep, functools.partial(phase2, True), 0)
        lax.fori_loop(0, jnp.where(first, 0, S // T2B), functools.partial(phase2, False), 0)
        def pre(i, carry):
            w = pltpu.bitcast(wb_ref[NP - 1, :, 3 * PW - NPRE:], bf16)
            pre_ref[rows(i, PB), :] = jnp.dot(xnb_ref[rows(i, PB), :], w, preferred_element_type=f32)
            ln_b(S // HT - 1)
            return carry

        lax.fori_loop(0, S // PB, pre, 0)

        @pl.when(first)
        def _():
            cp_mem.wait()
            cp_wob.wait()

            def pack(p, carry):
                for i, r in enumerate(_INTERLEAVE):
                    src = wob_ref[pl.ds(pl.multiple_of(p * PW + r, 64), 64), :]
                    wo2_ref[p, 32 * i:32 * (i + 1), :] = pltpu.bitcast(src, u32)
                return carry

            lax.fori_loop(0, NP, pack, 0)

    NI = NSEG // UNROLL
    out_at = [0, NI // 4, NI // 2, 3 * NI // 4, NI - 1, NI]

    def out_copy(k):
        r = pl.ds(out_at[k] * UNROLL * SEG, (out_at[k + 1] - out_at[k]) * UNROLL * SEG)
        return pltpu.make_async_copy(x_ref.at[r], out_hbm.at[r], sem_o)

    def layer_b(last):
        mem_ref[...] = mem0_ref[...].astype(f32)
        LM = L - 8
        srow = lax.broadcasted_iota(jnp.int32, (LM, 2 * L), 0)
        scol = lax.broadcasted_iota(jnp.int32, (LM, 2 * L), 1)
        first = scol < L
        kidx = jnp.where(first, scol, scol - L)
        mask = (srow < MEM) | (srow + 8 >= kidx)
        lo40 = lax.broadcasted_iota(jnp.int32, (L, PW), 1) % 128 < 64
        lo8 = lax.broadcasted_iota(jnp.int32, (8, 128), 1) < 64
        sub8 = lax.broadcasted_iota(jnp.int32, (8, 128), 0)
        WIN = 14
        NA = 384

        def softmax(s):
            s = jnp.where(mask, s * scale, -1e9)
            m1 = jnp.max(jnp.where(first, s, -jnp.inf), axis=1, keepdims=True)
            m2 = jnp.max(jnp.where(first, -jnp.inf, s), axis=1, keepdims=True)
            e = jnp.exp(s - jnp.where(first, m1, m2))
            l1 = jnp.sum(jnp.where(first, e, 0.0), axis=1, keepdims=True)
            l2 = jnp.sum(jnp.where(first, 0.0, e), axis=1, keepdims=True)
            return e * _recip(jnp.where(first, l1, l2))

        pre_at = {4: (0, 256), 8: (256, 512), 12: (512, D)}

        def step(s, mem):
            never = sub8 > s + 128

            def rot(x, j, t, dep):
                blk = x[8 * (j // 8):8 * (j // 8) + 8, 128 * t:128 * (t + 1)]
                if dep is not None:
                    blk = jnp.where(never, dep, blk)
                return pltpu.roll(blk, j % 8, 0) if j % 8 else blk

            def vpu_attn(q, k, v):
                qg = q[MEM:MEM + 8] * (scale * LOG2E)
                a0, b2 = qg[:, :128], qg[:, 256:]
                a1 = jnp.where(lo8, qg[:, 128:256], 0.0)
                b1 = jnp.where(lo8, 0.0, qg[:, 128:256])
                raw, cols, p1, p2 = [], [], None, None
                for j in range(MEM + 8):
                    k0, k2 = rot(k, j, 0, p2), rot(k, j, 2, p1)
                    k1 = rot(k, j, 1, raw[j - WIN] if j >= WIN else p2)
                    p1 = a0 * k0 + a1 * k1
                    p2 = b1 * k1 + b2 * k2
                    sc = jnp.where(lo8, jnp.sum(p1, axis=1, keepdims=True),
                                   jnp.sum(p2, axis=1, keepdims=True))
                    raw.append(sc)
                    cols.append(jnp.where(sub8 >= j - MEM, sc, -1e9 * LOG2E) if j > MEM else sc)
                m = functools.reduce(jnp.maximum, cols)
                accs, l = [None] * 3, None
                for j in range(MEM + 8):
                    e = jnp.exp2(cols[j] - m)
                    l = e if j == 0 else l + e
                    for t in range(3):
                        dep = accs[(2, 1, 0)[t]]
                        x = e * rot(v, j, t, e if dep is None else dep)
                        accs[t] = x if j == 0 else accs[t] + x
                rl = _recip(l)
                return jnp.concatenate([x * rl for x in accs], axis=1)

            r = rows(s, SEG)
            h = jnp.concatenate([mem, xnb_ref[r, :]], axis=0)
            qkv, pr, os_, ov, pm = {}, {}, {}, {}, []
            acc = {(0, NA): None, (NA, D): None}
            for c0, c1 in acc:
                acc[c0, c1] = jnp.concatenate(
                    [jnp.zeros((MEM, c1 - c0), f32), xres_ref[r, c0:c1]], axis=0)

            def proj(t):
                w = pltpu.bitcast(wb_ref[t], bf16)
                if t == 0:
                    part = jnp.dot(h[:, :NA], w[:NA], preferred_element_type=f32)
                    part = jnp.concatenate([part[:, :128], part[:, 128:]], axis=1)
                    qkv[t] = part + jnp.dot(h[:, NA:], w[NA:], preferred_element_type=f32)
                elif t == NP - 1:
                    tail = jnp.concatenate([pm[0], pre_ref[r, :]], axis=0)
                    qkv[t] = jnp.concatenate(
                        [jnp.dot(h, w[:, :3 * PW - NPRE], preferred_element_type=f32), tail], axis=1)
                else:
                    qkv[t] = jnp.dot(h, w, preferred_element_type=f32)
                ov[t] = vpu_attn(qkv[t][:, :PW], qkv[t][:, PW:2 * PW], qkv[t][:, 2 * PW:])
                if t in pre_at:
                    k0, k1 = pre_at[t]
                    w = pltpu.bitcast(wb_ref[NP - 1, k0 // 2:k1 // 2, 3 * PW - NPRE:], bf16)
                    y = jnp.dot(mem[:, k0:k1], w, preferred_element_type=f32)
                    pm[:] = [pm[0] + y if pm else jnp.concatenate([y[:, :128], y[:, 128:]], axis=1)]

            def scores(t):
                q, k = qkv[t][:, :PW], qkv[t][:, PW:2 * PW]
                qm = jnp.concatenate([q[:MEM], q[MEM + 8:]], axis=0)
                pr[t] = softmax(lax.dot_general(qm, _blockdiag(k).astype(bf16), _NT,
                                                preferred_element_type=f32))

            def pv(t):
                v = qkv[t][:, 2 * PW:]
                vv = jnp.concatenate([jnp.where(lo40, v, 0.0), jnp.where(lo40, 0.0, v)], axis=0)
                om = jnp.dot(pr[t], vv.astype(bf16), preferred_element_type=f32)
                os_[t] = jnp.concatenate([om[:MEM], ov[t], om[MEM:]], axis=0)

            def oproj(late, p0, p1):
                c0, c1 = (NA, D) if late else (0, NA)
                o = jnp.concatenate([os_[p] for p in range(p0, p1)], axis=1)
                w = pltpu.bitcast(jnp.concatenate(
                    [wo2_ref[p, :, c0:c1] for p in range(p0, p1)], axis=0), bf16)
                acc[c0, c1] = acc[c0, c1] + jnp.dot(o, w, preferred_element_type=f32)

            for t in range(NP):
                proj(t)
                if t >= 1:
                    scores(t - 1)
                if t >= 2:
                    pv(t - 2)
                if t >= 3:
                    oproj(False, t - 3, t - 2)
            oproj(True, 0, 3); scores(NP - 1); oproj(True, 3, 5); pv(NP - 2); oproj(True, 5, 7)
            oproj(False, NP - 3, NP - 2); oproj(True, 7, 9); oproj(False, NP - 2, NP - 1)
            pv(NP - 1); oproj(True, 9, 12); oproj(False, NP - 1, NP); oproj(True, 12, NP)
            y = jnp.concatenate([acc[0, NA], acc[NA, D]], axis=1)
            x_ref[r, :] = y[MEM:].astype(bf16)
            return y[:MEM]

        def steps(i, carry):
            for k in range(len(out_at) - 2):
                @pl.when(last & (i == out_at[k + 1]))
                def _():
                    out_copy(k).start()

            mem_ref[...] = lax.fori_loop(0, UNROLL, lambda u, mem: step(i * UNROLL + u, mem),
                                         mem_ref[...], unroll=True)
            return carry

        lax.fori_loop(0, NI, steps, 0)

    def layer(i, carry):
        layer_a(i == 0)
        layer_b(i == 1)
        return carry

    lax.fori_loop(0, 2, layer, 0)
    out_copy(len(out_at) - 2).start()
    for k in range(len(out_at) - 1):
        out_copy(k).wait()


@functools.partial(jax.jit, static_argnames=("B_seg_len",))
def pallas_interleave_layers__linear_kernel_hedgehog__memory_aug_recurrent_mem_tr__prompt_kernel(
    A_x, A_wqkv, A_w_phi, A_wo, B_x, B_mem0, B_Wq, B_Wk, B_Wv, B_Wo, B_seg_len=SEG,
):
    del B_x
    assert B_seg_len == SEG
    x = A_x.reshape(S, D)
    wp = A_w_phi.transpose(1, 2, 0)
    mem0 = B_mem0.reshape(MEM, D)
    wqt, wkt, wvt = (w.transpose(1, 2, 0).reshape(HB * DB, D) for w in (B_Wq, B_Wk, B_Wv))
    wob = B_Wo.reshape(HB * DB, D)

    hbm = pl.BlockSpec(memory_space=pl.ANY)
    out = pl.pallas_call(
        _kernel,
        out_shape=jax.ShapeDtypeStruct((S, D), bf16),
        in_specs=[hbm] * 9,
        out_specs=hbm,
        scratch_shapes=[
            pltpu.VMEM((S, D), bf16),
            pltpu.VMEM((D, 3 * D), bf16),
            pltpu.VMEM((DA, DA, HA), bf16),
            pltpu.VMEM((D, D), bf16),
            pltpu.VMEM((MEM, D), bf16),
            pltpu.VMEM((S, D), f32),
            pltpu.VMEM((S, D), f32),
            pltpu.VMEM((S // 128, D // 2, 128), u32),
            pltpu.VMEM((4, D // 2, D), u32),
            pltpu.VMEM((PR, D), f32),
            pltpu.VMEM((HA // 2, PR + 8, 2 * PR), f32),
            pltpu.VMEM((T2B // 128, 64, D), u32),
            pltpu.VMEM((N2, 3 * HB * DB // N2, D), bf16),
            pltpu.VMEM((HB * DB, D), bf16),
            pltpu.VMEM((NP, PW // 2, D), u32),
            pltpu.VMEM((NP, D // 2, 3 * PW), u32),
            pltpu.VMEM((S, NPRE), f32),
            pltpu.VMEM((MEM, D), f32),
            pltpu.SemaphoreType.DMA((10,)),
            pltpu.SemaphoreType.DMA((N2,)),
            pltpu.SemaphoreType.DMA,
        ],
        compiler_params=pltpu.CompilerParams(vmem_limit_bytes=110 * 1024 * 1024),
    )(x, A_wqkv, wp, A_wo, mem0, wqt, wkt, wvt, wob)
    return out.reshape(1, S, D)
```

```python
import functools

import jax
import jax.numpy as jnp
from jax import lax
import jax.experimental.pallas as pl
import jax.experimental.pallas.tpu as pltpu

f32 = jnp.float32
bf16 = jnp.bfloat16
u32 = jnp.uint32

S = 2048
D = 640
HA = 32
DA = D // HA
HB = 32
DB = 192
MEM = 8
SEG = 32
L = MEM + SEG
NSEG = S // SEG
NP = HB // 2
PW = 2 * DB
NG = 4
PR = 2 * DA
GR = D // NG
TB = 256
NB = S // TB
T2 = 256
N2 = S // T2
T2B = 512
LN_EPS = 1e-5
PB = 1024
NPRE = 256
LOG2E = 1.4426950408889634
UNROLL = 4

_NT = (((1,), (1,)), ((), ()))
_INTERLEAVE = [h * DB + c * 64 for c in range(3) for h in range(2)]


def _layernorm(x):
    m = jnp.mean(x, axis=-1, keepdims=True)
    xc = x - m
    v = jnp.mean(xc * xc, axis=-1, keepdims=True)
    return xc * lax.rsqrt(v + LN_EPS)


def _recip(x):
    r = pl.reciprocal(x, approx=True)
    return r * (2.0 - x * r)


def _fold(op, rows):
    r = functools.reduce(op, rows)
    r = op(r, pltpu.roll(r, 4, 0))
    return op(r, pltpu.roll(r, 2, 0))


def _hedgehog(p):
    rows = [p[8 * i:8 * (i + 1), :] for i in range(PR // 8)]
    mx = _fold(jnp.maximum, rows)
    mn = _fold(jnp.minimum, rows)
    ep = [jnp.exp2(r - mx) for r in rows]
    en = [jnp.exp2(mn - r) for r in rows]
    return ep, en, _fold(jnp.add, ep), _fold(jnp.add, en)


def _blockdiag(x):
    t0, t1, t2 = x[:, :128], x[:, 128:256], x[:, 256:]
    lane = lax.broadcasted_iota(jnp.int32, (L, 128), 1)
    z = jnp.zeros((L, 128), f32)
    top = jnp.concatenate([t0, jnp.where(lane < 64, t1, 0.0), z], axis=1)
    bot = jnp.concatenate([z, jnp.where(lane >= 64, t1, 0.0), t2], axis=1)
    return jnp.concatenate([top, bot], axis=0)


def _kernel(x_hbm, wqkv_hbm, wphi_hbm, wo_hbm, mem0_hbm, wqt_hbm, wkt_hbm, wvt_hbm, wob_hbm,
            out_hbm,
            x_ref, wqkv_ref, wphi_ref, wo_ref, mem0_ref, xres_ref, xnb_ref, xna_ref, wt_ref, wp2_ref,
            kvt_ref, o_ref, stage_ref, wob_ref, wo2_ref, wb_ref, pre_ref, mem_ref, sem_a, sem_b, sem_o):
    scale = DB ** -0.5
    XH = 2 * TB
    HT = 128
    CH = HB * DB // N2

    cp_x0 = pltpu.make_async_copy(x_hbm.at[:TB], x_ref.at[:TB], sem_a.at[0])
    cp_k = pltpu.make_async_copy(wqkv_hbm.at[:, D:2 * D], wqkv_ref.at[:, D:2 * D], sem_a.at[1])
    cp_v = pltpu.make_async_copy(wqkv_hbm.at[:, 2 * D:], wqkv_ref.at[:, 2 * D:], sem_a.at[8])
    cp_x0b = pltpu.make_async_copy(x_hbm.at[TB:XH], x_ref.at[TB:XH], sem_a.at[9])
    cp_x1 = pltpu.make_async_copy(x_hbm.at[XH:], x_ref.at[XH:], sem_a.at[2])
    cp_q = pltpu.make_async_copy(wqkv_hbm.at[:, :D], wqkv_ref.at[:, :D], sem_a.at[3])
    cp_wo = pltpu.make_async_copy(wo_hbm, wo_ref, sem_a.at[4])
    cp_wob = pltpu.make_async_copy(wob_hbm, wob_ref, sem_a.at[5])
    cp_phi = pltpu.make_async_copy(wphi_hbm, wphi_ref, sem_a.at[6])
    cp_mem = pltpu.make_async_copy(mem0_hbm, mem0_ref, sem_a.at[7])

    def rows(b, n=TB):
        return pl.ds(b * n if isinstance(b, int) else pl.multiple_of(b * n, n), n)

    def cp_b(m, c):
        src = (wqt_hbm, wkt_hbm, wvt_hbm)[m]
        return pltpu.make_async_copy(src.at[rows(c, CH)], stage_ref.at[c, m * CH:(m + 1) * CH],
                                     sem_b.at[c])

    for c in (cp_phi, cp_x0, cp_k, cp_mem):
        c.start()
    for m in range(3):
        cp_b(m, 0).start(priority=1)

    xres_ref[:HT, :] = jnp.zeros((HT, D), f32)
    cp_phi.wait()
    cp_v.start()
    hrow = lax.broadcasted_iota(jnp.int32, (HA, D), 0)
    hcol = lax.broadcasted_iota(jnp.int32, (HA, D), 1)

    def expand(i, wp):
        for d in (4 * i, 4 * i + 1, 4 * i + 2, 4 * i + 3):
            sel = jnp.where(hcol == hrow * DA + d, 1.0, 0.0)
            wp = wp + jnp.dot(wphi_ref[d].astype(f32), sel, preferred_element_type=f32)
        return wp

    wp = lax.fori_loop(0, DA // 4, expand, jnp.zeros((DA, D), f32))
    dup = jnp.where((lax.broadcasted_iota(jnp.int32, (PR, DA), 0) >> 1)
                    == lax.broadcasted_iota(jnp.int32, (PR, DA), 1), 1.0, 0.0)
    wp2_ref[...] = jnp.dot(dup, wp, preferred_element_type=f32)
    cp_x0.wait()

    def fold_phi(m):
        row = lax.broadcasted_iota(jnp.int32, (PR, 128), 0)
        col = lax.broadcasted_iota(jnp.int32, (PR, 128), 1)
        parts = []
        for t in range(D // 128):
            blocks = []
            for j in range(3 * t, 3 * t + 4):
                lo = (2 * j + (row & 1)) * DA - 128 * t
                blocks.append(jnp.where((col >= lo) & (col < lo + DA),
                                        wp2_ref[:, 128 * t:128 * (t + 1)], 0.0))
            w = wqkv_ref[:, m * D + 128 * t:m * D + 128 * (t + 1)]
            parts.append(lax.dot_general(jnp.concatenate(blocks, axis=0).astype(bf16), w, _NT,
                                         preferred_element_type=f32))
        out = [parts[0][:PR]]
        for t in range(D // 128):
            out.append(parts[t][PR:3 * PR])
            last = parts[t][3 * PR:]
            out.append(last + parts[t + 1][:PR] if t + 1 < D // 128 else last)
        wt_ref[m] = pltpu.bitcast((jnp.concatenate(out, axis=0) * LOG2E).astype(bf16), u32)

    def wt(m, g, dep=None):
        w = wt_ref[m, g * GR // 2:(g + 1) * GR // 2, :]
        if dep is not None:
            never, val = dep
            top = jnp.concatenate([jnp.where(never, val, w[:8, :128]), w[:8, 128:]], axis=1)
            w = jnp.concatenate([top, w[8:]], axis=0)
        return pltpu.bitcast(w, bf16)

    def layer_a(first):
        def ln_a(i):
            xn = _layernorm(x_ref[rows(i, HT), :].astype(f32)).astype(bf16)
            xt = pltpu.bitcast(xn.T, u32)
            xna_ref[i] = xt
            return functools.reduce(jnp.bitwise_or, [xt[64 * t:64 * t + 8] for t in range(D // 128)])

        kvt_ref[...] = jnp.zeros(kvt_ref.shape, f32)
        xn0 = _layernorm(x_ref[:TB, :].astype(f32)).astype(bf16).T
        for i in range(TB // HT):
            xna_ref[i] = pltpu.bitcast(xn0[:, i * HT:(i + 1) * HT], u32)

        @pl.when(first)
        def _():
            cp_x0b.start()
            cp_k.wait()
            cp_v.wait()
            fold_phi(1)
            wt_ref[2] = pltpu.bitcast(wqkv_ref[:, 2 * D:].T, u32)
            cp_x1.start()
            cp_x0b.wait()

        def phase1(b, carry):
            @pl.when(first & (b == XH // TB - 1))
            def _():
                cp_x1.wait()
                cp_q.start()
                cp_wo.start()

            for c in range(1, N2):
                @pl.when(first & (b == (c - 1) * NB // N2))
                def _():
                    for m in range(3):
                        cp_b(m, c).start(priority=1)

            xn = pltpu.bitcast(jnp.concatenate(
                [xna_ref[(TB // HT) * b + i] for i in range(TB // HT)], axis=1), bf16)
            ones = jnp.ones((8, TB), f32)
            pk, v1 = {}, {}

            never = lax.broadcasted_iota(jnp.int32, (8, 128), 0) > b + 64

            def proj_k(g, dep=None):
                pk[g] = jnp.dot(wt(1, g, dep), xn, preferred_element_type=f32)

            def proj_v(g, dep=None):
                v1[g] = jnp.dot(wt(2, g, dep), xn, preferred_element_type=f32)

            def kv(g):
                for j in range(GR // PR):
                    ep, en, sp, sn = _hedgehog(pk[g][j * PR:(j + 1) * PR])
                    rp, rn = _recip(sp), _recip(sn)
                    phik = jnp.concatenate([e * rp for e in ep] + [e * rn for e in en],
                                           axis=0).astype(bf16)
                    lhs = jnp.concatenate([v1[g][j * PR:(j + 1) * PR], ones], axis=0)
                    kvt_ref[g * (GR // PR) + j] += lax.dot_general(
                        lhs, phik, _NT, preferred_element_type=f32)

            nxt = jnp.minimum(b + 1, NB - 1) * (TB // HT)
            dep = [(never, ln_a(nxt + i)) for i in range(TB // HT)]
            proj_k(0); proj_k(1); proj_v(0); proj_k(2); proj_v(1, dep[0]); kv(0)
            proj_k(3); proj_v(2); proj_v(3); kv(1); kv(2); kv(3)
            return carry

        lax.fori_loop(0, NB, phase1, 0)

        @pl.when(first)
        def _():
            cp_q.wait()
            cp_wo.wait()
            fold_phi(0)
            wt_ref[3] = pltpu.bitcast(wo_ref[...], u32)

        rr = lax.broadcasted_iota(jnp.int32, (PR + 8, 2 * PR), 0)
        cc = lax.broadcasted_iota(jnp.int32, (PR + 8, 2 * PR), 1)
        second = ((rr >= DA) & (rr < PR)) | ((rr >= PR) & ((rr & 1) == 1))
        same_head = second == ((cc & 1) == 1)
        for j in range(HA // 2):
            kvt_ref[j] = jnp.where(same_head, kvt_ref[j], 0.0)

        def ln_b(i):
            xn = _layernorm(xres_ref[rows(i, HT), :])
            xnb_ref[rows(i, HT), :] = xn
            return pltpu.bitcast(functools.reduce(
                jnp.add, [xn[8 * t:8 * (t + 1), D - 128:] for t in range(HT // 8)]), u32)

        def phase2(prep, b, carry):
            NH = (T2 if prep else T2B) // HT
            if prep:
                @pl.when(b == N2 // 4)
                def _():
                    cp_wob.start(priority=1)

                for m in range(3):
                    cp_b(m, b).wait()

                for j in range(CH // PW):
                    p = b * (CH // PW) + j
                    for m in range(3):
                        r0 = m * CH + j * PW
                        if m == 2:
                            blk = jnp.concatenate(
                                [stage_ref[b, r0 + r:r0 + r + 64, :] for r in _INTERLEAVE], axis=0)
                        else:
                            blk = stage_ref[b, r0:r0 + PW, :]
                        wb_ref[p, :, m * PW:(m + 1) * PW] = pltpu.bitcast(blk.T, u32)

            never = lax.broadcasted_iota(jnp.int32, (8, 128), 0) > b + 64
            dep = (never, ln_b(jnp.maximum(NH * b - 1, 0)))
            sub = lax.broadcasted_iota(jnp.int32, (8, HT), 0)
            top, even = sub < 4, (sub & 1) == 0
            pq, ot, o, y = {}, {}, {}, {}

            def proj_q(i, g, dep=None):
                xn = pltpu.bitcast(xna_ref[NH * b + i], bf16)
                pq[i, g] = jnp.dot(wt(0, g, dep), xn, preferred_element_type=f32)

            def num(i, g):
                parts = []
                for j in range(GR // PR):
                    ep, en, sp, sn = _hedgehog(pq[i, g][j * PR:(j + 1) * PR])
                    ratio = sp * _recip(sn)
                    phiq = jnp.concatenate(ep + [e * ratio for e in en], axis=0).astype(bf16)
                    n = jnp.dot(kvt_ref[g * (GR // PR) + j], phiq, preferred_element_type=f32)
                    r = _recip(n[PR:, :] + 1e-6 * sp)
                    rs = pltpu.roll(r, 1, 0)
                    ra, rb = jnp.where(even, r, rs), jnp.where(even, rs, r)
                    parts += [n[8 * t:8 * (t + 1), :] * rr_
                              for t, rr_ in enumerate((ra, ra, jnp.where(top, ra, rb), rb, rb))]
                ot[i, g] = jnp.concatenate(parts, axis=0).astype(bf16)

            def out(i, k0, k1, c0=0, c1=D):
                if i not in o:
                    o_ref[i + (b >> 8)] = pltpu.bitcast(
                        jnp.concatenate([ot[i, g] for g in range(NG)], axis=0).T, u32)
                    o[i] = pltpu.bitcast(o_ref[i + (b >> 8)], bf16)
                    y[i] = {}
                if (c0, c1) not in y[i]:
                    y[i][c0, c1] = x_ref[rows(NH * b + i, HT), c0:c1].astype(f32)
                y[i][c0, c1] = y[i][c0, c1] + jnp.dot(
                    o[i][:, k0:k1], pltpu.bitcast(wt_ref[3, k0 // 2:k1 // 2, c0:c1], bf16),
                    preferred_element_type=f32)

            def finish(i, ln):
                xi = jnp.concatenate([y[i][c] for c in sorted(y[i])], axis=1)
                xres_ref[rows(NH * b + i, HT), :] = xi
                if ln:
                    xnb_ref[rows(NH * b + i, HT), :] = _layernorm(xi)

            proj_q(0, 0); proj_q(0, 1); proj_q(0, 2, dep); num(0, 0); proj_q(0, 3); num(0, 1)
            proj_q(1, 0); num(0, 2); proj_q(1, 1); num(0, 3); proj_q(1, 2); num(1, 0)
            proj_q(1, 3); num(1, 1)
            for i in range(2, NH):
                proj_q(i, 0); num(i - 1, 2); proj_q(i, 1); num(i - 1, 3)
                out(i - 2, 0, D); finish(i - 2, True)
                proj_q(i, 2); num(i, 0); proj_q(i, 3); num(i, 1)
            i = NH - 2
            out(i, 0, D, 0, 128); num(i + 1, 2); out(i, 0, D, 128, 256); num(i + 1, 3)
            out(i, 0, D, 256, D); finish(i, True)
            out(i + 1, 0, 384); out(i + 1, 384, D); finish(i + 1, False)
            return carry

        n_prep = jnp.where(first, N2, 0)
        lax.fori_loop(0, n_prep, functools.partial(phase2, True), 0)
        lax.fori_loop(0, jnp.where(first, 0, S // T2B), functools.partial(phase2, False), 0)

        def pre(i, carry):
            w = pltpu.bitcast(wb_ref[NP - 1, :, 3 * PW - NPRE:], bf16)
            pre_ref[rows(i, PB), :] = jnp.dot(xnb_ref[rows(i, PB), :], w, preferred_element_type=f32)
            ln_b(S // HT - 1)
            return carry

        lax.fori_loop(0, S // PB, pre, 0)

        @pl.when(first)
        def _():
            cp_mem.wait()
            cp_wob.wait()

            def pack(p, carry):
                for i, r in enumerate(_INTERLEAVE):
                    src = wob_ref[pl.ds(pl.multiple_of(p * PW + r, 64), 64), :]
                    wo2_ref[p, 32 * i:32 * (i + 1), :] = pltpu.bitcast(src, u32)
                return carry

            lax.fori_loop(0, NP, pack, 0)

    NI = NSEG // UNROLL
    out_at = [0, NI // 4, NI // 2, 3 * NI // 4, NI - 1, NI]

    def out_copy(k):
        r = pl.ds(out_at[k] * UNROLL * SEG, (out_at[k + 1] - out_at[k]) * UNROLL * SEG)
        return pltpu.make_async_copy(x_ref.at[r], out_hbm.at[r], sem_o)

    def layer_b(last):
        mem_ref[...] = mem0_ref[...].astype(f32)
        LM = L - 8
        srow = lax.broadcasted_iota(jnp.int32, (LM, 2 * L), 0)
        scol = lax.broadcasted_iota(jnp.int32, (LM, 2 * L), 1)
        first = scol < L
        kidx = jnp.where(first, scol, scol - L)
        mask = (srow < MEM) | (srow + 8 >= kidx)
        lo40 = lax.broadcasted_iota(jnp.int32, (L, PW), 1) % 128 < 64
        lo32 = lax.broadcasted_iota(jnp.int32, (LM, 128), 1) < 64
        lo8 = lax.broadcasted_iota(jnp.int32, (8, 128), 1) < 64
        sub8 = lax.broadcasted_iota(jnp.int32, (8, 128), 0)
        never = sub8 > last.astype(jnp.int32) + 128
        WIN = 14
        NA = 384

        def softmax(s):
            s = jnp.where(mask, s * scale, -1e9)
            m1 = jnp.max(jnp.where(first, s, -jnp.inf), axis=1, keepdims=True)
            m2 = jnp.max(jnp.where(first, -jnp.inf, s), axis=1, keepdims=True)
            e = jnp.exp(s - jnp.where(first, m1, m2))
            l1 = jnp.sum(jnp.where(first, e, 0.0), axis=1, keepdims=True)
            l2 = jnp.sum(jnp.where(first, 0.0, e), axis=1, keepdims=True)
            return e, _recip(jnp.where(lo32, l1, l2))

        pre_at = {0: (0, 256), 1: (256, 512), 2: (512, D)}

        def step(s, mem):
            def rot(x, j, t, dep):
                blk = x[8 * (j // 8):8 * (j // 8) + 8, 128 * t:128 * (t + 1)]
                if dep is not None:
                    blk = jnp.where(never, dep, blk)
                return pltpu.roll(blk, j % 8, 0) if j % 8 else blk

            def vpu_attn(q, k, v):
                qg = q[MEM:MEM + 8] * (scale * LOG2E)
                a0, b2 = qg[:, :128], qg[:, 256:]
                a1 = jnp.where(lo8, qg[:, 128:256], 0.0)
                b1 = jnp.where(lo8, 0.0, qg[:, 128:256])
                raw, cols, p1, p2 = [], [], None, None
                for j in range(MEM + 8):
                    k0, k2 = rot(k, j, 0, p2), rot(k, j, 2, p1)
                    k1 = rot(k, j, 1, raw[j - WIN] if j >= WIN else p2)
                    p1 = a0 * k0 + a1 * k1
                    p2 = b1 * k1 + b2 * k2
                    sc = jnp.where(lo8, jnp.sum(p1, axis=1, keepdims=True),
                                   jnp.sum(p2, axis=1, keepdims=True))
                    raw.append(sc)
                    cols.append(jnp.where(sub8 >= j - MEM, sc, -1e9 * LOG2E) if j > MEM else sc)
                m = functools.reduce(jnp.maximum, cols)
                accs, l = [None] * 3, None
                for j in range(MEM + 8):
                    e = jnp.exp2(cols[j] - m)
                    l = e if j == 0 else l + e
                    for t in range(3):
                        dep = accs[(2, 1, 0)[t]]
                        x = e * rot(v, j, t, e if dep is None else dep)
                        accs[t] = x if j == 0 else accs[t] + x
                rl = _recip(l)
                return jnp.concatenate([x * rl for x in accs], axis=1)

            r = rows(s, SEG)
            h = jnp.concatenate([mem, xnb_ref[r, :]], axis=0)
            qkv, pr, os_, ov, pm = {}, {}, {}, {}, []
            acc = {(0, NA): None, (NA, D): None}
            for c0, c1 in acc:
                acc[c0, c1] = jnp.concatenate(
                    [jnp.zeros((MEM, c1 - c0), f32), xres_ref[r, c0:c1]], axis=0)

            def proj(t):
                w = pltpu.bitcast(wb_ref[t], bf16)
                if t == 0:
                    part = jnp.dot(h[:, :NA], w[:NA], preferred_element_type=f32)
                    part = jnp.concatenate([part[:, :128], part[:, 128:]], axis=1)
                    qkv[t] = part + jnp.dot(h[:, NA:], w[NA:], preferred_element_type=f32)
                elif t == NP - 1:
                    tail = jnp.concatenate([pm[0], pre_ref[r, :]], axis=0)
                    qkv[t] = jnp.concatenate(
                        [jnp.dot(h, w[:, :3 * PW - NPRE], preferred_element_type=f32), tail], axis=1)
                else:
                    qkv[t] = jnp.dot(h, w, preferred_element_type=f32)
                ov[t] = vpu_attn(qkv[t][:, :PW], qkv[t][:, PW:2 * PW], qkv[t][:, 2 * PW:])
                if t in pre_at:
                    k0, k1 = pre_at[t]
                    w = pltpu.bitcast(wb_ref[NP - 1, k0 // 2:k1 // 2, 3 * PW - NPRE:], bf16)
                    y = jnp.dot(mem[:, k0:k1], w, preferred_element_type=f32)
                    pm[:] = [pm[0] + y if pm else jnp.concatenate([y[:, :128], y[:, 128:]], axis=1)]

            def scores(t):
                q, k = qkv[t][:, :PW], qkv[t][:, PW:2 * PW]
                qm = jnp.concatenate([q[:MEM], q[MEM + 8:]], axis=0)
                pr[t] = softmax(lax.dot_general(qm, _blockdiag(k).astype(bf16), _NT,
                                                preferred_element_type=f32))

            def pv(t):
                v = qkv[t][:, 2 * PW:]
                vv = jnp.concatenate([jnp.where(lo40, v, 0.0), jnp.where(lo40, 0.0, v)], axis=0)
                e, rl = pr[t]
                om = jnp.dot(e, vv.astype(bf16), preferred_element_type=f32)
                om = om * jnp.concatenate([rl] * 3, axis=1)
                os_[t] = jnp.concatenate([om[:MEM], ov[t], om[MEM:]], axis=0)

            def oproj(late, p0, p1):
                c0, c1 = (NA, D) if late else (0, NA)
                o = jnp.concatenate([os_[p] for p in range(p0, p1)], axis=1)
                w = pltpu.bitcast(jnp.concatenate(
                    [wo2_ref[p, :, c0:c1] for p in range(p0, p1)], axis=0), bf16)
                acc[c0, c1] = acc[c0, c1] + jnp.dot(o, w, preferred_element_type=f32)

            for t in range(NP):
                proj(t)
                if t >= 1:
                    scores(t - 1)
                if t >= 2:
                    pv(t - 2)
                if t >= 3:
                    oproj(False, t - 3, t - 2)
            oproj(True, 0, 3); scores(NP - 1); oproj(True, 3, 5); pv(NP - 2); oproj(True, 5, 7)
            oproj(False, NP - 3, NP - 2); oproj(True, 7, 9); oproj(False, NP - 2, NP - 1)
            pv(NP - 1); oproj(True, 9, 12); oproj(False, NP - 1, NP); oproj(True, 12, NP)
            y = jnp.concatenate([acc[0, NA], acc[NA, D]], axis=1)
            x_ref[r, :] = y[MEM:].astype(bf16)
            return y[:MEM]

        def steps(i, carry):
            for k in range(len(out_at) - 2):
                @pl.when(last & (i == out_at[k + 1]))
                def _():
                    out_copy(k).start()

            mem_ref[...] = lax.fori_loop(0, UNROLL, lambda u, mem: step(i * UNROLL + u, mem),
                                         mem_ref[...], unroll=True)
            return carry

        lax.fori_loop(0, NI, steps, 0)

    def layer(i, carry):
        layer_a(i == 0)
        layer_b(i == 1)
        return carry

    lax.fori_loop(0, 2, layer, 0)
    out_copy(len(out_at) - 2).start()
    for k in range(len(out_at) - 1):
        out_copy(k).wait()


@jax.jit
def pallas_interleave_layers__linear_kernel_hedgehog__memory_aug_recurrent_mem_tr__prompt_kernel(
    A_x, A_wqkv, A_w_phi, A_wo, B_x, B_mem0, B_Wq, B_Wk, B_Wv, B_Wo, B_seg_len=SEG,
):
    del B_x
    del B_seg_len
    x = A_x.reshape(S, D)
    wp = A_w_phi.transpose(1, 2, 0)
    mem0 = B_mem0.reshape(MEM, D)
    wqt, wkt, wvt = (w.transpose(1, 2, 0).reshape(HB * DB, D) for w in (B_Wq, B_Wk, B_Wv))
    wob = B_Wo.reshape(HB * DB, D)

    hbm = pl.BlockSpec(memory_space=pl.ANY)
    out = pl.pallas_call(
        _kernel,
        out_shape=jax.ShapeDtypeStruct((S, D), bf16),
        in_specs=[hbm] * 9,
        out_specs=hbm,
        scratch_shapes=[
            pltpu.VMEM((S, D), bf16),
            pltpu.VMEM((D, 3 * D), bf16),
            pltpu.VMEM((DA, DA, HA), bf16),
            pltpu.VMEM((D, D), bf16),
            pltpu.VMEM((MEM, D), bf16),
            pltpu.VMEM((S, D), f32),
            pltpu.VMEM((S, D), f32),
            pltpu.VMEM((S // 128, D // 2, 128), u32),
            pltpu.VMEM((4, D // 2, D), u32),
            pltpu.VMEM((PR, D), f32),
            pltpu.VMEM((HA // 2, PR + 8, 2 * PR), f32),
            pltpu.VMEM((T2B // 128, 64, D), u32),
            pltpu.VMEM((N2, 3 * HB * DB // N2, D), bf16),
            pltpu.VMEM((HB * DB, D), bf16),
            pltpu.VMEM((NP, PW // 2, D), u32),
            pltpu.VMEM((NP, D // 2, 3 * PW), u32),
            pltpu.VMEM((S, NPRE), f32),
            pltpu.VMEM((MEM, D), f32),
            pltpu.SemaphoreType.DMA((10,)),
            pltpu.SemaphoreType.DMA((N2,)),
            pltpu.SemaphoreType.DMA,
        ],
        compiler_params=pltpu.CompilerParams(vmem_limit_bytes=110 * 1024 * 1024),
    )(x, A_wqkv, wp, A_wo, mem0, wqt, wkt, wvt, wob)
    return out.reshape(1, S, D)
```

```python
import functools

import jax
import jax.numpy as jnp
from jax import lax
import jax.experimental.pallas as pl
import jax.experimental.pallas.tpu as pltpu

f32 = jnp.float32
bf16 = jnp.bfloat16
u32 = jnp.uint32

S = 2048
D = 640
HA = 32
DA = D // HA
HB = 32
DB = 192
MEM = 8
SEG = 32
L = MEM + SEG
NSEG = S // SEG
NP = HB // 2
PW = 2 * DB
NG = 4
PR = 2 * DA
GR = D // NG
TB = 256
NB = S // TB
T2 = 256
N2 = S // T2
T2B = 512
LN_EPS = 1e-5
PB = 1024
NPRE = 256
LOG2E = 1.4426950408889634
UNROLL = 4

_NT = (((1,), (1,)), ((), ()))
_INTERLEAVE = [h * DB + c * 64 for c in range(3) for h in range(2)]


def _layernorm(x):
    m = jnp.mean(x, axis=-1, keepdims=True)
    xc = x - m
    v = jnp.mean(xc * xc, axis=-1, keepdims=True)
    return xc * lax.rsqrt(v + LN_EPS)


def _recip(x):
    r = pl.reciprocal(x, approx=True)
    return r * (2.0 - x * r)


def _fold(op, rows):
    r = functools.reduce(op, rows)
    r = op(r, pltpu.roll(r, 4, 0))
    return op(r, pltpu.roll(r, 2, 0))


def _hedgehog(p):
    rows = [p[8 * i:8 * (i + 1), :] for i in range(PR // 8)]
    mx = _fold(jnp.maximum, rows)
    mn = _fold(jnp.minimum, rows)
    ep = [jnp.exp2(r - mx) for r in rows]
    en = [jnp.exp2(mn - r) for r in rows]
    return ep, en, _fold(jnp.add, ep), _fold(jnp.add, en)


def _blockdiag(x):
    t0, t1, t2 = x[:, :128], x[:, 128:256], x[:, 256:]
    lane = lax.broadcasted_iota(jnp.int32, (L, 128), 1)
    z = jnp.zeros((L, 128), f32)
    top = jnp.concatenate([t0, jnp.where(lane < 64, t1, 0.0), z], axis=1)
    bot = jnp.concatenate([z, jnp.where(lane >= 64, t1, 0.0), t2], axis=1)
    return jnp.concatenate([top, bot], axis=0)


def _kernel(x_hbm, wqkv_hbm, wphi_hbm, wo_hbm, mem0_hbm, wqt_hbm, wkt_hbm, wvt_hbm, wob_hbm,
            out_hbm,
            x_ref, wqkv_ref, wphi_ref, wo_ref, mem0_ref, xres_ref, xnb_ref, xna_ref, wt_ref, wp2_ref,
            kvt_ref, o_ref, stage_ref, wob_ref, wo2_ref, wb_ref, pre_ref, mem_ref, sem_a, sem_b, sem_o):
    scale = DB ** -0.5
    XH = 2 * TB
    HT = 128
    CH = HB * DB // N2

    cp_x0 = pltpu.make_async_copy(x_hbm.at[:TB], x_ref.at[:TB], sem_a.at[0])
    cp_k = pltpu.make_async_copy(wqkv_hbm.at[:, D:2 * D], wqkv_ref.at[:, D:2 * D], sem_a.at[1])
    cp_v = pltpu.make_async_copy(wqkv_hbm.at[:, 2 * D:], wqkv_ref.at[:, 2 * D:], sem_a.at[8])
    cp_x0b = pltpu.make_async_copy(x_hbm.at[TB:XH], x_ref.at[TB:XH], sem_a.at[9])
    cp_x1 = pltpu.make_async_copy(x_hbm.at[XH:], x_ref.at[XH:], sem_a.at[2])
    cp_q = pltpu.make_async_copy(wqkv_hbm.at[:, :D], wqkv_ref.at[:, :D], sem_a.at[3])
    cp_wo = pltpu.make_async_copy(wo_hbm, wo_ref, sem_a.at[4])
    cp_wob = pltpu.make_async_copy(wob_hbm, wob_ref, sem_a.at[5])
    cp_phi = pltpu.make_async_copy(wphi_hbm, wphi_ref, sem_a.at[6])
    cp_mem = pltpu.make_async_copy(mem0_hbm, mem0_ref, sem_a.at[7])

    def rows(b, n=TB):
        return pl.ds(b * n if isinstance(b, int) else pl.multiple_of(b * n, n), n)

    def cp_b(m, c):
        src = (wqt_hbm, wkt_hbm, wvt_hbm)[m]
        return pltpu.make_async_copy(src.at[rows(c, CH)], stage_ref.at[c, m * CH:(m + 1) * CH],
                                     sem_b.at[c])

    for c in (cp_phi, cp_x0, cp_k, cp_mem):
        c.start()
    for m in range(3):
        cp_b(m, 0).start(priority=1)

    xres_ref[:HT, :] = jnp.zeros((HT, D), f32)
    cp_phi.wait()
    cp_v.start()
    hrow = lax.broadcasted_iota(jnp.int32, (HA, D), 0)
    hcol = lax.broadcasted_iota(jnp.int32, (HA, D), 1)

    def expand(i, wp):
        for d in (4 * i, 4 * i + 1, 4 * i + 2, 4 * i + 3):
            sel = jnp.where(hcol == hrow * DA + d, 1.0, 0.0)
            wp = wp + jnp.dot(wphi_ref[d].astype(f32), sel, preferred_element_type=f32)
        return wp

    wp = lax.fori_loop(0, DA // 4, expand, jnp.zeros((DA, D), f32))
    dup = jnp.where((lax.broadcasted_iota(jnp.int32, (PR, DA), 0) >> 1)
                    == lax.broadcasted_iota(jnp.int32, (PR, DA), 1), 1.0, 0.0)
    wp2_ref[...] = jnp.dot(dup, wp, preferred_element_type=f32)
    cp_x0.wait()

    def fold_phi(m):
        row = lax.broadcasted_iota(jnp.int32, (PR, 128), 0)
        col = lax.broadcasted_iota(jnp.int32, (PR, 128), 1)
        parts = []
        for t in range(D // 128):
            blocks = []
            for j in range(3 * t, 3 * t + 4):
                lo = (2 * j + (row & 1)) * DA - 128 * t
                blocks.append(jnp.where((col >= lo) & (col < lo + DA),
                                        wp2_ref[:, 128 * t:128 * (t + 1)], 0.0))
            w = wqkv_ref[:, m * D + 128 * t:m * D + 128 * (t + 1)]
            parts.append(lax.dot_general(jnp.concatenate(blocks, axis=0).astype(bf16), w, _NT,
                                         preferred_element_type=f32))
        out = [parts[0][:PR]]
        for t in range(D // 128):
            out.append(parts[t][PR:3 * PR])
            last = parts[t][3 * PR:]
            out.append(last + parts[t + 1][:PR] if t + 1 < D // 128 else last)
        wt_ref[m] = pltpu.bitcast((jnp.concatenate(out, axis=0) * LOG2E).astype(bf16), u32)

    def wt(m, g, dep=None):
        w = wt_ref[m, g * GR // 2:(g + 1) * GR // 2, :]
        if dep is not None:
            never, val = dep
            top = jnp.concatenate([jnp.where(never, val, w[:8, :128]), w[:8, 128:]], axis=1)
            w = jnp.concatenate([top, w[8:]], axis=0)
        return pltpu.bitcast(w, bf16)

    def layer_a(first):
        def ln_a(i):
            xn = _layernorm(x_ref[rows(i, HT), :].astype(f32)).astype(bf16)
            xt = pltpu.bitcast(xn.T, u32)
            xna_ref[i] = xt
            return functools.reduce(jnp.bitwise_or, [xt[64 * t:64 * t + 8] for t in range(D // 128)])

        kvt_ref[...] = jnp.zeros(kvt_ref.shape, f32)
        xn0 = _layernorm(x_ref[:TB, :].astype(f32)).astype(bf16).T
        for i in range(TB // HT):
            xna_ref[i] = pltpu.bitcast(xn0[:, i * HT:(i + 1) * HT], u32)

        @pl.when(first)
        def _():
            cp_x0b.start()
            cp_k.wait()
            cp_v.wait()
            fold_phi(1)
            wt_ref[2] = pltpu.bitcast(wqkv_ref[:, 2 * D:].T, u32)
            cp_x1.start()
            cp_x0b.wait()

        def phase1(b, carry):
            @pl.when(first & (b == XH // TB - 1))
            def _():
                cp_x1.wait()
                cp_q.start()
                cp_wo.start()

            for c in range(1, N2):
                @pl.when(first & (b == (c - 1) * NB // N2))
                def _():
                    for m in range(3):
                        cp_b(m, c).start(priority=1)

            xn = pltpu.bitcast(jnp.concatenate(
                [xna_ref[(TB // HT) * b + i] for i in range(TB // HT)], axis=1), bf16)
            ones = jnp.ones((8, TB), f32)
            pk, v1 = {}, {}

            never = lax.broadcasted_iota(jnp.int32, (8, 128), 0) > b + 64

            def proj_k(g, dep=None):
                pk[g] = jnp.dot(wt(1, g, dep), xn, preferred_element_type=f32)

            def proj_v(g, dep=None):
                v1[g] = jnp.dot(wt(2, g, dep), xn, preferred_element_type=f32)

            def kv(g):
                for j in range(GR // PR):
                    ep, en, sp, sn = _hedgehog(pk[g][j * PR:(j + 1) * PR])
                    rp, rn = _recip(sp), _recip(sn)
                    phik = jnp.concatenate([e * rp for e in ep] + [e * rn for e in en],
                                           axis=0).astype(bf16)
                    lhs = jnp.concatenate([v1[g][j * PR:(j + 1) * PR], ones], axis=0)
                    kvt_ref[g * (GR // PR) + j] += lax.dot_general(
                        lhs, phik, _NT, preferred_element_type=f32)

            nxt = jnp.minimum(b + 1, NB - 1) * (TB // HT)
            dep = [(never, ln_a(nxt + i)) for i in range(TB // HT)]
            proj_k(0); proj_k(1); proj_v(0); proj_k(2); proj_v(1, dep[0]); kv(0)
            proj_k(3); proj_v(2); proj_v(3); kv(1); kv(2); kv(3)
            return carry

        lax.fori_loop(0, NB, phase1, 0)

        @pl.when(first)
        def _():
            cp_q.wait()
            cp_wo.wait()
            fold_phi(0)
            wt_ref[3] = pltpu.bitcast(wo_ref[...], u32)

        rr = lax.broadcasted_iota(jnp.int32, (PR + 8, 2 * PR), 0)
        cc = lax.broadcasted_iota(jnp.int32, (PR + 8, 2 * PR), 1)
        second = ((rr >= DA) & (rr < PR)) | ((rr >= PR) & ((rr & 1) == 1))
        same_head = second == ((cc & 1) == 1)
        for j in range(HA // 2):
            kvt_ref[j] = jnp.where(same_head, kvt_ref[j], 0.0)

        def ln_b(i):
            xn = _layernorm(xres_ref[rows(i, HT), :])
            xnb_ref[rows(i, HT), :] = xn
            return pltpu.bitcast(functools.reduce(
                jnp.add, [xn[8 * t:8 * (t + 1), D - 128:] for t in range(HT // 8)]), u32)

        def phase2(prep, b, carry):
            NH = (T2 if prep else T2B) // HT
            if prep:
                @pl.when(b == N2 // 4)
                def _():
                    cp_wob.start(priority=1)

                for m in range(3):
                    cp_b(m, b).wait()

                for j in range(CH // PW):
                    p = b * (CH // PW) + j
                    for m in range(3):
                        r0 = m * CH + j * PW
                        if m == 2:
                            blk = jnp.concatenate(
                                [stage_ref[b, r0 + r:r0 + r + 64, :] for r in _INTERLEAVE], axis=0)
                        else:
                            blk = stage_ref[b, r0:r0 + PW, :]
                        wb_ref[p, :, m * PW:(m + 1) * PW] = pltpu.bitcast(blk.T, u32)

            never = lax.broadcasted_iota(jnp.int32, (8, 128), 0) > b + 64
            dep = (never, ln_b(jnp.maximum(NH * b - 1, 0)))
            sub = lax.broadcasted_iota(jnp.int32, (8, HT), 0)
            top, even = sub < 4, (sub & 1) == 0
            pq, ot, o, y = {}, {}, {}, {}

            def proj_q(i, g, dep=None):
                xn = pltpu.bitcast(xna_ref[NH * b + i], bf16)
                pq[i, g] = jnp.dot(wt(0, g, dep), xn, preferred_element_type=f32)

            def num(i, g):
                parts = []
                for j in range(GR // PR):
                    ep, en, sp, sn = _hedgehog(pq[i, g][j * PR:(j + 1) * PR])
                    ratio = sp * _recip(sn)
                    phiq = jnp.concatenate(ep + [e * ratio for e in en], axis=0).astype(bf16)
                    n = jnp.dot(kvt_ref[g * (GR // PR) + j], phiq, preferred_element_type=f32)
                    r = _recip(n[PR:, :] + 1e-6 * sp)
                    rs = pltpu.roll(r, 1, 0)
                    ra, rb = jnp.where(even, r, rs), jnp.where(even, rs, r)
                    parts += [n[8 * t:8 * (t + 1), :] * rr_
                              for t, rr_ in enumerate((ra, ra, jnp.where(top, ra, rb), rb, rb))]
                ot[i, g] = jnp.concatenate(parts, axis=0).astype(bf16)

            def out(i, k0, k1, c0=0, c1=D):
                if i not in o:
                    o_ref[i + (b >> 8)] = pltpu.bitcast(
                        jnp.concatenate([ot[i, g] for g in range(NG)], axis=0).T, u32)
                    o[i] = pltpu.bitcast(o_ref[i + (b >> 8)], bf16)
                    y[i] = {}
                if (c0, c1) not in y[i]:
                    y[i][c0, c1] = x_ref[rows(NH * b + i, HT), c0:c1].astype(f32)
                y[i][c0, c1] = y[i][c0, c1] + jnp.dot(
                    o[i][:, k0:k1], pltpu.bitcast(wt_ref[3, k0 // 2:k1 // 2, c0:c1], bf16),
                    preferred_element_type=f32)

            def finish(i, ln):
                xi = jnp.concatenate([y[i][c] for c in sorted(y[i])], axis=1)
                xres_ref[rows(NH * b + i, HT), :] = xi
                if ln:
                    xnb_ref[rows(NH * b + i, HT), :] = _layernorm(xi)

            proj_q(0, 0); proj_q(0, 1); proj_q(0, 2, dep); num(0, 0); proj_q(0, 3); num(0, 1)
            proj_q(1, 0); num(0, 2); proj_q(1, 1); num(0, 3); proj_q(1, 2); num(1, 0)
            proj_q(1, 3); num(1, 1)
            for i in range(2, NH):
                proj_q(i, 0); num(i - 1, 2); proj_q(i, 1); num(i - 1, 3)
                out(i - 2, 0, D); finish(i - 2, True)
                proj_q(i, 2); num(i, 0); proj_q(i, 3); num(i, 1)
            i = NH - 2
            out(i, 0, D, 0, 128); num(i + 1, 2); out(i, 0, D, 128, 256); num(i + 1, 3)
            out(i, 0, D, 256, D); finish(i, True)
            out(i + 1, 0, 384); out(i + 1, 384, D); finish(i + 1, False)
            return carry

        n_prep = jnp.where(first, N2, 0)
        lax.fori_loop(0, n_prep, functools.partial(phase2, True), 0)
        lax.fori_loop(0, jnp.where(first, 0, S // T2B), functools.partial(phase2, False), 0)

        def pre(i, carry):
            w = pltpu.bitcast(wb_ref[NP - 1, :, 3 * PW - NPRE:], bf16)
            pre_ref[rows(i, PB), :] = jnp.dot(xnb_ref[rows(i, PB), :], w, preferred_element_type=f32)
            ln_b(S // HT - 1)
            return carry

        lax.fori_loop(0, S // PB, pre, 0)

        @pl.when(first)
        def _():
            cp_mem.wait()
            cp_wob.wait()

            def pack(p, carry):
                for i, r in enumerate(_INTERLEAVE):
                    src = wob_ref[pl.ds(pl.multiple_of(p * PW + r, 64), 64), :]
                    wo2_ref[p, 32 * i:32 * (i + 1), :] = pltpu.bitcast(src, u32)
                return carry

            lax.fori_loop(0, NP, pack, 0)

    NI = NSEG // UNROLL
    out_at = [0, NI // 4, NI // 2, 3 * NI // 4, NI - 1, NI]

    def out_copy(k):
        r = pl.ds(out_at[k] * UNROLL * SEG, (out_at[k + 1] - out_at[k]) * UNROLL * SEG)
        return pltpu.make_async_copy(x_ref.at[r], out_hbm.at[r], sem_o)

    def layer_b(last):
        mem_ref[...] = mem0_ref[...].astype(f32)
        LM = L - 8
        srow = lax.broadcasted_iota(jnp.int32, (LM, 2 * L), 0)
        scol = lax.broadcasted_iota(jnp.int32, (LM, 2 * L), 1)
        first = scol < L
        kidx = jnp.where(first, scol, scol - L)
        mask = (srow < MEM) | (srow + 8 >= kidx)
        lo40 = lax.broadcasted_iota(jnp.int32, (L, PW), 1) % 128 < 64
        lo32 = lax.broadcasted_iota(jnp.int32, (LM, 128), 1) < 64
        lo8 = lax.broadcasted_iota(jnp.int32, (8, 128), 1) < 64
        sub8 = lax.broadcasted_iota(jnp.int32, (8, 128), 0)
        never = sub8 > last.astype(jnp.int32) + 128
        lane8 = lax.broadcasted_iota(jnp.int32, (8, 128), 1)
        first8 = lane8 < L
        kidx8 = jnp.where(first8, lane8, lane8 - L)
        bits = [((sub8 - kidx8) & bb) != 0 for bb in (1, 2, 4)]
        NA = 384

        def softmax(s):
            s = jnp.where(mask, s * scale, -1e9)
            m1 = jnp.max(jnp.where(first, s, -jnp.inf), axis=1, keepdims=True)
            m2 = jnp.max(jnp.where(first, -jnp.inf, s), axis=1, keepdims=True)
            e = jnp.exp(s - jnp.where(first, m1, m2))
            l1 = jnp.sum(jnp.where(first, e, 0.0), axis=1, keepdims=True)
            l2 = jnp.sum(jnp.where(first, 0.0, e), axis=1, keepdims=True)
            return e, _recip(jnp.where(lo32, l1, l2))

        pre_at = {0: (0, 256), 1: (256, 512), 2: (512, D)}

        def step(s, mem):
            def rot(x, j, t, dep):
                blk = x[8 * (j // 8):8 * (j // 8) + 8, 128 * t:128 * (t + 1)]
                if dep is not None:
                    blk = jnp.where(never, dep, blk)
                return pltpu.roll(blk, j % 8, 0) if j % 8 else blk

            def split_q(qg):
                return (qg[:, :128], jnp.where(lo8, qg[:, 128:256], 0.0),
                        jnp.where(lo8, 0.0, qg[:, 128:256]), qg[:, 256:])

            def vpu_attn(q, k, v, more):
                qs = [split_q(q[MEM:MEM + 8] * (scale * LOG2E))]
                if more:
                    qs.append(split_q(q[MEM + 8:MEM + 16]))
                win = 10 if more else 14
                done, cols, extra, d1, d2 = [], [], [], None, None
                for j in range(MEM + 8 * len(qs)):
                    k0 = rot(k, j, 0, done[j - win] if j >= win else d1)
                    k1, k2 = rot(k, j, 1, d2), rot(k, j, 2, d1)
                    res = []
                    for g, (a0, a1, b1, b2) in enumerate(qs):
                        if j < MEM + 8 * (g + 1):
                            p1 = a0 * k0 + a1 * k1
                            p2 = b1 * k1 + b2 * k2
                            sc = jnp.where(first8 if g else lo8, jnp.sum(p1, axis=1, keepdims=True),
                                           jnp.sum(p2, axis=1, keepdims=True))
                            res.append((p1, p2, sc))
                            if g:
                                extra.append(sc)
                            else:
                                cols.append(jnp.where(sub8 >= j - MEM, sc, -1e9 * LOG2E)
                                            if j > MEM else sc)
                    d1, d2, dn = (functools.reduce(jnp.maximum, x) for x in zip(*res))
                    done.append(dn)
                if more:
                    for mk in bits:
                        extra = [jnp.where(mk, extra[i + 1], extra[i]) for i in range(0, len(extra), 2)]
                    x = extra[0]
                    for i in (1, 2):
                        x = jnp.where(kidx8 >= 8 * i, extra[i], x)
                    extra = [x[:, :2 * L]]
                m = functools.reduce(jnp.maximum, cols)
                accs, l = [None] * 3, None
                for j in range(MEM + 8):
                    e = jnp.exp2(cols[j] - m)
                    l = e if j == 0 else l + e
                    for t in range(3):
                        dep = accs[(2, 1, 0)[t]]
                        x = e * rot(v, j, t, e if dep is None else dep)
                        accs[t] = x if j == 0 else accs[t] + x
                rl = _recip(l)
                return jnp.concatenate([x * rl for x in accs], axis=1), extra

            r = rows(s, SEG)
            h = jnp.concatenate([mem, xnb_ref[r, :]], axis=0)
            qkv, pr, os_, ov, sv, pm = {}, {}, {}, {}, {}, []
            acc = {(0, NA): None, (NA, D): None}
            for c0, c1 in acc:
                acc[c0, c1] = jnp.concatenate(
                    [jnp.zeros((MEM, c1 - c0), f32), xres_ref[r, c0:c1]], axis=0)

            def proj(t):
                w = pltpu.bitcast(wb_ref[t], bf16)
                if t == 0:
                    part = jnp.dot(h[:, :NA], w[:NA], preferred_element_type=f32)
                    part = jnp.concatenate([part[:, :128], part[:, 128:]], axis=1)
                    qkv[t] = part + jnp.dot(h[:, NA:], w[NA:], preferred_element_type=f32)
                elif t == NP - 1:
                    tail = jnp.concatenate([pm[0], pre_ref[r, :]], axis=0)
                    qkv[t] = jnp.concatenate(
                        [jnp.dot(h, w[:, :3 * PW - NPRE], preferred_element_type=f32), tail], axis=1)
                else:
                    qkv[t] = jnp.dot(h, w, preferred_element_type=f32)
                ov[t], sv[t] = vpu_attn(qkv[t][:, :PW], qkv[t][:, PW:2 * PW], qkv[t][:, 2 * PW:],
                                        t < NP - 2)
                if t in pre_at:
                    k0, k1 = pre_at[t]
                    w = pltpu.bitcast(wb_ref[NP - 1, k0 // 2:k1 // 2, 3 * PW - NPRE:], bf16)
                    y = jnp.dot(mem[:, k0:k1], w, preferred_element_type=f32)
                    pm[:] = [pm[0] + y if pm else jnp.concatenate([y[:, :128], y[:, 128:]], axis=1)]

            def scores(t):
                q, k = qkv[t][:, :PW], qkv[t][:, PW:2 * PW]
                qm = jnp.concatenate([q[:MEM], q[MEM + 8 * (1 + len(sv[t])):]], axis=0)
                sm = lax.dot_general(qm, _blockdiag(k).astype(bf16), _NT, preferred_element_type=f32)
                pr[t] = softmax(jnp.concatenate([sm[:MEM]] + sv[t] + [sm[MEM:]], axis=0))

            def pv(t):
                v = qkv[t][:, 2 * PW:]
                vv = jnp.concatenate([jnp.where(lo40, v, 0.0), jnp.where(lo40, 0.0, v)], axis=0)
                e, rl = pr[t]
                om = jnp.dot(e.astype(bf16), vv.astype(bf16), preferred_element_type=f32)
                om = om * jnp.concatenate([rl] * 3, axis=1)
                os_[t] = jnp.concatenate([om[:MEM], ov[t], om[MEM:]], axis=0)

            def oproj(late, p0, p1):
                c0, c1 = (NA, D) if late else (0, NA)
                o = jnp.concatenate([os_[p] for p in range(p0, p1)], axis=1)
                w = pltpu.bitcast(jnp.concatenate(
                    [wo2_ref[p, :, c0:c1] for p in range(p0, p1)], axis=0), bf16)
                acc[c0, c1] = acc[c0, c1] + jnp.dot(o, w, preferred_element_type=f32)

            for t in range(NP):
                proj(t)
                if t >= 1:
                    scores(t - 1)
                if t >= 2:
                    pv(t - 2)
                if t >= 4:
                    oproj(False, t - 4, t - 3)
            oproj(True, 0, 3); scores(NP - 1); oproj(False, NP - 4, NP - 3)
            oproj(True, 3, 5); pv(NP - 2); oproj(True, 5, 7)
            oproj(False, NP - 3, NP - 2); oproj(True, 7, 9); oproj(False, NP - 2, NP - 1)
            pv(NP - 1); oproj(True, 9, 12); oproj(False, NP - 1, NP); oproj(True, 12, NP)
            y = jnp.concatenate([acc[0, NA], acc[NA, D]], axis=1)
            x_ref[r, :] = y[MEM:].astype(bf16)
            return y[:MEM]

        def steps(i, carry):
            for k in range(len(out_at) - 2):
                @pl.when(last & (i == out_at[k + 1]))
                def _():
                    out_copy(k).start()

            mem_ref[...] = lax.fori_loop(0, UNROLL, lambda u, mem: step(i * UNROLL + u, mem),
                                         mem_ref[...], unroll=True)
            return carry

        lax.fori_loop(0, NI, steps, 0)

    def layer(i, carry):
        layer_a(i == 0)
        layer_b(i == 1)
        return carry

    lax.fori_loop(0, 2, layer, 0)
    out_copy(len(out_at) - 2).start()
    for k in range(len(out_at) - 1):
        out_copy(k).wait()


@jax.jit
def pallas_interleave_layers__linear_kernel_hedgehog__memory_aug_recurrent_mem_tr__prompt_kernel(
    A_x, A_wqkv, A_w_phi, A_wo, B_x, B_mem0, B_Wq, B_Wk, B_Wv, B_Wo, B_seg_len=SEG,
):
    del B_x
    del B_seg_len
    x = A_x.reshape(S, D)
    wp = A_w_phi.transpose(1, 2, 0)
    mem0 = B_mem0.reshape(MEM, D)
    wqt, wkt, wvt = (w.transpose(1, 2, 0).reshape(HB * DB, D) for w in (B_Wq, B_Wk, B_Wv))
    wob = B_Wo.reshape(HB * DB, D)

    hbm = pl.BlockSpec(memory_space=pl.ANY)
    out = pl.pallas_call(
        _kernel,
        out_shape=jax.ShapeDtypeStruct((S, D), bf16),
        in_specs=[hbm] * 9,
        out_specs=hbm,
        scratch_shapes=[
            pltpu.VMEM((S, D), bf16),
            pltpu.VMEM((D, 3 * D), bf16),
            pltpu.VMEM((DA, DA, HA), bf16),
            pltpu.VMEM((D, D), bf16),
            pltpu.VMEM((MEM, D), bf16),
            pltpu.VMEM((S, D), f32),
            pltpu.VMEM((S, D), f32),
            pltpu.VMEM((S // 128, D // 2, 128), u32),
            pltpu.VMEM((4, D // 2, D), u32),
            pltpu.VMEM((PR, D), f32),
            pltpu.VMEM((HA // 2, PR + 8, 2 * PR), f32),
            pltpu.VMEM((T2B // 128, 64, D), u32),
            pltpu.VMEM((N2, 3 * HB * DB // N2, D), bf16),
            pltpu.VMEM((HB * DB, D), bf16),
            pltpu.VMEM((NP, PW // 2, D), u32),
            pltpu.VMEM((NP, D // 2, 3 * PW), u32),
            pltpu.VMEM((S, NPRE), f32),
            pltpu.VMEM((MEM, D), f32),
            pltpu.SemaphoreType.DMA((10,)),
            pltpu.SemaphoreType.DMA((N2,)),
            pltpu.SemaphoreType.DMA,
        ],
        compiler_params=pltpu.CompilerParams(vmem_limit_bytes=110 * 1024 * 1024),
    )(x, A_wqkv, wp, A_wo, mem0, wqt, wkt, wvt, wob)
    return out.reshape(1, S, D)
```

```python
import functools

import jax
import jax.numpy as jnp
from jax import lax
import jax.experimental.pallas as pl
import jax.experimental.pallas.tpu as pltpu

f32 = jnp.float32
bf16 = jnp.bfloat16
u32 = jnp.uint32

S = 2048
D = 640
HA = 32
DA = D // HA
HB = 32
DB = 192
MEM = 8
SEG = 32
L = MEM + SEG
NSEG = S // SEG
NP = HB // 2
PW = 2 * DB
NG = 4
PR = 2 * DA
GR = D // NG
TB = 256
NB = S // TB
T2 = 256
N2 = S // T2
T2B = 512
LN_EPS = 1e-5
PB = 1024
NW = 4
NPRE = 256
LOG2E = 1.4426950408889634
UNROLL = 4

_NT = (((1,), (1,)), ((), ()))
_INTERLEAVE = [h * DB + c * 64 for c in range(3) for h in range(2)]


def _layernorm(x):
    m = jnp.mean(x, axis=-1, keepdims=True)
    xc = x - m
    v = jnp.mean(xc * xc, axis=-1, keepdims=True)
    return xc * lax.rsqrt(v + LN_EPS)


def _recip(x):
    r = pl.reciprocal(x, approx=True)
    return r * (2.0 - x * r)


def _fold(op, rows):
    r = functools.reduce(op, rows)
    r = op(r, pltpu.roll(r, 4, 0))
    return op(r, pltpu.roll(r, 2, 0))


def _hedgehog(p):
    rows = [p[8 * i:8 * (i + 1), :] for i in range(PR // 8)]
    mx = _fold(jnp.maximum, rows)
    mn = _fold(jnp.minimum, rows)
    ep = [jnp.exp2(r - mx) for r in rows]
    en = [jnp.exp2(mn - r) for r in rows]
    return ep, en, _fold(jnp.add, ep), _fold(jnp.add, en)


def _blockdiag(x):
    t0, t1, t2 = x[:, :128], x[:, 128:256], x[:, 256:]
    lane = lax.broadcasted_iota(jnp.int32, (L, 128), 1)
    z = jnp.zeros((L, 128), f32)
    top = jnp.concatenate([t0, jnp.where(lane < 64, t1, 0.0), z], axis=1)
    bot = jnp.concatenate([z, jnp.where(lane >= 64, t1, 0.0), t2], axis=1)
    return jnp.concatenate([top, bot], axis=0)


def _kernel(x_hbm, wqkv_hbm, wphi_hbm, wo_hbm, mem0_hbm, wqt_hbm, wkt_hbm, wvt_hbm, wob_hbm,
            out_hbm,
            x_ref, wqkv_ref, wphi_ref, wo_ref, mem0_ref, xres_ref, xnb_ref, xna_ref, wt_ref, wp2_ref,
            kvt_ref, o_ref, stage_ref, wob_ref, wo2_ref, wb_ref, pre_ref, mem_ref, sem_a, sem_b, sem_w, sem_o):
    scale = DB ** -0.5
    XH = 2 * TB
    HT = 128
    CH = HB * DB // N2

    cp_x0 = pltpu.make_async_copy(x_hbm.at[:TB], x_ref.at[:TB], sem_a.at[0])
    cp_k = pltpu.make_async_copy(wqkv_hbm.at[:, D:2 * D], wqkv_ref.at[:, D:2 * D], sem_a.at[1])
    cp_v = pltpu.make_async_copy(wqkv_hbm.at[:, 2 * D:], wqkv_ref.at[:, 2 * D:], sem_a.at[8])
    cp_x0b = pltpu.make_async_copy(x_hbm.at[TB:XH], x_ref.at[TB:XH], sem_a.at[5])
    cp_x1 = pltpu.make_async_copy(x_hbm.at[XH:], x_ref.at[XH:], sem_a.at[2])
    cp_q = pltpu.make_async_copy(wqkv_hbm.at[:, :D], wqkv_ref.at[:, :D], sem_a.at[3])
    cp_wo = pltpu.make_async_copy(wo_hbm, wo_ref, sem_a.at[4])
    cp_phi = pltpu.make_async_copy(wphi_hbm, wphi_ref, sem_a.at[6])
    cp_mem = pltpu.make_async_copy(mem0_hbm, mem0_ref, sem_a.at[7])

    def rows(b, n=TB):
        return pl.ds(b * n if isinstance(b, int) else pl.multiple_of(b * n, n), n)

    def cp_b(m, c):
        src = (wqt_hbm, wkt_hbm, wvt_hbm)[m]
        return pltpu.make_async_copy(src.at[rows(c, CH)], stage_ref.at[c, m * CH:(m + 1) * CH],
                                     sem_b.at[c])

    WQ = HB * DB // NW

    def cp_wob(i):
        return pltpu.make_async_copy(wob_hbm.at[rows(i, WQ)], wob_ref.at[i], sem_w.at[i])

    for c in (cp_phi, cp_x0, cp_k, cp_mem):
        c.start()
    for m in range(3):
        cp_b(m, 0).start(priority=1)

    xres_ref[:HT, :] = jnp.zeros((HT, D), f32)
    cp_phi.wait()
    cp_v.start()
    hrow = lax.broadcasted_iota(jnp.int32, (HA, D), 0)
    hcol = lax.broadcasted_iota(jnp.int32, (HA, D), 1)

    def expand(i, wp):
        for d in (4 * i, 4 * i + 1, 4 * i + 2, 4 * i + 3):
            sel = jnp.where(hcol == hrow * DA + d, 1.0, 0.0)
            wp = wp + jnp.dot(wphi_ref[d].astype(f32), sel, preferred_element_type=f32)
        return wp

    wp = lax.fori_loop(0, DA // 4, expand, jnp.zeros((DA, D), f32))
    dup = jnp.where((lax.broadcasted_iota(jnp.int32, (PR, DA), 0) >> 1)
                    == lax.broadcasted_iota(jnp.int32, (PR, DA), 1), 1.0, 0.0)
    wp2_ref[...] = jnp.dot(dup, wp, preferred_element_type=f32)
    cp_x0.wait()

    def fold_phi(m):
        row = lax.broadcasted_iota(jnp.int32, (PR, 128), 0)
        col = lax.broadcasted_iota(jnp.int32, (PR, 128), 1)
        parts = []
        for t in range(D // 128):
            blocks = []
            for j in range(3 * t, 3 * t + 4):
                lo = (2 * j + (row & 1)) * DA - 128 * t
                blocks.append(jnp.where((col >= lo) & (col < lo + DA),
                                        wp2_ref[:, 128 * t:128 * (t + 1)], 0.0))
            w = wqkv_ref[:, m * D + 128 * t:m * D + 128 * (t + 1)]
            parts.append(lax.dot_general(jnp.concatenate(blocks, axis=0).astype(bf16), w, _NT,
                                         preferred_element_type=f32))
        out = [parts[0][:PR]]
        for t in range(D // 128):
            out.append(parts[t][PR:3 * PR])
            last = parts[t][3 * PR:]
            out.append(last + parts[t + 1][:PR] if t + 1 < D // 128 else last)
        wt_ref[m] = pltpu.bitcast((jnp.concatenate(out, axis=0) * LOG2E).astype(bf16), u32)

    def wt(m, g, dep=None):
        w = wt_ref[m, g * GR // 2:(g + 1) * GR // 2, :]
        if dep is not None:
            never, val = dep
            top = jnp.concatenate([jnp.where(never, val, w[:8, :128]), w[:8, 128:]], axis=1)
            w = jnp.concatenate([top, w[8:]], axis=0)
        return pltpu.bitcast(w, bf16)

    def layer_a(first):
        def ln_a(i):
            xn = _layernorm(x_ref[rows(i, HT), :].astype(f32)).astype(bf16)
            xt = pltpu.bitcast(xn.T, u32)
            xna_ref[i] = xt
            return functools.reduce(jnp.bitwise_or, [xt[64 * t:64 * t + 8] for t in range(D // 128)])

        kvt_ref[...] = jnp.zeros(kvt_ref.shape, f32)
        xn0 = _layernorm(x_ref[:TB, :].astype(f32)).astype(bf16).T
        for i in range(TB // HT):
            xna_ref[i] = pltpu.bitcast(xn0[:, i * HT:(i + 1) * HT], u32)

        @pl.when(first)
        def _():
            cp_x0b.start()
            cp_k.wait()
            cp_v.wait()
            fold_phi(1)
            wt_ref[2] = pltpu.bitcast(wqkv_ref[:, 2 * D:].T, u32)
            cp_x1.start()
            cp_x0b.wait()

        def phase1(b, carry):
            @pl.when(first & (b == XH // TB - 1))
            def _():
                cp_x1.wait()
                cp_q.start()
                cp_wo.start()

            for c in range(1, N2):
                @pl.when(first & (b == (c - 1) * NB // N2))
                def _():
                    for m in range(3):
                        cp_b(m, c).start(priority=1)

            xn = pltpu.bitcast(jnp.concatenate(
                [xna_ref[(TB // HT) * b + i] for i in range(TB // HT)], axis=1), bf16)
            ones = jnp.ones((8, TB), f32)
            pk, v1 = {}, {}

            never = lax.broadcasted_iota(jnp.int32, (8, 128), 0) > b + 64

            def proj_k(g, dep=None):
                pk[g] = jnp.dot(wt(1, g, dep), xn, preferred_element_type=f32)

            def proj_v(g, dep=None):
                v1[g] = jnp.dot(wt(2, g, dep), xn, preferred_element_type=f32)

            def kv(g):
                for j in range(GR // PR):
                    ep, en, sp, sn = _hedgehog(pk[g][j * PR:(j + 1) * PR])
                    rp, rn = _recip(sp), _recip(sn)
                    phik = jnp.concatenate([e * rp for e in ep] + [e * rn for e in en],
                                           axis=0).astype(bf16)
                    lhs = jnp.concatenate([v1[g][j * PR:(j + 1) * PR], ones], axis=0)
                    kvt_ref[g * (GR // PR) + j] += lax.dot_general(
                        lhs, phik, _NT, preferred_element_type=f32)

            nxt = jnp.minimum(b + 1, NB - 1) * (TB // HT)
            dep = [(never, ln_a(nxt + i)) for i in range(TB // HT)]
            proj_k(0); proj_k(1); proj_v(0); proj_k(2); proj_v(1, dep[0]); kv(0)
            proj_k(3); proj_v(2); proj_v(3); kv(1); kv(2); kv(3)
            return carry

        lax.fori_loop(0, NB, phase1, 0)

        @pl.when(first)
        def _():
            cp_q.wait()
            cp_wo.wait()
            fold_phi(0)
            wt_ref[3] = pltpu.bitcast(wo_ref[...], u32)

        rr = lax.broadcasted_iota(jnp.int32, (PR + 8, 2 * PR), 0)
        cc = lax.broadcasted_iota(jnp.int32, (PR + 8, 2 * PR), 1)
        second = ((rr >= DA) & (rr < PR)) | ((rr >= PR) & ((rr & 1) == 1))
        same_head = second == ((cc & 1) == 1)
        for j in range(HA // 2):
            kvt_ref[j] = jnp.where(same_head, kvt_ref[j], 0.0)

        def ln_b(i):
            xn = _layernorm(xres_ref[rows(i, HT), :])
            xnb_ref[rows(i, HT), :] = xn
            return pltpu.bitcast(functools.reduce(
                jnp.add, [xn[8 * t:8 * (t + 1), D - 128:] for t in range(HT // 8)]), u32)

        def phase2(prep, b, carry):
            NH = (T2 if prep else T2B) // HT
            if prep:
                for i in range(NW):
                    @pl.when(b == N2 - NW + i)
                    def _():
                        cp_wob(i).start(priority=1)

                for m in range(3):
                    cp_b(m, b).wait()

                for j in range(CH // PW):
                    p = b * (CH // PW) + j
                    for m in range(3):
                        r0 = m * CH + j * PW
                        if m == 2:
                            blk = jnp.concatenate(
                                [stage_ref[b, r0 + r:r0 + r + 64, :] for r in _INTERLEAVE], axis=0)
                        else:
                            blk = stage_ref[b, r0:r0 + PW, :]
                        wb_ref[p, :, m * PW:(m + 1) * PW] = pltpu.bitcast(blk.T, u32)

            never = lax.broadcasted_iota(jnp.int32, (8, 128), 0) > b + 64
            dep = (never, ln_b(jnp.maximum(NH * b - 1, 0)))
            sub = lax.broadcasted_iota(jnp.int32, (8, HT), 0)
            top, even = sub < 4, (sub & 1) == 0
            pq, ot, o, y = {}, {}, {}, {}

            def proj_q(i, g, dep=None):
                xn = pltpu.bitcast(xna_ref[NH * b + i], bf16)
                pq[i, g] = jnp.dot(wt(0, g, dep), xn, preferred_element_type=f32)

            def num(i, g):
                parts = []
                for j in range(GR // PR):
                    ep, en, sp, sn = _hedgehog(pq[i, g][j * PR:(j + 1) * PR])
                    ratio = sp * _recip(sn)
                    phiq = jnp.concatenate(ep + [e * ratio for e in en], axis=0).astype(bf16)
                    n = jnp.dot(kvt_ref[g * (GR // PR) + j], phiq, preferred_element_type=f32)
                    r = _recip(n[PR:, :] + 1e-6 * sp)
                    rs = pltpu.roll(r, 1, 0)
                    ra, rb = jnp.where(even, r, rs), jnp.where(even, rs, r)
                    parts += [n[8 * t:8 * (t + 1), :] * rr_
                              for t, rr_ in enumerate((ra, ra, jnp.where(top, ra, rb), rb, rb))]
                ot[i, g] = jnp.concatenate(parts, axis=0).astype(bf16)

            def out(i, k0, k1, c0=0, c1=D):
                if i not in o:
                    o_ref[i + (b >> 8)] = pltpu.bitcast(
                        jnp.concatenate([ot[i, g] for g in range(NG)], axis=0).T, u32)
                    o[i] = pltpu.bitcast(o_ref[i + (b >> 8)], bf16)
                    y[i] = {}
                if (c0, c1) not in y[i]:
                    y[i][c0, c1] = x_ref[rows(NH * b + i, HT), c0:c1].astype(f32)
                y[i][c0, c1] = y[i][c0, c1] + jnp.dot(
                    o[i][:, k0:k1], pltpu.bitcast(wt_ref[3, k0 // 2:k1 // 2, c0:c1], bf16),
                    preferred_element_type=f32)

            def finish(i, ln):
                xi = jnp.concatenate([y[i][c] for c in sorted(y[i])], axis=1)
                xres_ref[rows(NH * b + i, HT), :] = xi
                if ln:
                    xnb_ref[rows(NH * b + i, HT), :] = _layernorm(xi)

            proj_q(0, 0); proj_q(0, 1); proj_q(0, 2, dep); num(0, 0); proj_q(0, 3); num(0, 1)
            proj_q(1, 0); num(0, 2); proj_q(1, 1); num(0, 3); proj_q(1, 2); num(1, 0)
            proj_q(1, 3); num(1, 1)
            for i in range(2, NH):
                proj_q(i, 0); num(i - 1, 2); proj_q(i, 1); num(i - 1, 3)
                out(i - 2, 0, D); finish(i - 2, True)
                proj_q(i, 2); num(i, 0); proj_q(i, 3); num(i, 1)
            i = NH - 2
            out(i, 0, D, 0, 128); num(i + 1, 2); out(i, 0, D, 128, 256); num(i + 1, 3)
            out(i, 0, D, 256, D); finish(i, True)
            out(i + 1, 0, 384); out(i + 1, 384, D); finish(i + 1, False)
            return carry

        n_prep = jnp.where(first, N2, 0)
        lax.fori_loop(0, n_prep, functools.partial(phase2, True), 0)
        lax.fori_loop(0, jnp.where(first, 0, S // T2B), functools.partial(phase2, False), 0)

        def pre(prep, i, carry):
            n = S // NW if prep else PB
            if prep:
                cp_wob(i).wait()
                for j in range(WQ // PW):
                    for c, r in enumerate(_INTERLEAVE):
                        wo2_ref[i * (WQ // PW) + j, 32 * c:32 * (c + 1), :] = pltpu.bitcast(
                            wob_ref[i, j * PW + r:j * PW + r + 64, :], u32)
            w = pltpu.bitcast(wb_ref[NP - 1, :, 3 * PW - NPRE:], bf16)
            pre_ref[rows(i, n), :] = jnp.dot(xnb_ref[rows(i, n), :], w, preferred_element_type=f32)
            ln_b(S // HT - 1)
            return carry

        lax.fori_loop(0, jnp.where(first, NW, 0), functools.partial(pre, True), 0)
        lax.fori_loop(0, jnp.where(first, 0, S // PB), functools.partial(pre, False), 0)

        @pl.when(first)
        def _():
            cp_mem.wait()

    NI = NSEG // UNROLL
    out_at = [0, NI // 4, NI // 2, 3 * NI // 4, NI - 1, NI]

    def out_copy(k):
        r = pl.ds(out_at[k] * UNROLL * SEG, (out_at[k + 1] - out_at[k]) * UNROLL * SEG)
        return pltpu.make_async_copy(x_ref.at[r], out_hbm.at[r], sem_o)

    def layer_b(last):
        mem_ref[...] = mem0_ref[...].astype(f32)
        LM = L - 8
        srow = lax.broadcasted_iota(jnp.int32, (LM, 2 * L), 0)
        scol = lax.broadcasted_iota(jnp.int32, (LM, 2 * L), 1)
        first = scol < L
        kidx = jnp.where(first, scol, scol - L)
        mask = (srow < MEM) | (srow + 8 >= kidx)
        lo40 = lax.broadcasted_iota(jnp.int32, (L, PW), 1) % 128 < 64
        lo32 = lax.broadcasted_iota(jnp.int32, (LM, 128), 1) < 64
        lo8 = lax.broadcasted_iota(jnp.int32, (8, 128), 1) < 64
        sub8 = lax.broadcasted_iota(jnp.int32, (8, 128), 0)
        never = sub8 > last.astype(jnp.int32) + 128
        lane8 = lax.broadcasted_iota(jnp.int32, (8, 128), 1)
        first8 = lane8 < L
        kidx8 = jnp.where(first8, lane8, lane8 - L)
        bits = [((sub8 - kidx8) & bb) != 0 for bb in (1, 2, 4)]
        NA = 384

        def softmax(s):
            s = jnp.where(mask, s * scale, -1e9)
            m1 = jnp.max(jnp.where(first, s, -jnp.inf), axis=1, keepdims=True)
            m2 = jnp.max(jnp.where(first, -jnp.inf, s), axis=1, keepdims=True)
            e = jnp.exp(s - jnp.where(first, m1, m2))
            l1 = jnp.sum(jnp.where(first, e, 0.0), axis=1, keepdims=True)
            l2 = jnp.sum(jnp.where(first, 0.0, e), axis=1, keepdims=True)
            return e, _recip(jnp.where(lo32, l1, l2))

        pre_at = {0: (0, 256), 1: (256, 512), 2: (512, D)}

        def step(s, mem):
            def rot(x, j, t, dep):
                blk = x[8 * (j // 8):8 * (j // 8) + 8, 128 * t:128 * (t + 1)]
                if dep is not None:
                    blk = jnp.where(never, dep, blk)
                return pltpu.roll(blk, j % 8, 0) if j % 8 else blk

            def split_q(qg):
                return (qg[:, :128], jnp.where(lo8, qg[:, 128:256], 0.0),
                        jnp.where(lo8, 0.0, qg[:, 128:256]), qg[:, 256:])

            def vpu_attn(q, k, v, more):
                qs = [split_q(q[MEM:MEM + 8] * (scale * LOG2E))]
                if more:
                    qs.append(split_q(q[MEM + 8:MEM + 16]))
                win = 10 if more else 14
                done, cols, extra, d1, d2 = [], [], [], None, None
                for j in range(MEM + 8 * len(qs)):
                    k0 = rot(k, j, 0, done[j - win] if j >= win else d1)
                    k1, k2 = rot(k, j, 1, d2), rot(k, j, 2, d1)
                    res = []
                    for g, (a0, a1, b1, b2) in enumerate(qs):
                        if j < MEM + 8 * (g + 1):
                            p1 = a0 * k0 + a1 * k1
                            p2 = b1 * k1 + b2 * k2
                            sc = jnp.where(first8 if g else lo8, jnp.sum(p1, axis=1, keepdims=True),
                                           jnp.sum(p2, axis=1, keepdims=True))
                            res.append((p1, p2, sc))
                            if g:
                                extra.append(sc)
                            else:
                                cols.append(jnp.where(sub8 >= j - MEM, sc, -1e9 * LOG2E)
                                            if j > MEM else sc)
                    d1, d2, dn = (functools.reduce(jnp.maximum, x) for x in zip(*res))
                    done.append(dn)
                if more:
                    for mk in bits:
                        extra = [jnp.where(mk, extra[i + 1], extra[i]) for i in range(0, len(extra), 2)]
                    x = extra[0]
                    for i in (1, 2):
                        x = jnp.where(kidx8 >= 8 * i, extra[i], x)
                    extra = [x[:, :2 * L]]
                m = functools.reduce(jnp.maximum, cols)
                accs, l = [None] * 3, None
                for j in range(MEM + 8):
                    e = jnp.exp2(cols[j] - m)
                    l = e if j == 0 else l + e
                    for t in range(3):
                        dep = accs[(2, 1, 0)[t]]
                        x = e * rot(v, j, t, e if dep is None else dep)
                        accs[t] = x if j == 0 else accs[t] + x
                rl = _recip(l)
                return jnp.concatenate([x * rl for x in accs], axis=1), extra

            r = rows(s, SEG)
            h = jnp.concatenate([mem, xnb_ref[r, :]], axis=0)
            qkv, pr, os_, ov, sv, pm = {}, {}, {}, {}, {}, []
            acc = {(0, NA): None, (NA, D): None}
            for c0, c1 in acc:
                acc[c0, c1] = jnp.concatenate(
                    [jnp.zeros((MEM, c1 - c0), f32), xres_ref[r, c0:c1]], axis=0)

            def proj(t):
                w = pltpu.bitcast(wb_ref[t], bf16)
                if t == 0:
                    part = jnp.dot(h[:, :NA], w[:NA], preferred_element_type=f32)
                    part = jnp.concatenate([part[:, :128], part[:, 128:]], axis=1)
                    qkv[t] = part + jnp.dot(h[:, NA:], w[NA:], preferred_element_type=f32)
                elif t == NP - 1:
                    tail = jnp.concatenate([pm[0], pre_ref[r, :]], axis=0)
                    qkv[t] = jnp.concatenate(
                        [jnp.dot(h, w[:, :3 * PW - NPRE], preferred_element_type=f32), tail], axis=1)
                else:
                    qkv[t] = jnp.dot(h, w, preferred_element_type=f32)
                ov[t], sv[t] = vpu_attn(qkv[t][:, :PW], qkv[t][:, PW:2 * PW], qkv[t][:, 2 * PW:],
                                        t < NP - 2)
                if t in pre_at:
                    k0, k1 = pre_at[t]
                    w = pltpu.bitcast(wb_ref[NP - 1, k0 // 2:k1 // 2, 3 * PW - NPRE:], bf16)
                    y = jnp.dot(mem[:, k0:k1], w, preferred_element_type=f32)
                    pm[:] = [pm[0] + y if pm else jnp.concatenate([y[:, :128], y[:, 128:]], axis=1)]

            def scores(t):
                q, k = qkv[t][:, :PW], qkv[t][:, PW:2 * PW]
                qm = jnp.concatenate([q[:MEM], q[MEM + 8 * (1 + len(sv[t])):]], axis=0)
                sm = lax.dot_general(qm, _blockdiag(k).astype(bf16), _NT, preferred_element_type=f32)
                pr[t] = softmax(jnp.concatenate([sm[:MEM]] + sv[t] + [sm[MEM:]], axis=0))

            def pv(t):
                v = qkv[t][:, 2 * PW:]
                vv = jnp.concatenate([jnp.where(lo40, v, 0.0), jnp.where(lo40, 0.0, v)], axis=0)
                e, rl = pr[t]
                om = jnp.dot(e.astype(bf16), vv.astype(bf16), preferred_element_type=f32)
                om = om * jnp.concatenate([rl] * 3, axis=1)
                os_[t] = jnp.concatenate([om[:MEM], ov[t], om[MEM:]], axis=0)

            def oproj(late, p0, p1):
                c0, c1 = (NA, D) if late else (0, NA)
                o = jnp.concatenate([os_[p] for p in range(p0, p1)], axis=1)
                w = pltpu.bitcast(jnp.concatenate(
                    [wo2_ref[p, :, c0:c1] for p in range(p0, p1)], axis=0), bf16)
                acc[c0, c1] = acc[c0, c1] + jnp.dot(o, w, preferred_element_type=f32)

            for t in range(NP):
                proj(t)
                if t >= 1:
                    scores(t - 1)
                if t >= 2:
                    pv(t - 2)
                if t >= 4:
                    oproj(False, t - 4, t - 3)
            oproj(True, 0, 3); scores(NP - 1); oproj(False, NP - 4, NP - 3)
            oproj(True, 3, 5); pv(NP - 2); oproj(True, 5, 7)
            oproj(False, NP - 3, NP - 2); oproj(True, 7, 9); oproj(False, NP - 2, NP - 1)
            pv(NP - 1); oproj(True, 9, 12); oproj(False, NP - 1, NP); oproj(True, 12, NP)
            y = jnp.concatenate([acc[0, NA], acc[NA, D]], axis=1)
            x_ref[r, :] = y[MEM:].astype(bf16)
            return y[:MEM]

        def steps(i, carry):
            for k in range(len(out_at) - 2):
                @pl.when(last & (i == out_at[k + 1]))
                def _():
                    out_copy(k).start()

            mem_ref[...] = lax.fori_loop(0, UNROLL, lambda u, mem: step(i * UNROLL + u, mem),
                                         mem_ref[...], unroll=True)
            return carry

        lax.fori_loop(0, NI, steps, 0)

    def layer(i, carry):
        layer_a(i == 0)
        layer_b(i == 1)
        return carry

    lax.fori_loop(0, 2, layer, 0)
    out_copy(len(out_at) - 2).start()
    for k in range(len(out_at) - 1):
        out_copy(k).wait()


@jax.jit
def pallas_interleave_layers__linear_kernel_hedgehog__memory_aug_recurrent_mem_tr__prompt_kernel(
    A_x, A_wqkv, A_w_phi, A_wo, B_x, B_mem0, B_Wq, B_Wk, B_Wv, B_Wo, B_seg_len=SEG,
):
    del B_x
    del B_seg_len
    x = A_x.reshape(S, D)
    wp = A_w_phi.transpose(1, 2, 0)
    mem0 = B_mem0.reshape(MEM, D)
    wqt, wkt, wvt = (w.transpose(1, 2, 0).reshape(HB * DB, D) for w in (B_Wq, B_Wk, B_Wv))
    wob = B_Wo.reshape(HB * DB, D)

    hbm = pl.BlockSpec(memory_space=pl.ANY)
    out = pl.pallas_call(
        _kernel,
        out_shape=jax.ShapeDtypeStruct((S, D), bf16),
        in_specs=[hbm] * 9,
        out_specs=hbm,
        scratch_shapes=[
            pltpu.VMEM((S, D), bf16),
            pltpu.VMEM((D, 3 * D), bf16),
            pltpu.VMEM((DA, DA, HA), bf16),
            pltpu.VMEM((D, D), bf16),
            pltpu.VMEM((MEM, D), bf16),
            pltpu.VMEM((S, D), f32),
            pltpu.VMEM((S, D), f32),
            pltpu.VMEM((S // 128, D // 2, 128), u32),
            pltpu.VMEM((4, D // 2, D), u32),
            pltpu.VMEM((PR, D), f32),
            pltpu.VMEM((HA // 2, PR + 8, 2 * PR), f32),
            pltpu.VMEM((T2B // 128, 64, D), u32),
            pltpu.VMEM((N2, 3 * HB * DB // N2, D), bf16),
            pltpu.VMEM((NW, HB * DB // NW, D), bf16),
            pltpu.VMEM((NP, PW // 2, D), u32),
            pltpu.VMEM((NP, D // 2, 3 * PW), u32),
            pltpu.VMEM((S, NPRE), f32),
            pltpu.VMEM((MEM, D), f32),
            pltpu.SemaphoreType.DMA((9,)),
            pltpu.SemaphoreType.DMA((N2,)),
            pltpu.SemaphoreType.DMA((NW,)),
            pltpu.SemaphoreType.DMA,
        ],
        compiler_params=pltpu.CompilerParams(vmem_limit_bytes=110 * 1024 * 1024),
    )(x, A_wqkv, wp, A_wo, mem0, wqt, wkt, wvt, wob)
    return out.reshape(1, S, D)
```
